```python
import jax
import jax.numpy as jnp

def _softmax(x, axis=-1):
    return jax.nn.softmax(x, axis=axis)

def _gelu(x):
    return jax.nn.gelu(x, approximate=True)

def _silu(x):
    return jax.nn.silu(x)

def _sigmoid(x):
    return jax.nn.sigmoid(x)

def _layernorm(x, axis=-1, eps=1e-05):
    m = jnp.mean(x, axis=axis, keepdims=True)
    v = jnp.var(x, axis=axis, keepdims=True)
    return (x - m) / jnp.sqrt(v + eps)

def _scatter_add(tgt, idx, src, axis=0):
    return tgt.at[idx].add(src)

def _segment_sum(src, seg, n):
    return jax.ops.segment_sum(src, seg, n)

class _Rng:

    def __init__(self, key):
        self._k = key

    def _next(self):
        self._k, sub = jax.random.split(self._k)
        return sub

    def normal(self, shape):
        return jax.random.normal(self._next(), shape, dtype=jnp.bfloat16)

    def randint(self, lo, hi, shape):
        return jax.random.randint(self._next(), shape, lo, hi, dtype=jnp.int32)

    def uniform(self, shape, lo=0.0, hi=1.0):
        return jax.random.uniform(self._next(), shape, jnp.bfloat16, lo, hi)

    def permutation(self, n):
        return jax.random.permutation(self._next(), n)
kernel_name = 'adaLN_cond__memory_aug_recurrent_mem_tr__dense_activation_gelu__prompt'

def setup_inputs():
    _rng = _Rng(jax.random.key(int.from_bytes(__import__("os").urandom(4), "little")))
    _w = lambda a: (lambda t: t.astype(jnp.bfloat16) if jnp.issubdtype(t.dtype, jnp.floating) else t)(jnp.asarray(a))

    def _A_setup():
        B, S, Dm = (1, 2048, 1024)
        H, Dh = (32, 128)
        M, seg = (8, 32)
        seg = min(seg, S)
        S = S // seg * seg
        return {'x': _w((lambda *s: _rng.normal(s) * 0.05)(B, S, Dm)), 'mem0': _w((lambda *s: _rng.normal(s) * 0.05)(B, M, Dm)), 'Wq': _w((lambda *s: _rng.normal(s) * 0.05)(Dm, H, Dh) * Dm ** (-0.5)), 'Wk': _w((lambda *s: _rng.normal(s) * 0.05)(Dm, H, Dh) * Dm ** (-0.5)), 'Wv': _w((lambda *s: _rng.normal(s) * 0.05)(Dm, H, Dh) * Dm ** (-0.5)), 'Wo': _w((lambda *s: _rng.normal(s) * 0.05)(H, Dh, Dm) * (H * Dh) ** (-0.5)), 'seg_len': seg}
    _A_in = _A_setup()

    def _B_setup():
        B, S, D, F = (1, 2048, 1024, 3584)
        return {'x': _w((lambda *s: _rng.normal(s) * 0.05)(B, S, D)), 'w1': _w((lambda *s: _rng.normal(s) * 0.05)(D, F) * D ** (-0.5)), 'b1': _w((lambda *s: _rng.normal(s) * 0.05)(F) * 0.01), 'w2': _w((lambda *s: _rng.normal(s) * 0.05)(F, D) * F ** (-0.5)), 'b2': _w((lambda *s: _rng.normal(s) * 0.05)(D) * 0.01)}
    _B_in = _B_setup()
    return {'A_x': _A_in['x'], 'A_mem0': _A_in['mem0'], 'A_Wq': _A_in['Wq'], 'A_Wk': _A_in['Wk'], 'A_Wv': _A_in['Wv'], 'A_Wo': _A_in['Wo'], 'A_seg_len': _A_in['seg_len'], 'B_x': _B_in['x'], 'B_w1': _B_in['w1'], 'B_b1': _B_in['b1'], 'B_w2': _B_in['w2'], 'B_b2': _B_in['b2'], 'c': _w((lambda *s: _rng.normal(s) * 0.05)(1, 1024)), 'w_mod': _w((lambda *s: _rng.normal(s) * 0.05)(1024, 6 * 1024) * 1024 ** (-0.5))}

def reference(A_x, A_mem0, A_Wq, A_Wk, A_Wv, A_Wo, A_seg_len, B_x, B_w1, B_b1, B_w2, B_b2, c, w_mod):

    def _A_ref(x, mem0, Wq, Wk, Wv, Wo, seg_len):
        B, S, Dm = x.shape
        H, Dh = (Wq.shape[1], Wq.shape[2])
        M = mem0.shape[1]
        scale = Dh ** (-0.5)
        n_seg = S // seg_len
        L = M + seg_len
        idx = jnp.arange(L)
        mask = (idx[:, None] < M) | (idx[:, None] >= idx[None, :])
        mem = mem0
        outs = []
        for s in range(n_seg):
            xs = x[:, s * seg_len:(s + 1) * seg_len, :].copy()
            h = jnp.concatenate([mem, xs], axis=1)
            q = jnp.einsum('btd,dhe->bhte', h, Wq)
            k = jnp.einsum('btd,dhe->bhte', h, Wk)
            v = jnp.einsum('btd,dhe->bhte', h, Wv)
            scores = jnp.einsum('bhqe,bhke->bhqk', q, k) * scale
            scores = jnp.where(mask[None, None], scores, -1000000000.0)
            p = _softmax(scores, axis=-1)
            o = jnp.einsum('bhqk,bhke->bhqe', p, v)
            o = jnp.einsum('bhte,hed->btd', o, Wo)
            mem = o[:, :M, :].copy()
            outs.append(o[:, M:, :])
        return jnp.concatenate(outs, axis=1)

    def _B_ref(x, w1, b1, w2, b2):
        h = jnp.einsum('bsd,df->bsf', x, w1) + b1
        h = _gelu(h)
        return jnp.einsum('bsf,fd->bsd', h, w2) + b2
    x = A_x
    mod = (_silu(c) @ w_mod).reshape(c.shape[0], 6, 1, -1)
    sa, ca, ga, sb, cb, gb = (mod[:, 0].copy(), mod[:, 1].copy(), mod[:, 2].copy(), mod[:, 3].copy(), mod[:, 4].copy(), mod[:, 5].copy())
    h = _layernorm(x, axis=-1) * (1 + ca) + sa
    x = x + ga * _A_ref(h, A_mem0, A_Wq, A_Wk, A_Wv, A_Wo, A_seg_len)
    h = _layernorm(x, axis=-1) * (1 + cb) + sb
    x = x + gb * _B_ref(h, B_w1, B_b1, B_w2, B_b2)
    return x
```

```python
import functools

import jax
import jax.numpy as jnp
import jax.experimental.pallas as pl
import jax.experimental.pallas.tpu as pltpu

F32 = jnp.float32
BF16 = jnp.bfloat16
U32 = jnp.uint32

S = 2048
D = 1024
H = 32
DH = 128
M = 8
SEG = 32
NSEG = S // SEG
FF = 3584
NPAIR = H // 2
PITCH = 516
NSTAGE = 3
EPS = 1e-5
SCALE = DH ** (-0.5)


def _slab(mat, head):
    g, r = divmod(head, 16)
    hp, par = divmod(r, 2)
    return mat * H + 16 * g + 8 * par + hp


def _ln(xf):
    m = jnp.mean(xf, axis=-1, keepdims=True)
    xc = xf - m
    v = jnp.mean(xc * xc, axis=-1, keepdims=True)
    return xc * jax.lax.rsqrt(v + EPS)


def _dot(a, b):
    return jnp.dot(a, b, preferred_element_type=F32)


def _dot_nt(a, b):
    return jax.lax.dot_general(a, b, (((1,), (1,)), ((), ())), preferred_element_type=F32)


def _pack(xf):
    return pltpu.bitcast(xf.astype(BF16), U32)


def _unpack(u):
    return pltpu.bitcast(u, BF16)


def _kernel(x_hbm, mem0_hbm, wq_hbm, wk_hbm, wv_hbm, wo_hbm, w1_hbm, b1_hbm, w2_hbm, b2_hbm,
            c_hbm, wmod_hbm,
            out_hbm,
            x_v, out_v, stage, wqkv, wo_v, w1_v, w2_v, wmod_v,
            mem0_v, b1_v, b2_v, c_v,
            mod_v, bias1_v, h3_v, qkv3, code_v,
            lhs_v, obuf, o3a, att_v, x1_v, h2_v, g_v, hn_v,
            sem_small, sem_x, sem_stage, sem_w, sem_out):
    w_hbms = (wq_hbm, wk_hbm, wv_hbm)

    def small_copies():
        return [pltpu.make_async_copy(c_hbm, c_v, sem_small.at[0]),
                pltpu.make_async_copy(mem0_hbm, mem0_v, sem_small.at[1]),
                pltpu.make_async_copy(b1_hbm, b1_v, sem_small.at[2]),
                pltpu.make_async_copy(b2_hbm, b2_v, sem_small.at[3])]

    def wmod_copy(part):
        lo, n = (0, 2 * D) if part == 0 else (2 * D, 4 * D)
        return pltpu.make_async_copy(wmod_hbm.at[:, pl.ds(lo, n)], wmod_v.at[:, pl.ds(lo, n)],
                                     sem_w.at[part])

    def x_copy(part):
        lo, n = (24, 8) if part == 0 else (0, 24)
        return pltpu.make_async_copy(x_hbm.at[:, pl.ds(lo, n), :], x_v.at[:, pl.ds(lo, n), :],
                                     sem_x.at[part])

    def stage_copy(grp, chunk):
        mat, half = divmod(grp, 2)
        d0 = chunk * 128
        if not isinstance(chunk, int):
            d0 = pl.multiple_of(d0, 128)
        slot = grp % NSTAGE
        return pltpu.make_async_copy(
            w_hbms[mat].at[pl.ds(d0, 128), pl.ds(16 * half, 16), :],
            stage.at[slot, pl.ds(d0, 128)],
            sem_stage.at[slot * 8 + chunk])

    def slab_copies(src, dst, n, sem):
        return [pltpu.make_async_copy(src.at[:, pl.ds(j * 128, 128)], dst.at[j], sem)
                for j in range(n)]

    def relayout(grp, chunk):
        slot = grp % NSTAGE
        d0 = pl.multiple_of(chunk * 128, 128)
        j0 = pl.multiple_of(chunk * 64, 64)
        dst = wqkv.at[pl.ds(j0, 3 * H * PITCH - 448), :]
        base = 16 * grp * PITCH
        for j in range(64):
            a = pltpu.bitcast(stage[slot, d0 + 2 * j], U32)
            b = pltpu.bitcast(stage[slot, d0 + 2 * j + 1], U32)
            lo = (a & jnp.uint32(0xFFFF)) | (b << 16)
            hi = (a >> 16) | (b & jnp.uint32(0xFFFF0000))
            dst[pl.ds(base + j, 8, stride=PITCH), :] = lo
            dst[pl.ds(base + 8 * PITCH + j, 8, stride=PITCH), :] = hi

    def wslab(mat, head):
        return _unpack(wqkv[pl.ds(_slab(mat, head) * PITCH, D // 2), :])

    def modrow(i):
        return mod_v[0:1, i * D:(i + 1) * D]

    for cp in small_copies():
        cp.start()
    wmod_copy(0).start()
    x_copy(0).start()
    for grp in range(NSTAGE):
        for ch in range(8):
            stage_copy(grp, ch).start()

    ri = jax.lax.broadcasted_iota(jnp.int32, (80, 128), 0)
    ci = jax.lax.broadcasted_iota(jnp.int32, (80, 128), 1)

    def head_of(i):
        return jnp.where(i < 64, i // 32, (i - 64) // 8)

    def pos_of(i):
        return jnp.where(i < 64, i % 32, 32 + (i - 64) % 8)

    same = head_of(ri) == head_of(ci)
    pr, pc = pos_of(ri), pos_of(ci)
    keep = jnp.logical_or(pr < M, pr >= pc)
    code_v[...] = jnp.where(same, jnp.where(keep, 0.0, -1e9), -jnp.inf).astype(F32)

    for cp in small_copies():
        cp.wait()
    cf = c_v[...].astype(F32)
    sc = (cf * jax.nn.sigmoid(cf)).astype(BF16)
    sc16 = jnp.broadcast_to(sc, (16, D))
    bias1_v[...] = jnp.broadcast_to(b1_v[...].astype(F32), (8, FF))

    wmod_copy(0).wait()
    mod_v[:, 0:2 * D] = _dot(sc16, wmod_v[:, 0:2 * D])[0:8]

    x_copy(0).wait()

    def ln1(xb):
        return _ln(xb.astype(F32)) * (1.0 + modrow(1)) + modrow(0)

    def h3_body(i, carry):
        s0 = pl.multiple_of(i * 8, 8)
        xb = x_v[pl.ds(s0, 8), 24:32, :].astype(F32).reshape(64, D)
        h = _ln(xb) * (1.0 + modrow(1)) + modrow(0)
        h3_v[pl.ds(pl.multiple_of(i * 32, 32), 32), :] = _pack(h)
        return carry

    jax.lax.fori_loop(0, 8, h3_body, 0)

    def g0_body(ch, carry):
        stage_copy(0, ch).wait()
        relayout(0, ch)
        return carry

    jax.lax.fori_loop(0, 8, g0_body, 0)

    for grp in range(6):
        mat, half = divmod(grp, 2)
        if grp + NSTAGE < 6:
            for ch in range(8):
                stage_copy(grp + NSTAGE, ch).start()
        if grp == 3:
            x_copy(1).start()
            for cp in slab_copies(wo_hbm, wo_v, 8, sem_w.at[2]):
                cp.start()
            wmod_copy(1).start()
        if grp == 4:
            for cp in slab_copies(w1_hbm, w1_v, FF // 128, sem_w.at[3]):
                cp.start()
            for cp in slab_copies(w2_hbm, w2_v, 8, sem_w.at[4]):
                cp.start()

        def pair_body(p, carry, grp=grp):
            if grp + 1 < 6:
                stage_copy(grp + 1, p).wait()
            r0 = (16 * grp + p) * PITCH
            w0 = _unpack(wqkv[pl.ds(r0, D // 2), :])
            w1 = _unpack(wqkv[pl.ds(r0 + 8 * PITCH, D // 2), :])
            w = jnp.concatenate([w0, w1], axis=1)
            for mc in range(4):
                lhs = _unpack(h3_v[mc * 64:(mc + 1) * 64, :])
                y = _dot(lhs, w).reshape(16, 8, 256)
                y = jnp.concatenate([y[:, :, :128], y[:, :, 128:]], axis=1)
                qkv3[grp * 8 + p, mc * 16:(mc + 1) * 16] = _pack(y)
            if grp + 1 < 6:
                relayout(grp + 1, p)
            return carry

        jax.lax.fori_loop(0, 8, pair_body, 0)

    x_copy(1).wait()
    wmod_copy(1).wait()
    mod_v[:, 2 * D:] = _dot(sc16, wmod_v[:, 2 * D:])[0:8]
    for cp in slab_copies(wo_hbm, wo_v, 8, sem_w.at[2]):
        cp.wait()
    for cp in slab_copies(w1_hbm, w1_v, FF // 128, sem_w.at[3]):
        cp.wait()
    for cp in slab_copies(w2_hbm, w2_v, 8, sem_w.at[4]):
        cp.wait()

    lhs_v[...] = _pack(jnp.concatenate([mem0_v[...].astype(F32), ln1(x_v[0, 0:24, :])], axis=0))

    zpad = jnp.zeros((48, DH), BF16)

    def qkv_pair(g, seg):
        lhs = _unpack(lhs_v[...])
        res = []
        for mat in range(3):
            w = jnp.concatenate([wslab(mat, 2 * g), wslab(mat, 2 * g + 1)], axis=1)
            y = _dot(lhs, w).astype(BF16)
            gg, pp = divmod(g, 8)
            t3 = _unpack(qkv3[(2 * mat + gg) * 8 + pp, seg])
            parts = [y[:, :DH], y[:, DH:], t3]
            if mat > 0:
                parts.append(zpad)
            res.append(jnp.concatenate(parts, axis=0))
        return res

    def scores(q, k):
        s = _dot_nt(q, k) * SCALE
        code = code_v[...]
        s = jnp.where(code == 0.0, s, code)
        m = jnp.max(s, axis=-1, keepdims=True)
        e = jnp.exp(s - m)
        l = jnp.sum(e, axis=-1, keepdims=True)
        return e.astype(BF16), l

    def pv(g, e, l, v, second):
        o = _dot(e, v) * (1.0 / l)
        c0, c1 = 2 * g * DH, (2 * g + 1) * DH
        obuf[0:16, c0:c0 + DH] = _pack(o[0:32])
        obuf[0:16, c1:c1 + DH] = _pack(o[32:64])
        if not second:
            o3a[:, c0:c0 + DH] = o[64:72]
            o3a[:, c1:c1 + DH] = o[72:80]
        else:
            obuf[16:24, c0:c0 + DH] = _pack(jnp.concatenate([o3a[:, c0:c0 + DH], o[64:72]], axis=0))
            obuf[16:24, c1:c1 + DH] = _pack(jnp.concatenate([o3a[:, c1:c1 + DH], o[72:80]], axis=0))

    def step(seg, second, fillers):
        qkv = {}
        sm = {}
        fillers = list(fillers)
        for i in range(NPAIR + 2):
            if i < NPAIR:
                qkv[i] = qkv_pair(i, seg)
            elif fillers:
                fillers.pop(0)()
            if 0 <= i - 1 < NPAIR:
                q, k, _ = qkv[i - 1]
                sm[i - 1] = scores(q, k)
            if 0 <= i - 2 < NPAIR:
                e, l = sm.pop(i - 2)
                pv(i - 2, e, l, qkv.pop(i - 2)[2], second)
        if fillers:
            fillers.pop(0)()
        nrow = 24 if second else 16
        for j in range(8):
            y = _dot(_unpack(obuf[0:nrow, :]), wo_v[j])
            cs = slice(j * 128, (j + 1) * 128)
            lhs_v[:, cs] = _pack(jnp.concatenate([y[0:8], hn_v[:, cs]], axis=0))
            if not second:
                att_v[0:24, cs] = y[8:32]
            else:
                att_v[32:56, cs] = y[8:32]
                att_v[24:32, cs] = y[32:40]
                att_v[56:64, cs] = y[40:48]
        for f in fillers:
            f()

    def ffn_pre(tp):
        xb = x_v[pl.ds(2 * tp, 2)].astype(F32).reshape(64, D)
        x1 = xb + modrow(2) * att_v[...]
        x1_v[...] = x1
        h2_v[...] = _pack(_ln(x1) * (1.0 + modrow(4)) + modrow(3))

    def ffn1(lo, hi):
        def run():
            for j in range(lo, hi):
                cs = slice(j * 128, (j + 1) * 128)
                y = _dot(_unpack(h2_v[...]), w1_v[j]) + bias1_v[0:1, cs]
                g_v[:, cs] = _pack(jax.nn.gelu(y, approximate=True))
        return run

    def ffn2(tp, lo, hi):
        def run():
            for j in range(lo, hi):
                cs = slice(j * 128, (j + 1) * 128)
                y = _dot(_unpack(g_v[...]), w2_v[j]) + b2_v[:, cs].astype(F32)
                o = x1_v[:, cs] + mod_v[0:1, 5 * D + j * 128:5 * D + (j + 1) * 128] * y
                out_v[tp, :, cs] = o.astype(BF16)
        return run

    def out_copy(tp):
        return pltpu.make_async_copy(out_v.at[tp], out_hbm.at[tp], sem_out.at[0])

    def double_step(t, with_ffn):
        if with_ffn:
            ffn_pre(t - 1)
        hn_v[...] = ln1(x_v[2 * t + 1, 0:24, :])
        fa = [ffn1(0, 7), ffn1(7, 14), ffn1(14, 24), ffn1(24, 28)] if with_ffn else []
        step(2 * t, False, fa)
        nxt = jnp.minimum(2 * t + 2, NSEG - 1)
        hn_v[...] = ln1(x_v[nxt, 0:24, :])
        fb = [ffn2(t - 1, 0, 2), ffn2(t - 1, 2, 4), ffn2(t - 1, 4, 8)] if with_ffn else []
        step(2 * t + 1, True, fb)
        if with_ffn:
            out_copy(t - 1).start()

    double_step(0, False)

    def body(t, carry):
        double_step(t, True)
        return carry

    jax.lax.fori_loop(1, NSEG // 2, body, 0)

    last = NSEG // 2 - 1
    ffn_pre(last)
    ffn1(0, FF // 128)()
    ffn2(last, 0, 8)()
    out_copy(last).start()
    pltpu.make_async_copy(out_v, out_hbm, sem_out.at[0]).wait()


@functools.partial(jax.jit, static_argnames=("A_seg_len",))
def pallas_adaLN_cond__memory_aug_recurrent_mem_tr__dense_activation_gelu__prompt_kernel(
    A_x, A_mem0, A_Wq, A_Wk, A_Wv, A_Wo, A_seg_len, B_x, B_w1, B_b1, B_w2, B_b2, c, w_mod,
):
    assert A_x.shape == (1, S, D) and A_mem0.shape == (1, M, D) and A_seg_len == SEG
    assert A_Wq.shape == (D, H, DH) and B_w1.shape == (D, FF)
    any_spec = pl.BlockSpec(memory_space=pl.ANY)
    scratch = [
        pltpu.VMEM((NSEG, SEG, D), BF16),
        pltpu.VMEM((NSEG // 2, 2 * SEG, D), BF16),
        pltpu.VMEM((NSTAGE, D, 16, DH), BF16),
        pltpu.VMEM((3 * H * PITCH, DH), U32),
        pltpu.VMEM((8, H * DH, 128), BF16),
        pltpu.VMEM((FF // 128, D, 128), BF16),
        pltpu.VMEM((8, FF, 128), BF16),
        pltpu.VMEM((D, 6 * D), BF16),
        pltpu.VMEM((M, D), BF16),
        pltpu.VMEM((1, FF), BF16),
        pltpu.VMEM((1, D), BF16),
        pltpu.VMEM((1, D), BF16),
        pltpu.VMEM((8, 6 * D), F32),
        pltpu.VMEM((8, FF), F32),
        pltpu.VMEM((256, D), U32),
        pltpu.VMEM((48, NSEG, 8, DH), U32),
        pltpu.VMEM((80, 128), F32),
        pltpu.VMEM((16, D), U32),
        pltpu.VMEM((24, H * DH), U32),
        pltpu.VMEM((8, H * DH), F32),
        pltpu.VMEM((64, D), F32),
        pltpu.VMEM((64, D), F32),
        pltpu.VMEM((32, D), U32),
        pltpu.VMEM((32, FF), U32),
        pltpu.VMEM((24, D), F32),
        pltpu.SemaphoreType.DMA((4,)),
        pltpu.SemaphoreType.DMA((2,)),
        pltpu.SemaphoreType.DMA((NSTAGE * 8,)),
        pltpu.SemaphoreType.DMA((5,)),
        pltpu.SemaphoreType.DMA((1,)),
    ]
    out = pl.pallas_call(
        _kernel,
        out_shape=jax.ShapeDtypeStruct((NSEG // 2, 2 * SEG, D), BF16),
        in_specs=[any_spec] * 12,
        out_specs=any_spec,
        scratch_shapes=scratch,
        compiler_params=pltpu.CompilerParams(vmem_limit_bytes=120 * 1024 * 1024),
    )(
        A_x.reshape(NSEG, SEG, D), A_mem0.reshape(M, D), A_Wq, A_Wk, A_Wv,
        A_Wo.reshape(H * DH, D), B_w1, B_b1.reshape(1, FF), B_w2, B_b2.reshape(1, D),
        c, w_mod,
    )
    return out.reshape(1, S, D)
```

```python
import functools

import jax
import jax.numpy as jnp
import jax.experimental.pallas as pl
import jax.experimental.pallas.tpu as pltpu

F32 = jnp.float32
BF16 = jnp.bfloat16
U32 = jnp.uint32

S = 2048
D = 1024
H = 32
DH = 128
M = 8
SEG = 32
NSEG = S // SEG
FF = 3584
NPAIR = H // 2
PITCH = 516
NSTAGE = 3
STOP = 0
UEXTRA = 0
PVLAG = 3
FA = [(0, 5), (5, 10), (10, 15), (15, 24), (24, 28)]
FB = [(0, 2), (2, 4), (4, 6), (6, 8)]
NITER = NSEG // 2
EPS = 1e-5
SCALE = DH ** (-0.5)


def _pair_heads(gp):
    half, r = divmod(gp, 8)
    par, i = divmod(r, 4)
    h0 = 16 * half + 4 * i + par
    return h0, h0 + 2


def _ln(xf):
    m = jnp.mean(xf, axis=-1, keepdims=True)
    xc = xf - m
    v = jnp.mean(xc * xc, axis=-1, keepdims=True)
    return xc * jax.lax.rsqrt(v + EPS)


def _dot(a, b):
    return jnp.dot(a, b, preferred_element_type=F32)


def _dot_nt(a, b):
    return jax.lax.dot_general(a, b, (((1,), (1,)), ((), ())), preferred_element_type=F32)


def _pack(xf):
    return pltpu.bitcast(xf.astype(BF16), U32)


def _unpack(u):
    return pltpu.bitcast(u, BF16)


def _kernel(x_hbm, mem0_hbm, wq_hbm, wk_hbm, wv_hbm, wo_hbm, w1_hbm, b1_hbm, w2_hbm, b2_hbm,
            c_hbm, wmod_hbm,
            out_hbm,
            x_v, out_v, stage, wqkv, wo_v, w1_v, w2_v, wmod_v,
            mem0_v, b1_v, b2_v, c_v,
            mod_v, bias1_v, h3_v, qkv3, code_v,
            lhs_v, obuf, o3a, att_v, x1_v, h2_v, g_v, hn_v,
            sem_small, sem_x, sem_g0, sem_stage, sem_w, sem_out):
    w_hbms = (wq_hbm, wk_hbm, wv_hbm)

    def small_copies():
        return [pltpu.make_async_copy(c_hbm, c_v, sem_small.at[0]),
                pltpu.make_async_copy(mem0_hbm, mem0_v, sem_small.at[1]),
                pltpu.make_async_copy(b1_hbm, b1_v, sem_small.at[2]),
                pltpu.make_async_copy(b2_hbm, b2_v, sem_small.at[3])]

    def wmod_copy(part):
        lo, n = (0, 2 * D) if part == 0 else (2 * D, 4 * D)
        return pltpu.make_async_copy(wmod_hbm.at[:, pl.ds(lo, n)], wmod_v.at[:, pl.ds(lo, n)],
                                     sem_w.at[part])

    def x_copy(part):
        lo, n = (24, 8) if part == 0 else (0, 24)
        return pltpu.make_async_copy(x_hbm.at[:, pl.ds(lo, n), :], x_v.at[:, pl.ds(lo, n), :],
                                     sem_x.at[part])

    def stage_copy(grp, chunk, nchunk):
        mat, half = divmod(grp, 2)
        rows = D // nchunk
        d0 = chunk * rows
        if not isinstance(chunk, int):
            d0 = pl.multiple_of(d0, rows)
        sem = sem_g0.at[chunk] if grp == 0 else sem_stage.at[grp]
        return pltpu.make_async_copy(
            w_hbms[mat].at[pl.ds(d0, rows), pl.ds(16 * half, 16), :],
            stage.at[grp % NSTAGE, pl.ds(d0, rows)], sem)

    def slab_copies(src, dst, n, sem):
        return [pltpu.make_async_copy(src.at[:, pl.ds(j * 128, 128)], dst.at[j], sem)
                for j in range(n)]

    def relayout(src, dst, base, j0, j1, sh):
        for j in range(j0, j1):
            a = pltpu.bitcast(src[2 * j], U32)
            b = pltpu.bitcast(src[2 * j + 1], U32)
            if isinstance(sh, int):
                assert sh == 0
                y = (a & jnp.uint32(0xFFFF)) | (b << 16)
            else:
                y = ((a >> sh) & jnp.uint32(0xFFFF)) | ((b << (16 - sh)) & jnp.uint32(0xFFFF0000))
            dst[pl.ds(base + j, 8, stride=PITCH), :] = y

    def wpair(ref, slab0):
        return jnp.concatenate([_unpack(ref[pl.ds(slab0 * PITCH, D // 2), :]),
                                _unpack(ref[pl.ds((slab0 + 1) * PITCH, D // 2), :])], axis=1)

    def modrow(i):
        return mod_v[0:1, i * D:(i + 1) * D]

    def start_in_order(groups):
        def issue(i, carry):
            for k, grp in enumerate(groups):
                @pl.when(i == k)
                def _(grp=grp):
                    for cp in grp():
                        cp.start()
            return carry
        jax.lax.fori_loop(0, len(groups), issue, 0)

    start_in_order(
        [small_copies, lambda: [wmod_copy(0)], lambda: [x_copy(0)]]
        + [lambda ch=ch: [stage_copy(0, ch, 8)] for ch in range(8)]
        + ([lambda: [stage_copy(1, 0, 1)], lambda: [stage_copy(2, 0, 1)]] if STOP != 6 else []))

    ri = jax.lax.broadcasted_iota(jnp.int32, (80, 128), 0)
    ci = jax.lax.broadcasted_iota(jnp.int32, (80, 128), 1)

    def head_of(i):
        return jnp.where(i < 64, i // 32, (i - 64) // 8)

    def pos_of(i):
        return jnp.where(i < 64, i % 32, 32 + (i - 64) % 8)

    same = head_of(ri) == head_of(ci)
    pr, pc = pos_of(ri), pos_of(ci)
    keep = jnp.logical_or(pr < M, pr >= pc)
    code_v[...] = jnp.where(same, jnp.where(keep, 0.0, -1e9), -jnp.inf).astype(F32)

    for cp in small_copies():
        cp.wait()
    cf = c_v[...].astype(F32)
    sc = (cf * jax.nn.sigmoid(cf)).astype(BF16)
    sc16 = jnp.broadcast_to(sc, (16, D))
    bias1_v[...] = jnp.broadcast_to(b1_v[...].astype(F32), (8, FF))

    wmod_copy(0).wait()
    mod_v[:, 0:2 * D] = _dot(sc16, wmod_v[:, 0:2 * D])[0:8]

    x_copy(0).wait()

    def ln1(xb):
        return _ln(xb.astype(F32)) * (1.0 + modrow(1)) + modrow(0)

    def h3_body(i, carry):
        s0 = pl.multiple_of(i * 8, 8)
        xb = x_v[pl.ds(s0, 8), 24:32, :].astype(F32).reshape(64, D)
        h = _ln(xb) * (1.0 + modrow(1)) + modrow(0)
        h3_v[pl.ds(pl.multiple_of(i * 32, 32), 32), :] = _pack(h)
        return carry

    jax.lax.fori_loop(0, 8, h3_body, 0)

    def g0_body(ch, carry):
        stage_copy(0, ch, 8).wait()
        src = stage.at[0, pl.ds(pl.multiple_of(ch * 128, 128), 128)]
        dst = wqkv.at[pl.ds(pl.multiple_of(ch * 64, 64), 8 * PITCH - 448), :]
        relayout(src, dst, 0, 0, 64, 0)
        return carry

    jax.lax.fori_loop(0, 8, g0_body, 0)
    if STOP == 6:
        return
    if STOP == 1:
        stage_copy(1, 0, 1).wait()
        stage_copy(2, 0, 1).wait()
        return

    def x3_matmul(wref, slab0, idx, mc):
        lhs = _unpack(h3_v[mc * 64:(mc + 1) * 64, :])
        y = _dot(lhs, wpair(wref, slab0)).reshape(16, 8, 256)
        y = jnp.concatenate([y[:, :, :128], y[:, :, 128:]], axis=1)
        qkv3[idx, mc * 16:(mc + 1) * 16] = _pack(y)

    def unit_body(uu, carry):
        u = jnp.where(uu < 11, uu, 10) if UEXTRA else uu
        @pl.when(u == 1)
        def _():
            stage_copy(3, 0, 1).start()

        @pl.when(u == 2)
        def _():
            x_copy(1).start()
            for cp in slab_copies(wo_hbm, wo_v, 8, sem_w.at[2]):
                cp.start()

        @pl.when(u == 3)
        def _():
            stage_copy(4, 0, 1).start()

        @pl.when(u == 5)
        def _():
            stage_copy(5, 0, 1).start()

        @pl.when(u == 6)
        def _():
            wmod_copy(1).start()

        @pl.when(u == 7)
        def _():
            for cp in slab_copies(w1_hbm, w1_v, FF // 128, sem_w.at[3]):
                cp.start()

        @pl.when(u == 8)
        def _():
            for cp in slab_copies(w2_hbm, w2_v, 8, sem_w.at[4]):
                cp.start()

        gn = (u + 1) // 2
        src = stage.at[gn % NSTAGE]

        @pl.when(u % 2 == 1)
        def _():
            pltpu.make_async_copy(src, src, sem_stage.at[gn]).wait()

        sh = (((u + 1) % 2) * 16).astype(U32)
        view = wqkv.at[pl.ds(pl.multiple_of(u * (8 * PITCH), 8), 16 * PITCH), :]
        for p in range(4):
            for mc in range(4):
                x3_matmul(view, 2 * p, 4 * u + p, mc)
                relayout(src, view, 8 * PITCH, 32 * (4 * p + mc), 32 * (4 * p + mc + 1), sh)
        return carry

    jax.lax.fori_loop(0, 11 + UEXTRA, unit_body, 0)

    x_copy(1).wait()
    wmod_copy(1).wait()
    for cp in slab_copies(wo_hbm, wo_v, 8, sem_w.at[2]):
        cp.wait()

    if STOP == 2:
        for cp in slab_copies(w1_hbm, w1_v, FF // 128, sem_w.at[3]):
            cp.wait()
        for cp in slab_copies(w2_hbm, w2_v, 8, sem_w.at[4]):
            cp.wait()
        return
    for p in range(4):
        x3_matmul(wqkv, 88 + 2 * p, 44 + p, 0)

    def x3_rest(mc, p0, p1):
        def run():
            for p in range(p0, p1):
                x3_matmul(wqkv, 88 + 2 * p, 44 + p, mc)
        return run

    def mod_rest(i):
        def run():
            mod_v[:, i * D:(i + 1) * D] = _dot(sc16, wmod_v[:, i * D:(i + 1) * D])[0:8]
        return run

    lhs_v[...] = _pack(jnp.concatenate([mem0_v[...].astype(F32), ln1(x_v[0, 0:24, :])], axis=0))

    zpad = jnp.zeros((48, DH), BF16)

    def qkv_pair(g, seg):
        lhs = _unpack(lhs_v[...])
        res = []
        for mat in range(3):
            y = _dot(lhs, wpair(wqkv, mat * H + 2 * g)).astype(BF16)
            t3 = _unpack(qkv3[mat * NPAIR + g, seg])
            parts = [y[:, :DH], y[:, DH:], t3]
            if mat > 0:
                parts.append(zpad)
            res.append(jnp.concatenate(parts, axis=0))
        return res

    def scores(q, k):
        s = _dot_nt(q, k) * SCALE
        code = code_v[...]
        s = jnp.where(code == 0.0, s, code)
        m = jnp.max(s, axis=-1, keepdims=True)
        e = jnp.exp(s - m)
        l = jnp.sum(e, axis=-1, keepdims=True)
        r = pl.reciprocal(l, approx=True)
        r = r * (2.0 - l * r)
        return (e * r).astype(BF16)

    def pv(g, p, v, second):
        o = _dot(p, v)
        c0, c1 = (h * DH for h in _pair_heads(g))
        obuf[0:16, c0:c0 + DH] = _pack(o[0:32])
        obuf[0:16, c1:c1 + DH] = _pack(o[32:64])
        if not second:
            o3a[:, c0:c0 + DH] = o[64:72]
            o3a[:, c1:c1 + DH] = o[72:80]
        else:
            obuf[16:24, c0:c0 + DH] = _pack(jnp.concatenate([o3a[:, c0:c0 + DH], o[64:72]], axis=0))
            obuf[16:24, c1:c1 + DH] = _pack(jnp.concatenate([o3a[:, c1:c1 + DH], o[72:80]], axis=0))

    def step(seg, second, fillers):
        qkv = {}
        sm = {}
        fillers = list(fillers)
        for i in range(NPAIR + PVLAG):
            if i < NPAIR:
                qkv[i] = qkv_pair(i, seg)
            elif fillers:
                fillers.pop(0)()
            if 0 <= i - 1 < NPAIR:
                q, k, _ = qkv[i - 1]
                sm[i - 1] = scores(q, k)
            if 0 <= i - PVLAG < NPAIR:
                pv(i - PVLAG, sm.pop(i - PVLAG), qkv.pop(i - PVLAG)[2], second)
        if fillers:
            fillers.pop(0)()
        nrow = 24 if second else 16
        for j in range(8):
            y = _dot(_unpack(obuf[0:nrow, :]), wo_v[j])
            cs = slice(j * 128, (j + 1) * 128)
            lhs_v[:, cs] = _pack(jnp.concatenate([y[0:8], hn_v[:, cs]], axis=0))
            if not second:
                att_v[0:24, cs] = y[8:32]
            else:
                att_v[32:56, cs] = y[8:32]
                att_v[24:32, cs] = y[32:40]
                att_v[56:64, cs] = y[40:48]
        for f in fillers:
            f()

    def ffn_pre(tp):
        xb = x_v[pl.ds(2 * tp, 2)].astype(F32).reshape(64, D)
        x1 = xb + modrow(2) * att_v[...]
        x1_v[...] = x1
        h2_v[...] = _pack(_ln(x1) * (1.0 + modrow(4)) + modrow(3))

    def ffn1(lo, hi):
        def run():
            for j in range(lo, hi):
                cs = slice(j * 128, (j + 1) * 128)
                y = _dot(_unpack(h2_v[...]), w1_v[j]) + bias1_v[0:1, cs]
                g_v[:, cs] = _pack(jax.nn.gelu(y, approximate=True))
        return run

    def ffn2(tp, lo, hi):
        def run():
            for j in range(lo, hi):
                cs = slice(j * 128, (j + 1) * 128)
                y = _dot(_unpack(g_v[...]), w2_v[j]) + b2_v[:, cs].astype(F32)
                o = x1_v[:, cs] + mod_v[0:1, 5 * D + j * 128:5 * D + (j + 1) * 128] * y
                out_v[tp, :, cs] = o.astype(BF16)
        return run

    def out_copy(tp):
        return pltpu.make_async_copy(out_v.at[tp], out_hbm.at[tp], sem_out.at[0])

    def seq(*fs):
        def run():
            for f in fs:
                f()
        return run

    def double_step(t, with_ffn):
        if with_ffn:
            ffn_pre(t - 1)
            fa = [ffn1(a, b) for a, b in FA]
            fb = [ffn2(t - 1, a, b) for a, b in FB]
        else:
            fa = [x3_rest(1, 0, 2), x3_rest(1, 2, 4), x3_rest(2, 0, 2), mod_rest(2), mod_rest(3)]
            fb = [x3_rest(2, 2, 4), x3_rest(3, 0, 2), x3_rest(3, 2, 4), mod_rest(4), mod_rest(5)]
        hn_v[...] = ln1(x_v[2 * t + 1, 0:24, :])
        step(2 * t, False, fa)
        nxt = jnp.minimum(2 * t + 2, NSEG - 1)
        hn_v[...] = ln1(x_v[nxt, 0:24, :])
        step(2 * t + 1, True, fb)
        if with_ffn:
            out_copy(t - 1).start()

    double_step(0, False)
    for cp in slab_copies(w1_hbm, w1_v, FF // 128, sem_w.at[3]):
        cp.wait()
    for cp in slab_copies(w2_hbm, w2_v, 8, sem_w.at[4]):
        cp.wait()

    if STOP == 3:
        return

    def body(t, carry):
        double_step(t, True)
        return carry

    jax.lax.fori_loop(1, NITER, body, 0)

    last = NITER - 1
    ffn_pre(last)
    ffn1(0, FF // 128)()
    ffn2(last, 0, 8)()
    out_copy(last).start()
    pltpu.make_async_copy(out_v.at[0:NITER], out_hbm.at[0:NITER], sem_out.at[0]).wait()


@functools.partial(jax.jit, static_argnames=("A_seg_len",))
def pallas_adaLN_cond__memory_aug_recurrent_mem_tr__dense_activation_gelu__prompt_kernel(
    A_x, A_mem0, A_Wq, A_Wk, A_Wv, A_Wo, A_seg_len, B_x, B_w1, B_b1, B_w2, B_b2, c, w_mod,
):
    assert A_x.shape == (1, S, D) and A_mem0.shape == (1, M, D) and A_seg_len == SEG
    assert A_Wq.shape == (D, H, DH) and B_w1.shape == (D, FF)
    any_spec = pl.BlockSpec(memory_space=pl.ANY)
    scratch = [
        pltpu.VMEM((NSEG, SEG, D), BF16),
        pltpu.VMEM((NSEG // 2, 2 * SEG, D), BF16),
        pltpu.VMEM((NSTAGE, D, 16, DH), BF16),
        pltpu.VMEM((3 * H * PITCH, DH), U32),
        pltpu.VMEM((8, H * DH, 128), BF16),
        pltpu.VMEM((FF // 128, D, 128), BF16),
        pltpu.VMEM((8, FF, 128), BF16),
        pltpu.VMEM((D, 6 * D), BF16),
        pltpu.VMEM((M, D), BF16),
        pltpu.VMEM((1, FF), BF16),
        pltpu.VMEM((1, D), BF16),
        pltpu.VMEM((1, D), BF16),
        pltpu.VMEM((8, 6 * D), F32),
        pltpu.VMEM((8, FF), F32),
        pltpu.VMEM((256, D), U32),
        pltpu.VMEM((48, NSEG, 8, DH), U32),
        pltpu.VMEM((80, 128), F32),
        pltpu.VMEM((16, D), U32),
        pltpu.VMEM((24, H * DH), U32),
        pltpu.VMEM((8, H * DH), F32),
        pltpu.VMEM((64, D), F32),
        pltpu.VMEM((64, D), F32),
        pltpu.VMEM((32, D), U32),
        pltpu.VMEM((32, FF), U32),
        pltpu.VMEM((24, D), F32),
        pltpu.SemaphoreType.DMA((4,)),
        pltpu.SemaphoreType.DMA((2,)),
        pltpu.SemaphoreType.DMA((8,)),
        pltpu.SemaphoreType.DMA((6,)),
        pltpu.SemaphoreType.DMA((5,)),
        pltpu.SemaphoreType.DMA((1,)),
    ]
    out = pl.pallas_call(
        _kernel,
        out_shape=jax.ShapeDtypeStruct((NSEG // 2, 2 * SEG, D), BF16),
        in_specs=[any_spec] * 12,
        out_specs=any_spec,
        scratch_shapes=scratch,
        compiler_params=pltpu.CompilerParams(vmem_limit_bytes=120 * 1024 * 1024),
    )(
        A_x.reshape(NSEG, SEG, D), A_mem0.reshape(M, D), A_Wq, A_Wk, A_Wv,
        A_Wo.reshape(H * DH, D), B_w1, B_b1.reshape(1, FF), B_w2, B_b2.reshape(1, D),
        c, w_mod,
    )
    return out.reshape(1, S, D)
```

```python
import functools

import jax
import jax.numpy as jnp
import jax.experimental.pallas as pl
import jax.experimental.pallas.tpu as pltpu

F32 = jnp.float32
BF16 = jnp.bfloat16
U32 = jnp.uint32

S = 2048
D = 1024
H = 32
DH = 128
M = 8
SEG = 32
NSEG = S // SEG
FF = 3584
NPAIR = H // 2
PITCH = 516
NSTAGE = 3
STOP = 0
PVLAG = 3
NS = 16
FA = {16: (0, 5), 17: (5, 10), 18: (10, 15), 19: (15, 24), 20: (24, 28)}
FB = {16: (0, 2), 17: (2, 4), 18: (4, 6), 19: (6, 8)}
PERSLAB = False
SCR = True
NITER = NSEG // 2
EPS = 1e-5
SCALE = DH ** (-0.5)


def _pair_heads(gp):
    half, r = divmod(gp, 8)
    par, i = divmod(r, 4)
    h0 = 16 * half + 4 * i + par
    return h0, h0 + 2


def _ln(xf):
    m = jnp.mean(xf, axis=-1, keepdims=True)
    xc = xf - m
    v = jnp.mean(xc * xc, axis=-1, keepdims=True)
    return xc * jax.lax.rsqrt(v + EPS)


def _dot(a, b):
    return jnp.dot(a, b, preferred_element_type=F32)


def _dot_nt(a, b):
    return jax.lax.dot_general(a, b, (((1,), (1,)), ((), ())), preferred_element_type=F32)


def _pack(xf):
    return pltpu.bitcast(xf.astype(BF16), U32)


def _unpack(u):
    return pltpu.bitcast(u, BF16)


def _kernel(x_hbm, mem0_hbm, wq_hbm, wk_hbm, wv_hbm, wo_hbm, w1_hbm, b1_hbm, w2_hbm, b2_hbm,
            c_hbm, wmod_hbm,
            out_hbm,
            x_v, out_v, stage, wqkv, wo_v, w1_v, w2_v, wmod_v,
            mem0_v, b1_v, b2_v, c_v,
            mod_v, bias1_v, h3_v, qkv3, code_v,
            lhs_v, qkv_s, p_s, obuf, o3a, att_v, x1_v, h2_v, g_v, hn_v,
            sem_small, sem_x, sem_g0, sem_stage, sem_w, sem_out):
    w_hbms = (wq_hbm, wk_hbm, wv_hbm)

    def small_copies():
        return [pltpu.make_async_copy(c_hbm, c_v, sem_small.at[0]),
                pltpu.make_async_copy(mem0_hbm, mem0_v, sem_small.at[1]),
                pltpu.make_async_copy(b1_hbm, b1_v, sem_small.at[2]),
                pltpu.make_async_copy(b2_hbm, b2_v, sem_small.at[3])]

    def wmod_copy(part):
        lo, n = (0, 2 * D) if part == 0 else (2 * D, 4 * D)
        return pltpu.make_async_copy(wmod_hbm.at[:, pl.ds(lo, n)], wmod_v.at[:, pl.ds(lo, n)],
                                     sem_w.at[part])

    def x_copy(part):
        lo, n = (24, 8) if part == 0 else (0, 24)
        return pltpu.make_async_copy(x_hbm.at[:, pl.ds(lo, n), :], x_v.at[:, pl.ds(lo, n), :],
                                     sem_x.at[part])

    def stage_copy(grp, chunk, nchunk):
        mat, half = divmod(grp, 2)
        rows = D // nchunk
        d0 = chunk * rows
        if not isinstance(chunk, int):
            d0 = pl.multiple_of(d0, rows)
        sem = sem_g0.at[chunk] if grp == 0 else sem_stage.at[grp]
        return pltpu.make_async_copy(
            w_hbms[mat].at[pl.ds(d0, rows), pl.ds(16 * half, 16), :],
            stage.at[grp % NSTAGE, pl.ds(d0, rows)], sem)

    def slab_copies(src, dst, n, sem):
        return [pltpu.make_async_copy(src.at[:, pl.ds(j * 128, 128)], dst.at[j], sem)
                for j in range(n)]

    def relayout(src, dst, base, j0, j1, sh):
        for j in range(j0, j1):
            a = pltpu.bitcast(src[2 * j], U32)
            b = pltpu.bitcast(src[2 * j + 1], U32)
            if isinstance(sh, int):
                assert sh == 0
                y = (a & jnp.uint32(0xFFFF)) | (b << 16)
            else:
                y = ((a >> sh) & jnp.uint32(0xFFFF)) | ((b << (16 - sh)) & jnp.uint32(0xFFFF0000))
            dst[pl.ds(base + j, 8, stride=PITCH), :] = y

    def wpair(ref, slab0):
        return jnp.concatenate([_unpack(ref[pl.ds(slab0 * PITCH, D // 2), :]),
                                _unpack(ref[pl.ds((slab0 + 1) * PITCH, D // 2), :])], axis=1)

    def modrow(i):
        return mod_v[0:1, i * D:(i + 1) * D]

    def start_in_order(groups):
        def issue(i, carry):
            for k, grp in enumerate(groups):
                @pl.when(i == k)
                def _(grp=grp):
                    for cp in grp():
                        cp.start()
            return carry
        jax.lax.fori_loop(0, len(groups), issue, 0)

    start_in_order(
        [small_copies, lambda: [wmod_copy(0)], lambda: [x_copy(0)]]
        + [lambda ch=ch: [stage_copy(0, ch, 8)] for ch in range(8)]
        + ([lambda: [stage_copy(1, 0, 1)], lambda: [stage_copy(2, 0, 1)]] if STOP != 6 else []))

    ri = jax.lax.broadcasted_iota(jnp.int32, (80, 128), 0)
    ci = jax.lax.broadcasted_iota(jnp.int32, (80, 128), 1)

    def head_of(i):
        return jnp.where(i < 64, i // 32, (i - 64) // 8)

    def pos_of(i):
        return jnp.where(i < 64, i % 32, 32 + (i - 64) % 8)

    same = head_of(ri) == head_of(ci)
    pr, pc = pos_of(ri), pos_of(ci)
    keep = jnp.logical_or(pr < M, pr >= pc)
    code_v[...] = jnp.where(same, jnp.where(keep, 0.0, -1e9), -jnp.inf).astype(F32)

    for cp in small_copies():
        cp.wait()
    cf = c_v[...].astype(F32)
    sc = (cf * jax.nn.sigmoid(cf)).astype(BF16)
    sc16 = jnp.broadcast_to(sc, (16, D))
    bias1_v[...] = jnp.broadcast_to(b1_v[...].astype(F32), (8, FF))

    wmod_copy(0).wait()
    mod_v[:, 0:2 * D] = _dot(sc16, wmod_v[:, 0:2 * D])[0:8]

    x_copy(0).wait()

    def ln1(xb):
        return _ln(xb.astype(F32)) * (1.0 + modrow(1)) + modrow(0)

    def h3_body(i, carry):
        s0 = pl.multiple_of(i * 8, 8)
        xb = x_v[pl.ds(s0, 8), 24:32, :].astype(F32).reshape(64, D)
        h = _ln(xb) * (1.0 + modrow(1)) + modrow(0)
        h3_v[pl.ds(pl.multiple_of(i * 32, 32), 32), :] = _pack(h)
        return carry

    jax.lax.fori_loop(0, 8, h3_body, 0)

    def g0_body(ch, carry):
        stage_copy(0, ch, 8).wait()
        src = stage.at[0, pl.ds(pl.multiple_of(ch * 128, 128), 128)]
        dst = wqkv.at[pl.ds(pl.multiple_of(ch * 64, 64), 8 * PITCH - 448), :]
        relayout(src, dst, 0, 0, 64, 0)
        return carry

    jax.lax.fori_loop(0, 8, g0_body, 0)
    if STOP == 6:
        return
    if STOP == 1:
        stage_copy(1, 0, 1).wait()
        stage_copy(2, 0, 1).wait()
        return

    def x3_matmul(wref, slab0, u, p, mc):
        lhs = _unpack(h3_v[mc * 64:(mc + 1) * 64, :])
        y = _dot(lhs, wpair(wref, slab0)).reshape(16, 8, 256)
        y = jnp.concatenate([y[:, :, :128], y[:, :, 128:]], axis=1).reshape(256, DH)
        qkv3[u, mc * 128:(mc + 1) * 128, p * DH:(p + 1) * DH] = _pack(y)

    def unit_body(u, carry):
        @pl.when(u == 1)
        def _():
            stage_copy(3, 0, 1).start()

        @pl.when(u == 2)
        def _():
            x_copy(1).start()
            for cp in slab_copies(wo_hbm, wo_v, 8, sem_w.at[2]):
                cp.start()

        @pl.when(u == 3)
        def _():
            stage_copy(4, 0, 1).start()

        @pl.when(u == 5)
        def _():
            stage_copy(5, 0, 1).start()

        @pl.when(u == 6)
        def _():
            wmod_copy(1).start()

        @pl.when(u == 7)
        def _():
            for cp in slab_copies(w1_hbm, w1_v, FF // 128, sem_w.at[3]):
                cp.start()

        @pl.when(u == 8)
        def _():
            for cp in slab_copies(w2_hbm, w2_v, 8, sem_w.at[4]):
                cp.start()

        gn = (u + 1) // 2
        src = stage.at[gn % NSTAGE]

        @pl.when(jnp.logical_and(u % 2 == 1, u < 11))
        def _():
            pltpu.make_async_copy(src, src, sem_stage.at[gn]).wait()

        sh = (((u + 1) % 2) * 16).astype(U32)
        view = wqkv.at[pl.ds(pl.multiple_of(u * (8 * PITCH), 8), 16 * PITCH), :]
        for p in range(4):
            for mc in range(4):
                x3_matmul(view, 2 * p, u, p, mc)
                relayout(src, view, 8 * PITCH, 32 * (4 * p + mc), 32 * (4 * p + mc + 1), sh)
        return carry

    jax.lax.fori_loop(0, 12, unit_body, 0)

    x_copy(1).wait()
    wmod_copy(1).wait()
    for cp in slab_copies(wo_hbm, wo_v, 8, sem_w.at[2]):
        cp.wait()

    if STOP == 2:
        for cp in slab_copies(w1_hbm, w1_v, FF // 128, sem_w.at[3]):
            cp.wait()
        for cp in slab_copies(w2_hbm, w2_v, 8, sem_w.at[4]):
            cp.wait()
        return

    def mod_rest(i):
        def run():
            cs = slice(2 * D + i * 512, 2 * D + (i + 1) * 512)
            mod_v[:, cs] = _dot(sc16, wmod_v[:, cs])[0:8]
        return run

    lhs_v[...] = _pack(jnp.concatenate([mem0_v[...].astype(F32), ln1(x_v[0, 0:24, :])], axis=0))

    zpad = jnp.zeros((24, DH), U32)

    def qkv_pair(g, seg):
        res = []
        if not PERSLAB:
            lhs = _unpack(lhs_v[...])
        for mat in range(3):
            sl = mat * H + 2 * g
            if PERSLAB:
                ys = []
                for i in range(2):
                    w = _unpack(wqkv[pl.ds((sl + i) * PITCH, D // 2), :])
                    y = _pack(_dot(_unpack(lhs_v[...]), w))
                    if SCR:
                        qkv_s[16 * i:16 * (i + 1), pl.ds(((g % NS) * 3 + mat) * DH, DH)] = y
                    ys.append(y)
            else:
                y = _dot(lhs, wpair(wqkv, sl))
                ys = [_pack(y[:, :DH]), _pack(y[:, DH:])]
                if SCR:
                    for i in range(2):
                        qkv_s[16 * i:16 * (i + 1), pl.ds(((g % NS) * 3 + mat) * DH, DH)] = ys[i]

            def get(mat=mat, ys=ys):
                parts = [qkv_s[:, pl.ds(((g % NS) * 3 + mat) * DH, DH)]] if SCR else list(ys)
                u3, p3 = divmod(mat * NPAIR + g, 4)
                parts.append(qkv3[u3, pl.ds(pl.multiple_of(seg * 8, 8), 8), p3 * DH:(p3 + 1) * DH])
                if mat > 0:
                    parts.append(zpad)
                return _unpack(jnp.concatenate(parts, axis=0))
            res.append(get)
        return res

    def scores(q, k):
        s = _dot_nt(q, k) * SCALE
        code = code_v[...]
        s = jnp.where(code == 0.0, s, code)
        m = jnp.max(s, axis=-1, keepdims=True)
        e = jnp.exp(s - m)
        l = jnp.sum(e, axis=-1, keepdims=True)
        r = pl.reciprocal(l, approx=True)
        r = r * (2.0 - l * r)
        return (e * r).astype(BF16)

    def pv(g, p, v, second):
        o = _dot(p, v)
        c0, c1 = (h * DH for h in _pair_heads(g))
        obuf[0:16, c0:c0 + DH] = _pack(o[0:32])
        obuf[0:16, c1:c1 + DH] = _pack(o[32:64])
        if not second:
            o3a[:, c0:c0 + DH] = o[64:72]
            o3a[:, c1:c1 + DH] = o[72:80]
        else:
            obuf[16:24, c0:c0 + DH] = _pack(jnp.concatenate([o3a[:, c0:c0 + DH], o[64:72]], axis=0))
            obuf[16:24, c1:c1 + DH] = _pack(jnp.concatenate([o3a[:, c1:c1 + DH], o[72:80]], axis=0))

    def step(seg, second, fillers):
        qkv = {}
        sm = {}
        for i in range(NPAIR + PVLAG + 1):
            if i < NPAIR:
                qkv[i] = qkv_pair(i, seg)
            if i in fillers:
                fillers[i]()
            if 0 <= i - 1 < NPAIR:
                q, k, _ = qkv[i - 1]
                p = scores(q(), k())
                if SCR:
                    p_s[:, pl.ds(((i - 1) % NS) * DH, DH)] = pltpu.bitcast(p, U32)
                sm[i - 1] = p
            if 0 <= i - PVLAG < NPAIR:
                g = i - PVLAG
                p = _unpack(p_s[:, pl.ds((g % NS) * DH, DH)]) if SCR else sm[g]
                pv(g, p, qkv.pop(g)[2](), second)
        nrow = 24 if second else 16
        for j in range(8):
            y = _dot(_unpack(obuf[0:nrow, :]), wo_v[j])
            cs = slice(j * 128, (j + 1) * 128)
            lhs_v[:, cs] = _pack(jnp.concatenate([y[0:8], hn_v[:, cs]], axis=0))
            if not second:
                att_v[0:24, cs] = y[8:32]
            else:
                att_v[32:56, cs] = y[8:32]
                att_v[24:32, cs] = y[32:40]
                att_v[56:64, cs] = y[40:48]
        if NPAIR + PVLAG + 1 in fillers:
            fillers[NPAIR + PVLAG + 1]()

    def ffn_pre(tp):
        xb = x_v[pl.ds(2 * tp, 2)].astype(F32).reshape(64, D)
        x1 = xb + modrow(2) * att_v[...]
        x1_v[...] = x1
        h2_v[...] = _pack(_ln(x1) * (1.0 + modrow(4)) + modrow(3))

    def ffn1(lo, hi):
        def run():
            for j in range(lo, hi):
                cs = slice(j * 128, (j + 1) * 128)
                y = _dot(_unpack(h2_v[...]), w1_v[j]) + bias1_v[0:1, cs]
                g_v[:, cs] = _pack(jax.nn.gelu(y, approximate=True))
        return run

    def ffn2(tp, lo, hi):
        def run():
            for j in range(lo, hi):
                cs = slice(j * 128, (j + 1) * 128)
                y = _dot(_unpack(g_v[...]), w2_v[j]) + b2_v[:, cs].astype(F32)
                o = x1_v[:, cs] + mod_v[0:1, 5 * D + j * 128:5 * D + (j + 1) * 128] * y
                out_v[tp, :, cs] = o.astype(BF16)
        return run

    def out_copy(tp):
        return pltpu.make_async_copy(out_v.at[tp], out_hbm.at[tp], sem_out.at[0])

    def seq(*fs):
        def run():
            for f in fs:
                f()
        return run

    def double_step(t, with_ffn):
        if with_ffn:
            ffn_pre(t - 1)
            fa = {k: ffn1(a, b) for k, (a, b) in FA.items()}
            fb = {k: ffn2(t - 1, a, b) for k, (a, b) in FB.items()}
        else:
            fa = {NPAIR + k: mod_rest(k) for k in range(4)}
            fb = {NPAIR + k: mod_rest(4 + k) for k in range(4)}
        hn_v[...] = ln1(x_v[2 * t + 1, 0:24, :])
        step(2 * t, False, fa)
        nxt = jnp.minimum(2 * t + 2, NSEG - 1)
        hn_v[...] = ln1(x_v[nxt, 0:24, :])
        step(2 * t + 1, True, fb)
        if with_ffn:
            out_copy(t - 1).start()

    double_step(0, False)
    for cp in slab_copies(w1_hbm, w1_v, FF // 128, sem_w.at[3]):
        cp.wait()
    for cp in slab_copies(w2_hbm, w2_v, 8, sem_w.at[4]):
        cp.wait()

    if STOP == 3:
        return

    def body(t, carry):
        double_step(t, True)
        return carry

    jax.lax.fori_loop(1, NITER, body, 0)

    last = NITER - 1
    ffn_pre(last)
    ffn1(0, FF // 128)()
    ffn2(last, 0, 8)()
    out_copy(last).start()
    pltpu.make_async_copy(out_v.at[0:NITER], out_hbm.at[0:NITER], sem_out.at[0]).wait()


@functools.partial(jax.jit, static_argnames=("A_seg_len",))
def pallas_adaLN_cond__memory_aug_recurrent_mem_tr__dense_activation_gelu__prompt_kernel(
    A_x, A_mem0, A_Wq, A_Wk, A_Wv, A_Wo, A_seg_len, B_x, B_w1, B_b1, B_w2, B_b2, c, w_mod,
):
    assert A_x.shape == (1, S, D) and A_mem0.shape == (1, M, D) and A_seg_len == SEG
    assert A_Wq.shape == (D, H, DH) and B_w1.shape == (D, FF)
    any_spec = pl.BlockSpec(memory_space=pl.ANY)
    scratch = [
        pltpu.VMEM((NSEG, SEG, D), BF16),
        pltpu.VMEM((NSEG // 2, 2 * SEG, D), BF16),
        pltpu.VMEM((NSTAGE, D, 16, DH), BF16),
        pltpu.VMEM(((3 * H + 8) * PITCH, DH), U32),
        pltpu.VMEM((8, H * DH, 128), BF16),
        pltpu.VMEM((FF // 128, D, 128), BF16),
        pltpu.VMEM((8, FF, 128), BF16),
        pltpu.VMEM((D, 6 * D), BF16),
        pltpu.VMEM((M, D), BF16),
        pltpu.VMEM((1, FF), BF16),
        pltpu.VMEM((1, D), BF16),
        pltpu.VMEM((1, D), BF16),
        pltpu.VMEM((8, 6 * D), F32),
        pltpu.VMEM((8, FF), F32),
        pltpu.VMEM((256, D), U32),
        pltpu.VMEM((12, NSEG * 8, 4 * DH), U32),
        pltpu.VMEM((80, 128), F32),
        pltpu.VMEM((16, D), U32),
        pltpu.VMEM((32, NS * 3 * DH), U32),
        pltpu.VMEM((40, NS * DH), U32),
        pltpu.VMEM((24, H * DH), U32),
        pltpu.VMEM((8, H * DH), F32),
        pltpu.VMEM((64, D), F32),
        pltpu.VMEM((64, D), F32),
        pltpu.VMEM((32, D), U32),
        pltpu.VMEM((32, FF), U32),
        pltpu.VMEM((24, D), F32),
        pltpu.SemaphoreType.DMA((4,)),
        pltpu.SemaphoreType.DMA((2,)),
        pltpu.SemaphoreType.DMA((8,)),
        pltpu.SemaphoreType.DMA((6,)),
        pltpu.SemaphoreType.DMA((5,)),
        pltpu.SemaphoreType.DMA((1,)),
    ]
    out = pl.pallas_call(
        _kernel,
        out_shape=jax.ShapeDtypeStruct((NSEG // 2, 2 * SEG, D), BF16),
        in_specs=[any_spec] * 12,
        out_specs=any_spec,
        scratch_shapes=scratch,
        compiler_params=pltpu.CompilerParams(vmem_limit_bytes=120 * 1024 * 1024),
    )(
        A_x.reshape(NSEG, SEG, D), A_mem0.reshape(M, D), A_Wq, A_Wk, A_Wv,
        A_Wo.reshape(H * DH, D), B_w1, B_b1.reshape(1, FF), B_w2, B_b2.reshape(1, D),
        c, w_mod,
    )
    return out.reshape(1, S, D)
```

```python
import functools

import jax
import jax.numpy as jnp
import jax.experimental.pallas as pl
import jax.experimental.pallas.tpu as pltpu

F32 = jnp.float32
BF16 = jnp.bfloat16
U32 = jnp.uint32

S = 2048
D = 1024
H = 32
DH = 128
M = 8
SEG = 32
NSEG = S // SEG
FF = 3584
NPAIR = H // 2
PITCH = 516
NSTAGE = 3
STOP = 0
PVLAG = 3
SLAG = 1
NS = 16
FA = {16: (0, 5), 17: (5, 10), 18: (10, 15), 19: (15, 24), 20: (24, 28)}
FB = {16: (0, 2), 17: (2, 4), 18: (4, 6), 19: (6, 8)}
PERSLAB = False
SCR = True
NITER = NSEG // 2
EPS = 1e-5
SCALE = DH ** (-0.5)


def _pair_heads(gp):
    half, r = divmod(gp, 8)
    par, i = divmod(r, 4)
    h0 = 16 * half + 4 * i + par
    return h0, h0 + 2


def _ln(xf):
    m = jnp.mean(xf, axis=-1, keepdims=True)
    xc = xf - m
    v = jnp.mean(xc * xc, axis=-1, keepdims=True)
    return xc * jax.lax.rsqrt(v + EPS)


def _dot(a, b):
    return jnp.dot(a, b, preferred_element_type=F32)


def _dot_nt(a, b):
    return jax.lax.dot_general(a, b, (((1,), (1,)), ((), ())), preferred_element_type=F32)


def _pack(xf):
    return pltpu.bitcast(xf.astype(BF16), U32)


def _unpack(u):
    return pltpu.bitcast(u, BF16)


def _kernel(x_hbm, mem0_hbm, wq_hbm, wk_hbm, wv_hbm, wo_hbm, w1_hbm, b1_hbm, w2_hbm, b2_hbm,
            c_hbm, wmod_hbm,
            out_hbm,
            x_v, out_v, stage, wqkv, wo_v, w1_v, w2_v, wmod_v,
            mem0_v, b1_v, b2_v, c_v,
            mod_v, bias1_v, h3_v, qkv3, code_v,
            lhs_v, qkv_s, p_s, obuf, o3a, att_v, x1_v, h2_v, g_v, hn_v,
            sem_small, sem_x, sem_g0, sem_stage, sem_w, sem_out):
    w_hbms = (wq_hbm, wk_hbm, wv_hbm)

    def small_copies():
        return [pltpu.make_async_copy(c_hbm, c_v, sem_small.at[0]),
                pltpu.make_async_copy(mem0_hbm, mem0_v, sem_small.at[1]),
                pltpu.make_async_copy(b1_hbm, b1_v, sem_small.at[2]),
                pltpu.make_async_copy(b2_hbm, b2_v, sem_small.at[3])]

    def wmod_copy(part):
        lo, n = (0, 2 * D) if part == 0 else (2 * D, 4 * D)
        return pltpu.make_async_copy(wmod_hbm.at[:, pl.ds(lo, n)], wmod_v.at[:, pl.ds(lo, n)],
                                     sem_w.at[part])

    def x_copy(part):
        lo, n = (24, 8) if part == 0 else (0, 24)
        return pltpu.make_async_copy(x_hbm.at[:, pl.ds(lo, n), :], x_v.at[:, pl.ds(lo, n), :],
                                     sem_x.at[part])

    def stage_copy(grp, chunk, nchunk):
        mat, half = divmod(grp, 2)
        rows = D // nchunk
        d0 = chunk * rows
        if not isinstance(chunk, int):
            d0 = pl.multiple_of(d0, rows)
        sem = sem_g0.at[chunk] if grp == 0 else sem_stage.at[grp]
        return pltpu.make_async_copy(
            w_hbms[mat].at[pl.ds(d0, rows), pl.ds(16 * half, 16), :],
            stage.at[grp % NSTAGE, pl.ds(d0, rows)], sem)

    def slab_copies(src, dst, n, sem):
        return [pltpu.make_async_copy(src.at[:, pl.ds(j * 128, 128)], dst.at[j], sem)
                for j in range(n)]

    def relayout(src, dst, base, j0, j1, sh):
        for j in range(j0, j1):
            a = pltpu.bitcast(src[2 * j], U32)
            b = pltpu.bitcast(src[2 * j + 1], U32)
            if isinstance(sh, int):
                assert sh == 0
                y = (a & jnp.uint32(0xFFFF)) | (b << 16)
            else:
                y = ((a >> sh) & jnp.uint32(0xFFFF)) | ((b << (16 - sh)) & jnp.uint32(0xFFFF0000))
            dst[pl.ds(base + j, 8, stride=PITCH), :] = y

    def wpair(ref, slab0):
        return jnp.concatenate([_unpack(ref[pl.ds(slab0 * PITCH, D // 2), :]),
                                _unpack(ref[pl.ds((slab0 + 1) * PITCH, D // 2), :])], axis=1)

    def modrow(i):
        return mod_v[0:1, i * D:(i + 1) * D]

    def start_in_order(groups):
        def issue(i, carry):
            for k, grp in enumerate(groups):
                @pl.when(i == k)
                def _(grp=grp):
                    for cp in grp():
                        cp.start()
            return carry
        jax.lax.fori_loop(0, len(groups), issue, 0)

    start_in_order(
        [small_copies, lambda: [wmod_copy(0)], lambda: [x_copy(0)]]
        + [lambda ch=ch: [stage_copy(0, ch, 8)] for ch in range(8)]
        + ([lambda: [stage_copy(1, 0, 1)], lambda: [stage_copy(2, 0, 1)]] if STOP != 6 else []))

    ri = jax.lax.broadcasted_iota(jnp.int32, (80, 128), 0)
    ci = jax.lax.broadcasted_iota(jnp.int32, (80, 128), 1)

    def head_of(i):
        return jnp.where(i < 64, i // 32, (i - 64) // 8)

    def pos_of(i):
        return jnp.where(i < 64, i % 32, 32 + (i - 64) % 8)

    same = head_of(ri) == head_of(ci)
    pr, pc = pos_of(ri), pos_of(ci)
    keep = jnp.logical_or(pr < M, pr >= pc)
    code_v[...] = jnp.where(same, jnp.where(keep, 0.0, -1e9), -jnp.inf).astype(F32)

    for cp in small_copies():
        cp.wait()
    cf = c_v[...].astype(F32)
    sc = (cf * jax.nn.sigmoid(cf)).astype(BF16)
    sc16 = jnp.broadcast_to(sc, (16, D))
    bias1_v[...] = jnp.broadcast_to(b1_v[...].astype(F32), (8, FF))

    wmod_copy(0).wait()
    mod_v[:, 0:2 * D] = _dot(sc16, wmod_v[:, 0:2 * D])[0:8]

    x_copy(0).wait()

    def ln1(xb):
        return _ln(xb.astype(F32)) * (1.0 + modrow(1)) + modrow(0)

    def h3_body(i, carry):
        s0 = pl.multiple_of(i * 8, 8)
        xb = x_v[pl.ds(s0, 8), 24:32, :].astype(F32).reshape(64, D)
        h = _ln(xb) * (1.0 + modrow(1)) + modrow(0)
        h3_v[pl.ds(pl.multiple_of(i * 32, 32), 32), :] = _pack(h)
        return carry

    jax.lax.fori_loop(0, 8, h3_body, 0)

    def g0_body(ch, carry):
        stage_copy(0, ch, 8).wait()
        src = stage.at[0, pl.ds(pl.multiple_of(ch * 128, 128), 128)]
        dst = wqkv.at[pl.ds(pl.multiple_of(ch * 64, 64), 8 * PITCH - 448), :]
        relayout(src, dst, 0, 0, 64, 0)
        return carry

    jax.lax.fori_loop(0, 8, g0_body, 0)
    if STOP == 6:
        return
    if STOP == 1:
        stage_copy(1, 0, 1).wait()
        stage_copy(2, 0, 1).wait()
        return

    def x3_matmul(wref, slab0, u, p, mc):
        lhs = _unpack(h3_v[mc * 64:(mc + 1) * 64, :])
        y = _dot(lhs, wpair(wref, slab0)).reshape(16, 8, 256)
        y = jnp.concatenate([y[:, :, :128], y[:, :, 128:]], axis=1).reshape(256, DH)
        qkv3[u, mc * 128:(mc + 1) * 128, p * DH:(p + 1) * DH] = _pack(y)

    def unit_body(u, carry):
        @pl.when(u == 1)
        def _():
            stage_copy(3, 0, 1).start()

        @pl.when(u == 2)
        def _():
            x_copy(1).start()
            for cp in slab_copies(wo_hbm, wo_v, 8, sem_w.at[2]):
                cp.start()

        @pl.when(u == 3)
        def _():
            stage_copy(4, 0, 1).start()

        @pl.when(u == 5)
        def _():
            stage_copy(5, 0, 1).start()

        @pl.when(u == 6)
        def _():
            wmod_copy(1).start()

        @pl.when(u == 7)
        def _():
            for cp in slab_copies(w1_hbm, w1_v, FF // 128, sem_w.at[3]):
                cp.start()

        @pl.when(u == 8)
        def _():
            for cp in slab_copies(w2_hbm, w2_v, 8, sem_w.at[4]):
                cp.start()

        gn = (u + 1) // 2
        src = stage.at[gn % NSTAGE]

        @pl.when(jnp.logical_and(u % 2 == 1, u < 11))
        def _():
            pltpu.make_async_copy(src, src, sem_stage.at[gn]).wait()

        sh = (((u + 1) % 2) * 16).astype(U32)
        view = wqkv.at[pl.ds(pl.multiple_of(u * (8 * PITCH), 8), 16 * PITCH), :]
        for p in range(4):
            for mc in range(4):
                x3_matmul(view, 2 * p, u, p, mc)
                relayout(src, view, 8 * PITCH, 32 * (4 * p + mc), 32 * (4 * p + mc + 1), sh)
        return carry

    jax.lax.fori_loop(0, 12, unit_body, 0)

    x_copy(1).wait()
    wmod_copy(1).wait()
    for cp in slab_copies(wo_hbm, wo_v, 8, sem_w.at[2]):
        cp.wait()

    if STOP == 2:
        for cp in slab_copies(w1_hbm, w1_v, FF // 128, sem_w.at[3]):
            cp.wait()
        for cp in slab_copies(w2_hbm, w2_v, 8, sem_w.at[4]):
            cp.wait()
        return

    def mod_rest(i):
        def run():
            cs = slice(2 * D + i * 512, 2 * D + (i + 1) * 512)
            mod_v[:, cs] = _dot(sc16, wmod_v[:, cs])[0:8]
        return run

    lhs_v[...] = _pack(jnp.concatenate([mem0_v[...].astype(F32), ln1(x_v[0, 0:24, :])], axis=0))

    zpad = jnp.zeros((24, DH), U32)

    def qkv_pair(g, seg):
        res = []
        if not PERSLAB:
            lhs = _unpack(lhs_v[...])
        for mat in range(3):
            sl = mat * H + 2 * g
            if PERSLAB:
                ys = []
                for i in range(2):
                    w = _unpack(wqkv[pl.ds((sl + i) * PITCH, D // 2), :])
                    y = _pack(_dot(_unpack(lhs_v[...]), w))
                    if SCR:
                        qkv_s[16 * i:16 * (i + 1), pl.ds(((g % NS) * 3 + mat) * DH, DH)] = y
                    ys.append(y)
            else:
                y = _dot(lhs, wpair(wqkv, sl))
                ys = [_pack(y[:, :DH]), _pack(y[:, DH:])]
                if SCR:
                    for i in range(2):
                        qkv_s[16 * i:16 * (i + 1), pl.ds(((g % NS) * 3 + mat) * DH, DH)] = ys[i]

            def get(mat=mat, ys=ys):
                parts = [qkv_s[:, pl.ds(((g % NS) * 3 + mat) * DH, DH)]] if SCR else list(ys)
                u3, p3 = divmod(mat * NPAIR + g, 4)
                parts.append(qkv3[u3, pl.ds(pl.multiple_of(seg * 8, 8), 8), p3 * DH:(p3 + 1) * DH])
                if mat > 0:
                    parts.append(zpad)
                return _unpack(jnp.concatenate(parts, axis=0))
            res.append(get)
        return res

    def scores(q, k):
        s = _dot_nt(q, k) * SCALE
        code = code_v[...]
        s = jnp.where(code == 0.0, s, code)
        m = jnp.max(s, axis=-1, keepdims=True)
        e = jnp.exp(s - m)
        l = jnp.sum(e, axis=-1, keepdims=True)
        r = pl.reciprocal(l, approx=True)
        r = r * (2.0 - l * r)
        return (e * r).astype(BF16)

    def pv(g, p, v, second):
        o = _dot(p, v)
        c0, c1 = (h * DH for h in _pair_heads(g))
        obuf[0:16, c0:c0 + DH] = _pack(o[0:32])
        obuf[0:16, c1:c1 + DH] = _pack(o[32:64])
        if not second:
            o3a[:, c0:c0 + DH] = o[64:72]
            o3a[:, c1:c1 + DH] = o[72:80]
        else:
            obuf[16:24, c0:c0 + DH] = _pack(jnp.concatenate([o3a[:, c0:c0 + DH], o[64:72]], axis=0))
            obuf[16:24, c1:c1 + DH] = _pack(jnp.concatenate([o3a[:, c1:c1 + DH], o[72:80]], axis=0))

    def step(seg, second, fillers):
        qkv = {}
        sm = {}
        for i in range(NPAIR + PVLAG + 1):
            if i < NPAIR:
                qkv[i] = qkv_pair(i, seg)
            if i in fillers:
                fillers[i]()
            if 0 <= i - SLAG < NPAIR:
                q, k, _ = qkv[i - SLAG]
                p = scores(q(), k())
                if SCR:
                    p_s[:, pl.ds(((i - SLAG) % NS) * DH, DH)] = pltpu.bitcast(p, U32)
                sm[i - SLAG] = p
            if 0 <= i - PVLAG < NPAIR:
                g = i - PVLAG
                p = _unpack(p_s[:, pl.ds((g % NS) * DH, DH)]) if SCR else sm[g]
                pv(g, p, qkv.pop(g)[2](), second)
        nrow = 24 if second else 16
        for j in range(8):
            y = _dot(_unpack(obuf[0:nrow, :]), wo_v[j])
            cs = slice(j * 128, (j + 1) * 128)
            lhs_v[:, cs] = _pack(jnp.concatenate([y[0:8], hn_v[:, cs]], axis=0))
            if not second:
                att_v[0:24, cs] = y[8:32]
            else:
                att_v[32:56, cs] = y[8:32]
                att_v[24:32, cs] = y[32:40]
                att_v[56:64, cs] = y[40:48]
        if NPAIR + PVLAG + 1 in fillers:
            fillers[NPAIR + PVLAG + 1]()

    def ffn_pre(tp):
        xb = x_v[pl.ds(2 * tp, 2)].astype(F32).reshape(64, D)
        x1 = xb + modrow(2) * att_v[...]
        x1_v[...] = x1
        h2_v[...] = _pack(_ln(x1) * (1.0 + modrow(4)) + modrow(3))

    def ffn1(lo, hi):
        def run():
            for j in range(lo, hi):
                cs = slice(j * 128, (j + 1) * 128)
                y = _dot(_unpack(h2_v[...]), w1_v[j]) + bias1_v[0:1, cs]
                g_v[:, cs] = _pack(jax.nn.gelu(y, approximate=True))
        return run

    def ffn2(tp, lo, hi):
        def run():
            for j in range(lo, hi):
                cs = slice(j * 128, (j + 1) * 128)
                y = _dot(_unpack(g_v[...]), w2_v[j]) + b2_v[:, cs].astype(F32)
                o = x1_v[:, cs] + mod_v[0:1, 5 * D + j * 128:5 * D + (j + 1) * 128] * y
                out_v[tp, :, cs] = o.astype(BF16)
        return run

    def out_copy(tp):
        return pltpu.make_async_copy(out_v.at[tp], out_hbm.at[tp], sem_out.at[0])

    def seq(*fs):
        def run():
            for f in fs:
                f()
        return run

    def double_step(t, with_ffn):
        if with_ffn:
            ffn_pre(t - 1)
            fa = {k: ffn1(a, b) for k, (a, b) in FA.items()}
            fb = {k: ffn2(t - 1, a, b) for k, (a, b) in FB.items()}
        else:
            fa = {NPAIR + k: mod_rest(k) for k in range(4)}
            fb = {NPAIR + k: mod_rest(4 + k) for k in range(4)}
        hn_v[...] = ln1(x_v[2 * t + 1, 0:24, :])
        step(2 * t, False, fa)
        nxt = jnp.minimum(2 * t + 2, NSEG - 1)
        hn_v[...] = ln1(x_v[nxt, 0:24, :])
        step(2 * t + 1, True, fb)
        if with_ffn:
            out_copy(t - 1).start()

    double_step(0, False)
    for cp in slab_copies(w1_hbm, w1_v, FF // 128, sem_w.at[3]):
        cp.wait()
    for cp in slab_copies(w2_hbm, w2_v, 8, sem_w.at[4]):
        cp.wait()

    if STOP == 3:
        return

    def body(t, carry):
        double_step(t, True)
        return carry

    jax.lax.fori_loop(1, NITER, body, 0)

    last = NITER - 1
    ffn_pre(last)
    ffn1(0, FF // 128)()
    ffn2(last, 0, 8)()
    out_copy(last).start()
    pltpu.make_async_copy(out_v.at[0:NITER], out_hbm.at[0:NITER], sem_out.at[0]).wait()


@functools.partial(jax.jit, static_argnames=("A_seg_len",))
def pallas_adaLN_cond__memory_aug_recurrent_mem_tr__dense_activation_gelu__prompt_kernel(
    A_x, A_mem0, A_Wq, A_Wk, A_Wv, A_Wo, A_seg_len, B_x, B_w1, B_b1, B_w2, B_b2, c, w_mod,
):
    assert A_x.shape == (1, S, D) and A_mem0.shape == (1, M, D) and A_seg_len == SEG
    assert A_Wq.shape == (D, H, DH) and B_w1.shape == (D, FF)
    any_spec = pl.BlockSpec(memory_space=pl.ANY)
    scratch = [
        pltpu.VMEM((NSEG, SEG, D), BF16),
        pltpu.VMEM((NSEG // 2, 2 * SEG, D), BF16),
        pltpu.VMEM((NSTAGE, D, 16, DH), BF16),
        pltpu.VMEM(((3 * H + 8) * PITCH, DH), U32),
        pltpu.VMEM((8, H * DH, 128), BF16),
        pltpu.VMEM((FF // 128, D, 128), BF16),
        pltpu.VMEM((8, FF, 128), BF16),
        pltpu.VMEM((D, 6 * D), BF16),
        pltpu.VMEM((M, D), BF16),
        pltpu.VMEM((1, FF), BF16),
        pltpu.VMEM((1, D), BF16),
        pltpu.VMEM((1, D), BF16),
        pltpu.VMEM((8, 6 * D), F32),
        pltpu.VMEM((8, FF), F32),
        pltpu.VMEM((256, D), U32),
        pltpu.VMEM((12, NSEG * 8, 4 * DH), U32),
        pltpu.VMEM((80, 128), F32),
        pltpu.VMEM((16, D), U32),
        pltpu.VMEM((32, NS * 3 * DH), U32),
        pltpu.VMEM((40, NS * DH), U32),
        pltpu.VMEM((24, H * DH), U32),
        pltpu.VMEM((8, H * DH), F32),
        pltpu.VMEM((64, D), F32),
        pltpu.VMEM((64, D), F32),
        pltpu.VMEM((32, D), U32),
        pltpu.VMEM((32, FF), U32),
        pltpu.VMEM((24, D), F32),
        pltpu.SemaphoreType.DMA((4,)),
        pltpu.SemaphoreType.DMA((2,)),
        pltpu.SemaphoreType.DMA((8,)),
        pltpu.SemaphoreType.DMA((6,)),
        pltpu.SemaphoreType.DMA((5,)),
        pltpu.SemaphoreType.DMA((1,)),
    ]
    out = pl.pallas_call(
        _kernel,
        out_shape=jax.ShapeDtypeStruct((NSEG // 2, 2 * SEG, D), BF16),
        in_specs=[any_spec] * 12,
        out_specs=any_spec,
        scratch_shapes=scratch,
        compiler_params=pltpu.CompilerParams(vmem_limit_bytes=120 * 1024 * 1024),
    )(
        A_x.reshape(NSEG, SEG, D), A_mem0.reshape(M, D), A_Wq, A_Wk, A_Wv,
        A_Wo.reshape(H * DH, D), B_w1, B_b1.reshape(1, FF), B_w2, B_b2.reshape(1, D),
        c, w_mod,
    )
    return out.reshape(1, S, D)
```

```python
import functools

import jax
import jax.numpy as jnp
import jax.experimental.pallas as pl
import jax.experimental.pallas.tpu as pltpu

F32 = jnp.float32
BF16 = jnp.bfloat16
U32 = jnp.uint32

S = 2048
D = 1024
H = 32
DH = 128
M = 8
SEG = 32
NSEG = S // SEG
FF = 3584
NPAIR = H // 2
PITCH = 516
NSTAGE = 3
STOP = 0
PVLAG = 3
SLAG = 1
NS = 16
FA = {16: (0, 5), 17: (5, 10), 18: (10, 15), 19: (15, 24), 20: (24, 28)}
FB = {16: (0, 2), 17: (2, 4), 18: (4, 6), 19: (6, 8)}
PERSLAB = False
SCR = True
NITER = NSEG // 2
EPS = 1e-5
SCALE = DH ** (-0.5)


def _pair_heads(gp):
    half, r = divmod(gp, 8)
    par, i = divmod(r, 4)
    h0 = 16 * half + 4 * i + par
    return h0, h0 + 2


def _ln(xf):
    m = jnp.mean(xf, axis=-1, keepdims=True)
    xc = xf - m
    v = jnp.mean(xc * xc, axis=-1, keepdims=True)
    return xc * jax.lax.rsqrt(v + EPS)


def _dot(a, b):
    return jnp.dot(a, b, preferred_element_type=F32)


def _dot_nt(a, b):
    return jax.lax.dot_general(a, b, (((1,), (1,)), ((), ())), preferred_element_type=F32)


def _pack(xf):
    return pltpu.bitcast(xf.astype(BF16), U32)


def _unpack(u):
    return pltpu.bitcast(u, BF16)


def _kernel(x_hbm, mem0_hbm, wq_hbm, wk_hbm, wv_hbm, wo_hbm, w1_hbm, b1_hbm, w2_hbm, b2_hbm,
            c_hbm, wmod_hbm,
            out_hbm,
            x_v, out_v, stage, wqkv, wo_v, w1_v, w2_v, wmod_v,
            mem0_v, b1_v, b2_v, c_v,
            mod_v, bias_v, h3_v, qkv3, code_v,
            lhs_v, qkv_s, p_s, obuf, o3a, att_v, x1_v, h2_v, g_v, hn_v,
            sem_small, sem_x, sem_g0, sem_stage, sem_w, sem_out):
    w_hbms = (wq_hbm, wk_hbm, wv_hbm)

    def small_copies():
        return [pltpu.make_async_copy(c_hbm, c_v, sem_small.at[0]),
                pltpu.make_async_copy(mem0_hbm, mem0_v, sem_small.at[1]),
                pltpu.make_async_copy(b1_hbm, b1_v, sem_small.at[2]),
                pltpu.make_async_copy(b2_hbm, b2_v, sem_small.at[3])]

    def wmod_copy(part):
        lo, n = (0, 2 * D) if part == 0 else (2 * D, 4 * D)
        return pltpu.make_async_copy(wmod_hbm.at[:, pl.ds(lo, n)], wmod_v.at[:, pl.ds(lo, n)],
                                     sem_w.at[part])

    def x_copy(part):
        lo, n = (24, 8) if part == 0 else (0, 24)
        return pltpu.make_async_copy(x_hbm.at[:, pl.ds(lo, n), :], x_v.at[:, pl.ds(lo, n), :],
                                     sem_x.at[part])

    def stage_copy(grp, chunk, nchunk):
        mat, half = divmod(grp, 2)
        rows = D // nchunk
        d0 = chunk * rows
        if not isinstance(chunk, int):
            d0 = pl.multiple_of(d0, rows)
        sem = sem_g0.at[chunk] if grp == 0 else sem_stage.at[grp]
        return pltpu.make_async_copy(
            w_hbms[mat].at[pl.ds(d0, rows), pl.ds(16 * half, 16), :],
            stage.at[grp % NSTAGE, pl.ds(d0, rows)], sem)

    def slab_copies(src, dst, n, sem):
        return [pltpu.make_async_copy(src.at[:, pl.ds(j * 128, 128)], dst.at[j], sem)
                for j in range(n)]

    def relayout(src, dst, base, j0, j1, sh):
        for j in range(j0, j1):
            a = pltpu.bitcast(src[2 * j], U32)
            b = pltpu.bitcast(src[2 * j + 1], U32)
            if isinstance(sh, int):
                assert sh == 0
                y = (a & jnp.uint32(0xFFFF)) | (b << 16)
            else:
                y = ((a >> sh) & jnp.uint32(0xFFFF)) | ((b << (16 - sh)) & jnp.uint32(0xFFFF0000))
            dst[pl.ds(base + j, 8, stride=PITCH), :] = y

    def wpair(ref, slab0):
        return jnp.concatenate([_unpack(ref[pl.ds(slab0 * PITCH, D // 2), :]),
                                _unpack(ref[pl.ds((slab0 + 1) * PITCH, D // 2), :])], axis=1)

    def modrow(i):
        return mod_v[0:1, i * D:(i + 1) * D]

    def start_in_order(groups):
        def issue(i, carry):
            for k, grp in enumerate(groups):
                @pl.when(i == k)
                def _(grp=grp):
                    for cp in grp():
                        cp.start()
            return carry
        jax.lax.fori_loop(0, len(groups), issue, 0)

    start_in_order(
        [small_copies, lambda: [wmod_copy(0)], lambda: [x_copy(0)]]
        + [lambda ch=ch: [stage_copy(0, ch, 8)] for ch in range(8)]
        + ([lambda: [stage_copy(1, 0, 1)], lambda: [stage_copy(2, 0, 1)]] if STOP != 6 else []))

    ri = jax.lax.broadcasted_iota(jnp.int32, (80, 128), 0)
    ci = jax.lax.broadcasted_iota(jnp.int32, (80, 128), 1)

    def head_of(i):
        return jnp.where(i < 64, i // 32, (i - 64) // 8)

    def pos_of(i):
        return jnp.where(i < 64, i % 32, 32 + (i - 64) % 8)

    same = head_of(ri) == head_of(ci)
    pr, pc = pos_of(ri), pos_of(ci)
    keep = jnp.logical_or(pr < M, pr >= pc)
    code_v[...] = jnp.where(same, jnp.where(keep, 0.0, -1e9), -jnp.inf).astype(F32)

    for cp in small_copies():
        cp.wait()
    cf = c_v[...].astype(F32)
    sc = (cf * jax.nn.sigmoid(cf)).astype(BF16)
    sc16 = jnp.broadcast_to(sc, (16, D))
    bias_v[:, 0:FF] = jnp.broadcast_to(b1_v[...].astype(F32).reshape(1, FF), (8, FF))
    bias_v[:, FF:] = jnp.broadcast_to(b2_v[...].astype(F32).reshape(1, D), (8, D))

    wmod_copy(0).wait()
    mod_v[:, 0:2 * D] = _dot(sc16, wmod_v[:, 0:2 * D])[0:8]

    x_copy(0).wait()

    def ln1(xb):
        return _ln(xb.astype(F32)) * (1.0 + modrow(1)) + modrow(0)

    def h3_body(i, carry):
        s0 = pl.multiple_of(i * 8, 8)
        xb = x_v[pl.ds(s0, 8), 24:32, :].astype(F32).reshape(64, D)
        h = _ln(xb) * (1.0 + modrow(1)) + modrow(0)
        h3_v[pl.ds(pl.multiple_of(i * 32, 32), 32), :] = _pack(h)
        return carry

    jax.lax.fori_loop(0, 8, h3_body, 0)

    def g0_body(ch, carry):
        stage_copy(0, ch, 8).wait()
        src = stage.at[0, pl.ds(pl.multiple_of(ch * 128, 128), 128)]
        dst = wqkv.at[pl.ds(pl.multiple_of(ch * 64, 64), 8 * PITCH - 448), :]
        relayout(src, dst, 0, 0, 64, 0)
        return carry

    jax.lax.fori_loop(0, 8, g0_body, 0)
    if STOP == 6:
        return
    if STOP == 1:
        stage_copy(1, 0, 1).wait()
        stage_copy(2, 0, 1).wait()
        return

    def x3_matmul(wref, slab0, u, p, mc):
        lhs = _unpack(h3_v[mc * 64:(mc + 1) * 64, :])
        y = _dot(lhs, wpair(wref, slab0)).reshape(16, 8, 256)
        y = jnp.concatenate([y[:, :, :128], y[:, :, 128:]], axis=1).reshape(256, DH)
        qkv3[u, mc * 128:(mc + 1) * 128, p * DH:(p + 1) * DH] = _pack(y)

    def unit_body(u, carry):
        @pl.when(u == 1)
        def _():
            stage_copy(3, 0, 1).start()

        @pl.when(u == 2)
        def _():
            x_copy(1).start()
            for cp in slab_copies(wo_hbm, wo_v, 8, sem_w.at[2]):
                cp.start()

        @pl.when(u == 3)
        def _():
            stage_copy(4, 0, 1).start()

        @pl.when(u == 5)
        def _():
            stage_copy(5, 0, 1).start()

        @pl.when(u == 6)
        def _():
            wmod_copy(1).start()

        @pl.when(u == 7)
        def _():
            for cp in slab_copies(w1_hbm, w1_v, FF // 128, sem_w.at[3]):
                cp.start()

        @pl.when(u == 8)
        def _():
            for cp in slab_copies(w2_hbm, w2_v, 8, sem_w.at[4]):
                cp.start()

        gn = (u + 1) // 2
        src = stage.at[gn % NSTAGE]

        @pl.when(jnp.logical_and(u % 2 == 1, u < 11))
        def _():
            pltpu.make_async_copy(src, src, sem_stage.at[gn]).wait()

        sh = (((u + 1) % 2) * 16).astype(U32)
        view = wqkv.at[pl.ds(pl.multiple_of(u * (8 * PITCH), 8), 16 * PITCH), :]
        for p in range(4):
            for mc in range(4):
                x3_matmul(view, 2 * p, u, p, mc)
                relayout(src, view, 8 * PITCH, 32 * (4 * p + mc), 32 * (4 * p + mc + 1), sh)
        return carry

    jax.lax.fori_loop(0, 12, unit_body, 0)

    x_copy(1).wait()
    wmod_copy(1).wait()
    for cp in slab_copies(wo_hbm, wo_v, 8, sem_w.at[2]):
        cp.wait()

    if STOP == 2:
        for cp in slab_copies(w1_hbm, w1_v, FF // 128, sem_w.at[3]):
            cp.wait()
        for cp in slab_copies(w2_hbm, w2_v, 8, sem_w.at[4]):
            cp.wait()
        return

    def mod_rest(i):
        def run():
            cs = slice(2 * D + i * 512, 2 * D + (i + 1) * 512)
            mod_v[:, cs] = _dot(sc16, wmod_v[:, cs])[0:8]
        return run

    lhs_v[...] = _pack(jnp.concatenate([mem0_v[...].astype(F32), ln1(x_v[0, 0:24, :])], axis=0))

    zpad = jnp.zeros((24, DH), U32)

    def qkv_pair(g, seg):
        res = []
        if not PERSLAB:
            lhs = _unpack(lhs_v[...])
        for mat in range(3):
            sl = mat * H + 2 * g
            if PERSLAB:
                ys = []
                for i in range(2):
                    w = _unpack(wqkv[pl.ds((sl + i) * PITCH, D // 2), :])
                    y = _pack(_dot(_unpack(lhs_v[...]), w))
                    if SCR:
                        qkv_s[16 * i:16 * (i + 1), pl.ds(((g % NS) * 3 + mat) * DH, DH)] = y
                    ys.append(y)
            else:
                y = _dot(lhs, wpair(wqkv, sl))
                ys = [_pack(y[:, :DH]), _pack(y[:, DH:])]
                if SCR:
                    for i in range(2):
                        qkv_s[16 * i:16 * (i + 1), pl.ds(((g % NS) * 3 + mat) * DH, DH)] = ys[i]

            def get(mat=mat, ys=ys):
                parts = [qkv_s[:, pl.ds(((g % NS) * 3 + mat) * DH, DH)]] if SCR else list(ys)
                u3, p3 = divmod(mat * NPAIR + g, 4)
                parts.append(qkv3[u3, pl.ds(pl.multiple_of(seg * 8, 8), 8), p3 * DH:(p3 + 1) * DH])
                if mat > 0:
                    parts.append(zpad)
                return _unpack(jnp.concatenate(parts, axis=0))
            res.append(get)
        return res

    def scores(q, k):
        s = _dot_nt(q, k) * SCALE
        code = code_v[...]
        s = jnp.where(code == 0.0, s, code)
        m = jnp.max(s, axis=-1, keepdims=True)
        e = jnp.exp(s - m)
        l = jnp.sum(e, axis=-1, keepdims=True)
        r = pl.reciprocal(l, approx=True)
        r = r * (2.0 - l * r)
        return (e * r).astype(BF16)

    def pv(g, p, v, second):
        o = _dot(p, v)
        c0, c1 = (h * DH for h in _pair_heads(g))
        obuf[0:16, c0:c0 + DH] = _pack(o[0:32])
        obuf[0:16, c1:c1 + DH] = _pack(o[32:64])
        if not second:
            o3a[:, c0:c0 + DH] = o[64:72]
            o3a[:, c1:c1 + DH] = o[72:80]
        else:
            obuf[16:24, c0:c0 + DH] = _pack(jnp.concatenate([o3a[:, c0:c0 + DH], o[64:72]], axis=0))
            obuf[16:24, c1:c1 + DH] = _pack(jnp.concatenate([o3a[:, c1:c1 + DH], o[72:80]], axis=0))

    def step(seg, second, fillers):
        qkv = {}
        sm = {}
        for i in range(NPAIR + PVLAG + 1):
            if i < NPAIR:
                qkv[i] = qkv_pair(i, seg)
            if i in fillers:
                fillers[i]()
            if 0 <= i - SLAG < NPAIR:
                q, k, _ = qkv[i - SLAG]
                p = scores(q(), k())
                if SCR:
                    p_s[:, pl.ds(((i - SLAG) % NS) * DH, DH)] = pltpu.bitcast(p, U32)
                sm[i - SLAG] = p
            if 0 <= i - PVLAG < NPAIR:
                g = i - PVLAG
                p = _unpack(p_s[:, pl.ds((g % NS) * DH, DH)]) if SCR else sm[g]
                pv(g, p, qkv.pop(g)[2](), second)
        nrow = 24 if second else 16
        for j in range(8):
            y = _dot(_unpack(obuf[0:nrow, :]), wo_v[j])
            cs = slice(j * 128, (j + 1) * 128)
            lhs_v[:, cs] = _pack(jnp.concatenate([y[0:8], hn_v[:, cs]], axis=0))
            if not second:
                att_v[0:24, cs] = y[8:32]
            else:
                att_v[32:56, cs] = y[8:32]
                att_v[24:32, cs] = y[32:40]
                att_v[56:64, cs] = y[40:48]
        if NPAIR + PVLAG + 1 in fillers:
            fillers[NPAIR + PVLAG + 1]()

    def ffn_pre(tp):
        xb = x_v[pl.ds(2 * tp, 2)].astype(F32).reshape(64, D)
        x1 = xb + modrow(2) * att_v[...]
        x1_v[...] = x1
        h2_v[...] = _pack(_ln(x1) * (1.0 + modrow(4)) + modrow(3))

    def ffn1(lo, hi):
        def run():
            for j in range(lo, hi):
                cs = slice(j * 128, (j + 1) * 128)
                y = _dot(_unpack(h2_v[...]), w1_v[j]) + bias_v[0:1, cs]
                g_v[:, cs] = _pack(jax.nn.gelu(y, approximate=True))
        return run

    def ffn2(tp, lo, hi):
        def run():
            for j in range(lo, hi):
                cs = slice(j * 128, (j + 1) * 128)
                y = _dot(_unpack(g_v[...]), w2_v[j]) + bias_v[0:1, FF + j * 128:FF + (j + 1) * 128]
                o = x1_v[:, cs] + mod_v[0:1, 5 * D + j * 128:5 * D + (j + 1) * 128] * y
                out_v[tp, :, cs] = o.astype(BF16)
        return run

    def out_copy(tp):
        return pltpu.make_async_copy(out_v.at[tp], out_hbm.at[tp], sem_out.at[0])

    def seq(*fs):
        def run():
            for f in fs:
                f()
        return run

    def double_step(t, with_ffn):
        if with_ffn:
            ffn_pre(t - 1)
            fa = {k: ffn1(a, b) for k, (a, b) in FA.items()}
            fb = {k: ffn2(t - 1, a, b) for k, (a, b) in FB.items()}
        else:
            fa = {NPAIR + k: mod_rest(k) for k in range(4)}
            fb = {NPAIR + k: mod_rest(4 + k) for k in range(4)}
        hn_v[...] = ln1(x_v[2 * t + 1, 0:24, :])
        step(2 * t, False, fa)
        nxt = jnp.minimum(2 * t + 2, NSEG - 1)
        hn_v[...] = ln1(x_v[nxt, 0:24, :])
        step(2 * t + 1, True, fb)
        if with_ffn:
            out_copy(t - 1).start()

    double_step(0, False)
    for cp in slab_copies(w1_hbm, w1_v, FF // 128, sem_w.at[3]):
        cp.wait()
    for cp in slab_copies(w2_hbm, w2_v, 8, sem_w.at[4]):
        cp.wait()

    if STOP == 3:
        return

    def body(t, carry):
        double_step(t, True)
        return carry

    jax.lax.fori_loop(1, NITER, body, 0)

    last = NITER - 1
    ffn_pre(last)
    ffn1(0, FF // 128)()
    ffn2(last, 0, 8)()
    out_copy(last).start()
    pltpu.make_async_copy(out_v.at[0:NITER], out_hbm.at[0:NITER], sem_out.at[0]).wait()


@functools.partial(jax.jit, static_argnames=("A_seg_len",))
def pallas_adaLN_cond__memory_aug_recurrent_mem_tr__dense_activation_gelu__prompt_kernel(
    A_x, A_mem0, A_Wq, A_Wk, A_Wv, A_Wo, A_seg_len, B_x, B_w1, B_b1, B_w2, B_b2, c, w_mod,
):
    assert A_x.shape == (1, S, D) and A_mem0.shape == (1, M, D) and A_seg_len == SEG
    assert A_Wq.shape == (D, H, DH) and B_w1.shape == (D, FF)
    any_spec = pl.BlockSpec(memory_space=pl.ANY)
    scratch = [
        pltpu.VMEM((NSEG, SEG, D), BF16),
        pltpu.VMEM((NSEG // 2, 2 * SEG, D), BF16),
        pltpu.VMEM((NSTAGE, D, 16, DH), BF16),
        pltpu.VMEM(((3 * H + 8) * PITCH, DH), U32),
        pltpu.VMEM((8, H * DH, 128), BF16),
        pltpu.VMEM((FF // 128, D, 128), BF16),
        pltpu.VMEM((8, FF, 128), BF16),
        pltpu.VMEM((D, 6 * D), BF16),
        pltpu.VMEM((M, D), BF16),
        pltpu.VMEM((FF,), BF16),
        pltpu.VMEM((D,), BF16),
        pltpu.VMEM((1, D), BF16),
        pltpu.VMEM((8, 6 * D), F32),
        pltpu.VMEM((8, FF + D), F32),
        pltpu.VMEM((256, D), U32),
        pltpu.VMEM((12, NSEG * 8, 4 * DH), U32),
        pltpu.VMEM((80, 128), F32),
        pltpu.VMEM((16, D), U32),
        pltpu.VMEM((32, NS * 3 * DH), U32),
        pltpu.VMEM((40, NS * DH), U32),
        pltpu.VMEM((24, H * DH), U32),
        pltpu.VMEM((8, H * DH), F32),
        pltpu.VMEM((64, D), F32),
        pltpu.VMEM((64, D), F32),
        pltpu.VMEM((32, D), U32),
        pltpu.VMEM((32, FF), U32),
        pltpu.VMEM((24, D), F32),
        pltpu.SemaphoreType.DMA((4,)),
        pltpu.SemaphoreType.DMA((2,)),
        pltpu.SemaphoreType.DMA((8,)),
        pltpu.SemaphoreType.DMA((6,)),
        pltpu.SemaphoreType.DMA((5,)),
        pltpu.SemaphoreType.DMA((1,)),
    ]
    out = pl.pallas_call(
        _kernel,
        out_shape=jax.ShapeDtypeStruct((NSEG // 2, 2 * SEG, D), BF16),
        in_specs=[any_spec] * 12,
        out_specs=any_spec,
        scratch_shapes=scratch,
        compiler_params=pltpu.CompilerParams(vmem_limit_bytes=120 * 1024 * 1024),
    )(
        A_x.reshape(NSEG, SEG, D), A_mem0.reshape(M, D), A_Wq, A_Wk, A_Wv,
        A_Wo.reshape(H * DH, D), B_w1, B_b1, B_w2, B_b2,
        c, w_mod,
    )
    return out.reshape(1, S, D)
```

```python
import functools

import jax
import jax.numpy as jnp
import jax.experimental.pallas as pl
import jax.experimental.pallas.tpu as pltpu

F32 = jnp.float32
BF16 = jnp.bfloat16
U32 = jnp.uint32

S = 2048
D = 1024
H = 32
DH = 128
M = 8
SEG = 32
NSEG = S // SEG
FF = 3584
NPAIR = H // 2
PITCH = 516
XA = 8
NSTAGE = 4
STOP = 0
XHU = 2
PVLAG = 3
SLAG = 1
NS = 16
FA = {16: (0, 5), 17: (5, 10), 18: (10, 15), 19: (15, 24), 20: (24, 28)}
FB = {16: (0, 2), 17: (2, 4), 18: (4, 6), 19: (6, 8)}
PERSLAB = False
SCR = True
NITER = NSEG // 2
EPS = 1e-5
SCALE = DH ** (-0.5)


def _pair_heads(gp):
    half, r = divmod(gp, 8)
    par, i = divmod(r, 4)
    h0 = 16 * half + 4 * i + par
    return h0, h0 + 2


def _ln(xf):
    m = jnp.mean(xf, axis=-1, keepdims=True)
    xc = xf - m
    v = jnp.mean(xc * xc, axis=-1, keepdims=True)
    return xc * jax.lax.rsqrt(v + EPS)


def _dot(a, b):
    return jnp.dot(a, b, preferred_element_type=F32)


def _dot_nt(a, b):
    return jax.lax.dot_general(a, b, (((1,), (1,)), ((), ())), preferred_element_type=F32)


def _pack(xf):
    return pltpu.bitcast(xf.astype(BF16), U32)


def _unpack(u):
    return pltpu.bitcast(u, BF16)


def _kernel(x_hbm, mem0_hbm, wq_hbm, wk_hbm, wv_hbm, wo_hbm, w1_hbm, b1_hbm, w2_hbm, b2_hbm,
            c_hbm, wmod_hbm,
            out_hbm,
            x_v, out_v, stage, wqkv, wo_v, w1_v, w2_v, wm0_v, wm1_v,
            mem0_v, b1_v, b2_v, c_v,
            mod_v, modq_v, sc_v, bias_v, xh_v, h3_v, acc_v, qkv3, code_v,
            lhs_v, qkv_s, p_s, obuf, o3a, att_v, x1_v, h2_v, g_v, hn_v,
            sem_small, sem_x, sem_q, sem_stage, sem_w, sem_out):
    w_hbms = (wq_hbm, wk_hbm, wv_hbm)

    def mo(i, n):
        return i if isinstance(i, int) else pl.multiple_of(i, n)

    def small_copies():
        return [pltpu.make_async_copy(c_hbm, c_v, sem_small.at[0]),
                pltpu.make_async_copy(mem0_hbm, mem0_v, sem_small.at[1]),
                pltpu.make_async_copy(b1_hbm, b1_v, sem_small.at[2]),
                pltpu.make_async_copy(b2_hbm, b2_v, sem_small.at[3])]

    def x_copy(part):
        s0, ns, lo, n = [(0, NSEG, 24, 8), (0, XA, 0, 24), (XA, NSEG - XA, 0, 24)][part]
        return pltpu.make_async_copy(x_hbm.at[pl.ds(s0, ns), pl.ds(lo, n), :],
                                     x_v.at[pl.ds(s0, ns), pl.ds(lo, n), :], sem_x.at[part])

    def wq_chunk_copy(j, sem):
        d0 = mo((j >> 1) * 128, 128)
        hf = j & 1
        return pltpu.make_async_copy(wq_hbm.at[pl.ds(d0, 128), pl.ds(mo(16 * hf, 16), 16), :],
                                     stage.at[hf, pl.ds(d0, 128)], sem)

    def wm0_copy(i, sem):
        c0 = mo((i & 1) * D + (i >> 1) * 128, 128)
        return pltpu.make_async_copy(wmod_hbm.at[:, pl.ds(c0, 128)], wm0_v.at[i], sem)

    def g2_piece_copy(j, sem):
        d0 = mo(j * 64, 64)
        return pltpu.make_async_copy(wk_hbm.at[pl.ds(d0, 64), pl.ds(0, 16), :],
                                     stage.at[2, pl.ds(d0, 64)], sem)

    def group_copy(grp):
        mat, half = divmod(grp, 2)
        return pltpu.make_async_copy(w_hbms[mat].at[:, pl.ds(16 * half, 16), :],
                                     stage.at[grp % NSTAGE], sem_stage.at[grp])

    def slab_copies(src, c0, dst, sem):
        return [pltpu.make_async_copy(src.at[:, pl.ds(c0 + j * 256, 256)], dst.at[j], sem)
                for j in range(dst.shape[0])]

    wo_copies = lambda: slab_copies(wo_hbm, 0, wo_v, sem_w.at[0])
    wm1_copies = lambda: slab_copies(wmod_hbm, 2 * D, wm1_v, sem_w.at[1])
    w1_copies = lambda: slab_copies(w1_hbm, 0, w1_v, sem_w.at[2])
    w2_copies = lambda: slab_copies(w2_hbm, 0, w2_v, sem_w.at[3])

    def wcol(ref, j):
        return ref[j // 2, :, (j % 2) * 128:(j % 2 + 1) * 128]

    def relayout(src, dst, base, j0, j1, sh):
        for j in range(j0, j1):
            a = pltpu.bitcast(src[2 * j], U32)
            b = pltpu.bitcast(src[2 * j + 1], U32)
            if sh is None or isinstance(sh, int):
                y = (a & jnp.uint32(0xFFFF)) | (b << 16)
            else:
                y = ((a >> sh) & jnp.uint32(0xFFFF)) | ((b << (16 - sh)) & jnp.uint32(0xFFFF0000))
            dst[pl.ds(base + j, 8, stride=PITCH), :] = y
            if sh is None:
                y = (a >> 16) | (b & jnp.uint32(0xFFFF0000))
                dst[pl.ds(base + 8 * PITCH + j, 8, stride=PITCH), :] = y

    def wpair(ref, slab0, n=D // 2):
        return jnp.concatenate([_unpack(ref[pl.ds(slab0 * PITCH, n), :]),
                                _unpack(ref[pl.ds((slab0 + 1) * PITCH, n), :])], axis=1)

    def modrow(i):
        return mod_v[0:1, i * D:(i + 1) * D]

    def first_copies():
        return [wm0_copy(i, sem_q.at[16]) for i in range(2)] + [wq_chunk_copy(0, sem_q.at[16])]

    def q_copies(j, do):
        do(g2_piece_copy(j, sem_q.at[j]))

        @pl.when(j < 15)
        def _():
            do(wq_chunk_copy(j + 1, sem_q.at[j]))

        @pl.when(j < 14)
        def _():
            do(wm0_copy(j + 2, sem_q.at[j]))

    def issue(i, carry):
        @pl.when(i == 0)
        def _():
            for cp in small_copies():
                cp.start()
            x_copy(0).start()

        @pl.when(i == 1)
        def _():
            for cp in first_copies():
                cp.start()

        @pl.when(jnp.logical_and(i >= 2, i < 18))
        def _():
            q_copies(i - 2, lambda cp: cp.start())

        @pl.when(i == 18)
        def _():
            group_copy(3).start()
            x_copy(1).start()
        return carry

    jax.lax.fori_loop(0, 19, issue, 0)

    ri = jax.lax.broadcasted_iota(jnp.int32, (80, 128), 0)
    ci = jax.lax.broadcasted_iota(jnp.int32, (80, 128), 1)

    def head_of(i):
        return jnp.where(i < 64, i // 32, (i - 64) // 8)

    def pos_of(i):
        return jnp.where(i < 64, i % 32, 32 + (i - 64) % 8)

    same = head_of(ri) == head_of(ci)
    pr, pc = pos_of(ri), pos_of(ci)
    keep = jnp.logical_or(pr < M, pr >= pc)
    code_v[...] = jnp.where(same, jnp.where(keep, 0.0, -1e9), -jnp.inf).astype(F32)

    for cp in small_copies():
        cp.wait()
    cf = c_v[...].astype(F32)
    sc_v[...] = _pack(jnp.broadcast_to(cf * jax.nn.sigmoid(cf), (16, D)))
    bias_v[:, 0:FF] = jnp.broadcast_to(b1_v[...].astype(F32).reshape(1, FF), (8, FF))
    bias_v[:, FF:] = jnp.broadcast_to(b2_v[...].astype(F32).reshape(1, D), (8, D))

    x_copy(0).wait()

    def xh_body(i, carry):
        for h in range(XHU):
            s0 = pl.multiple_of((i * XHU + h) * 8, 8)
            xh = _ln(x_v[pl.ds(s0, 8), 24:32, :].astype(F32).reshape(64, D))
            r0 = pl.multiple_of((i * XHU + h) * 64, 64)
            for kt in range(8):
                xh_v[kt, pl.ds(r0, 64), :] = xh[:, kt * 128:(kt + 1) * 128]
        return carry

    jax.lax.fori_loop(0, 8 // XHU, xh_body, 0)

    def mod_slab(i):
        modq_v[i] = _dot(_unpack(sc_v[...]), wm0_v[i])[0:8]

    def h3_chunk(kt):
        sa = modq_v[2 * kt, 0:1, :]
        ca = modq_v[2 * kt + 1, 0:1, :]
        return _pack(xh_v[kt] * (1.0 + ca) + sa)

    for cp in first_copies():
        cp.wait()
    modq_v[2:16] = jnp.zeros((14, 8, 128), F32)
    for i in range(2):
        mod_slab(i)
    h3_v[0] = h3_chunk(0)
    relayout(stage.at[0], wqkv, 0, 0, 64, None)

    def q_body(j, carry):
        q_copies(j, lambda cp: cp.wait())
        kt, hf = j >> 1, j & 1
        jn = jnp.minimum(j + 1, 15)
        ktn, hfn = jn >> 1, jn & 1
        hview = h3_v.at[pl.ds(kt, 2)]
        wview = wqkv.at[pl.ds(pl.multiple_of(hf * (16 * PITCH) + kt * 64, 8), 16 * PITCH - 448), :]
        aview = acc_v.at[pl.ds(pl.multiple_of(hf * 8, 8), 8)]
        qsrc = stage.at[hfn, pl.ds(pl.multiple_of(ktn * 128, 128), 128)]
        qdst = wqkv.at[pl.ds(pl.multiple_of(hfn * (16 * PITCH) + ktn * 64, 8), 16 * PITCH - 448), :]
        ksrc = stage.at[2, pl.ds(pl.multiple_of(j * 64, 64), 64)]
        kdst = wqkv.at[pl.ds(pl.multiple_of(32 * PITCH + j * 32, 8), 8 * PITCH - 480), :]
        for p in range(8):
            y = _dot(_unpack(hview[0]), wpair(wview, 2 * p, 64))
            aview[p] = jnp.where(kt > 0, aview[p], 0.0) + y
            if p == 1:
                mod_slab(jnp.minimum(j + 2, 15))
            if p == 5:
                hview[1] = h3_chunk(jnp.minimum(kt + 1, 7))
            relayout(qsrc, qdst, 0, 8 * p, 8 * p + 8, None)
            relayout(ksrc, kdst, 0, 4 * p, 4 * p + 4, 0)
        return carry

    jax.lax.fori_loop(0, 16, q_body, 0)
    for kt in range(8):
        mod_v[:, kt * 128:(kt + 1) * 128] = modq_v[2 * kt]
        mod_v[:, D + kt * 128:D + (kt + 1) * 128] = modq_v[2 * kt + 1]
    if STOP == 1:
        group_copy(3).wait()
        x_copy(1).wait()
        return

    def ln1(xb):
        return _ln(xb.astype(F32)) * (1.0 + modrow(1)) + modrow(0)

    def store_x3(dst, half, mc, y):
        y = y.reshape(16, 8, 256)
        y = jnp.concatenate([y[:, :, :128], y[:, :, 128:]], axis=1).reshape(256, DH)
        dst[mc * 128:(mc + 1) * 128, half * DH:(half + 1) * DH] = _pack(y)

    def unit_body(u, carry):
        for k, cps in enumerate([lambda: [group_copy(4), group_copy(5)], wo_copies, wm1_copies,
                                 w1_copies, w2_copies, lambda: [x_copy(2)]]):
            @pl.when(u == 4 + k)
            def _(cps=cps):
                for cp in cps():
                    cp.start()

        gn = (u + 1) >> 1
        src = stage.at[gn & (NSTAGE - 1)]

        @pl.when(jnp.logical_and(u & 1 == 1, u < 11))
        def _():
            pltpu.make_async_copy(src, src, sem_stage.at[gn]).wait()

        sh = (((u + 1) & 1) * 16).astype(U32)
        view = wqkv.at[pl.ds(pl.multiple_of(u * (8 * PITCH), 8), 16 * PITCH), :]
        for p in range(4):
            for mc in range(4):
                lhs = _unpack(jnp.concatenate(
                    [h3_v[kt, mc * 64:(mc + 1) * 64, :] for kt in range(8)], axis=1))
                store_x3(qkv3.at[2 * u + p // 2], p % 2, mc, _dot(lhs, wpair(view, 2 * p)))
                relayout(src, view, 8 * PITCH, 32 * (4 * p + mc), 32 * (4 * p + mc + 1), sh)
                if p % 2 == 0:
                    store_x3(qkv3.at[u - 4], p // 2, mc,
                             acc_v[2 * (u - 4) + p // 2, mc * 128:(mc + 1) * 128, :])
        return carry

    jax.lax.fori_loop(4, 12, unit_body, 0)

    x_copy(1).wait()
    for cp in wo_copies() + wm1_copies():
        cp.wait()
    if STOP == 2:
        for cp in w1_copies() + w2_copies() + [x_copy(2)]:
            cp.wait()
        return

    def mod_rest(i):
        def run():
            for j in range(2 * i, 2 * i + 2):
                mod_v[:, 2 * D + j * 256:2 * D + (j + 1) * 256] = _dot(
                    _unpack(sc_v[...]), wm1_v[j])[0:8]
        return run

    lhs_v[...] = _pack(jnp.concatenate([mem0_v[...].astype(F32), ln1(x_v[0, 0:24, :])], axis=0))

    zpad = jnp.zeros((24, DH), U32)

    def qkv_pair(g, seg):
        res = []
        if not PERSLAB:
            lhs = _unpack(lhs_v[...])
        for mat in range(3):
            sl = mat * H + 2 * g
            if PERSLAB:
                ys = []
                for i in range(2):
                    w = _unpack(wqkv[pl.ds((sl + i) * PITCH, D // 2), :])
                    y = _pack(_dot(_unpack(lhs_v[...]), w))
                    if SCR:
                        qkv_s[16 * i:16 * (i + 1), pl.ds(((g % NS) * 3 + mat) * DH, DH)] = y
                    ys.append(y)
            else:
                y = _dot(lhs, wpair(wqkv, sl))
                ys = [_pack(y[:, :DH]), _pack(y[:, DH:])]
                if SCR:
                    for i in range(2):
                        qkv_s[16 * i:16 * (i + 1), pl.ds(((g % NS) * 3 + mat) * DH, DH)] = ys[i]

            def get(mat=mat, ys=ys):
                parts = [qkv_s[:, pl.ds(((g % NS) * 3 + mat) * DH, DH)]] if SCR else list(ys)
                u3, p3 = divmod(mat * NPAIR + g, 2)
                parts.append(qkv3[u3, pl.ds(pl.multiple_of(seg * 8, 8), 8), p3 * DH:(p3 + 1) * DH])
                if mat > 0:
                    parts.append(zpad)
                return _unpack(jnp.concatenate(parts, axis=0))
            res.append(get)
        return res

    def scores(q, k):
        s = _dot_nt(q, k) * SCALE
        code = code_v[...]
        s = jnp.where(code == 0.0, s, code)
        m = jnp.max(s, axis=-1, keepdims=True)
        e = jnp.exp(s - m)
        l = jnp.sum(e, axis=-1, keepdims=True)
        r = pl.reciprocal(l, approx=True)
        r = r * (2.0 - l * r)
        return (e * r).astype(BF16)

    def pv(g, p, v, second):
        o = _dot(p, v)
        c0, c1 = (h * DH for h in _pair_heads(g))
        obuf[0:16, c0:c0 + DH] = _pack(o[0:32])
        obuf[0:16, c1:c1 + DH] = _pack(o[32:64])
        if not second:
            o3a[:, c0:c0 + DH] = o[64:72]
            o3a[:, c1:c1 + DH] = o[72:80]
        else:
            obuf[16:24, c0:c0 + DH] = _pack(jnp.concatenate([o3a[:, c0:c0 + DH], o[64:72]], axis=0))
            obuf[16:24, c1:c1 + DH] = _pack(jnp.concatenate([o3a[:, c1:c1 + DH], o[72:80]], axis=0))

    def step(seg, second, fillers):
        qkv = {}
        sm = {}
        for i in range(NPAIR + PVLAG + 1):
            if i < NPAIR:
                qkv[i] = qkv_pair(i, seg)
            if i in fillers:
                fillers[i]()
            if 0 <= i - SLAG < NPAIR:
                q, k, _ = qkv[i - SLAG]
                p = scores(q(), k())
                if SCR:
                    p_s[:, pl.ds(((i - SLAG) % NS) * DH, DH)] = pltpu.bitcast(p, U32)
                sm[i - SLAG] = p
            if 0 <= i - PVLAG < NPAIR:
                g = i - PVLAG
                p = _unpack(p_s[:, pl.ds((g % NS) * DH, DH)]) if SCR else sm[g]
                pv(g, p, qkv.pop(g)[2](), second)
        nrow = 24 if second else 16
        for j in range(8):
            y = _dot(_unpack(obuf[0:nrow, :]), wcol(wo_v, j))
            cs = slice(j * 128, (j + 1) * 128)
            lhs_v[:, cs] = _pack(jnp.concatenate([y[0:8], hn_v[:, cs]], axis=0))
            if not second:
                att_v[0:24, cs] = y[8:32]
            else:
                att_v[32:56, cs] = y[8:32]
                att_v[24:32, cs] = y[32:40]
                att_v[56:64, cs] = y[40:48]
        if NPAIR + PVLAG + 1 in fillers:
            fillers[NPAIR + PVLAG + 1]()

    def ffn_pre(tp):
        xb = x_v[pl.ds(2 * tp, 2)].astype(F32).reshape(64, D)
        x1 = xb + modrow(2) * att_v[...]
        x1_v[...] = x1
        h2_v[...] = _pack(_ln(x1) * (1.0 + modrow(4)) + modrow(3))

    def ffn1(lo, hi):
        def run():
            for j in range(lo, hi):
                cs = slice(j * 128, (j + 1) * 128)
                y = _dot(_unpack(h2_v[...]), wcol(w1_v, j)) + bias_v[0:1, cs]
                g_v[:, cs] = _pack(jax.nn.gelu(y, approximate=True))
        return run

    def ffn2(tp, lo, hi):
        def run():
            for j in range(lo, hi):
                cs = slice(j * 128, (j + 1) * 128)
                y = _dot(_unpack(g_v[...]), wcol(w2_v, j)) + bias_v[0:1, FF + j * 128:FF + (j + 1) * 128]
                o = x1_v[:, cs] + mod_v[0:1, 5 * D + j * 128:5 * D + (j + 1) * 128] * y
                out_v[tp, :, cs] = o.astype(BF16)
        return run

    def out_copy(tp):
        return pltpu.make_async_copy(out_v.at[tp], out_hbm.at[tp], sem_out.at[0])

    def seq(*fs):
        def run():
            for f in fs:
                f()
        return run

    def double_step(t, with_ffn):
        if with_ffn:
            ffn_pre(t - 1)
            fa = {k: ffn1(a, b) for k, (a, b) in FA.items()}
            fb = {k: ffn2(t - 1, a, b) for k, (a, b) in FB.items()}
        else:
            fa = {NPAIR + k: mod_rest(k) for k in range(4)}
            fb = {NPAIR + k: mod_rest(4 + k) for k in range(4)}
        hn_v[...] = ln1(x_v[2 * t + 1, 0:24, :])
        step(2 * t, False, fa)
        nxt = jnp.minimum(2 * t + 2, NSEG - 1)
        hn_v[...] = ln1(x_v[nxt, 0:24, :])
        step(2 * t + 1, True, fb)
        if with_ffn:
            out_copy(t - 1).start()

    double_step(0, False)
    for cp in w1_copies() + w2_copies():
        cp.wait()
    if STOP == 3:
        x_copy(2).wait()
        return

    def body(t, carry):
        @pl.when(t == 2)
        def _():
            x_copy(2).wait()
        double_step(t, True)
        return carry

    jax.lax.fori_loop(1, NITER, body, 0)

    last = NITER - 1
    ffn_pre(last)
    ffn1(0, FF // 128)()
    ffn2(last, 0, 8)()
    out_copy(last).start()
    pltpu.make_async_copy(out_v.at[0:NITER], out_hbm.at[0:NITER], sem_out.at[0]).wait()


@functools.partial(jax.jit, static_argnames=("A_seg_len",))
def pallas_adaLN_cond__memory_aug_recurrent_mem_tr__dense_activation_gelu__prompt_kernel(
    A_x, A_mem0, A_Wq, A_Wk, A_Wv, A_Wo, A_seg_len, B_x, B_w1, B_b1, B_w2, B_b2, c, w_mod,
):
    assert A_x.shape == (1, S, D) and A_mem0.shape == (1, M, D) and A_seg_len == SEG
    assert A_Wq.shape == (D, H, DH) and B_w1.shape == (D, FF)
    any_spec = pl.BlockSpec(memory_space=pl.ANY)
    scratch = [
        pltpu.VMEM((NSEG, SEG, D), BF16),
        pltpu.VMEM((NSEG // 2, 2 * SEG, D), BF16),
        pltpu.VMEM((NSTAGE, D, 16, DH), BF16),
        pltpu.VMEM(((3 * H + 8) * PITCH, DH), U32),
        pltpu.VMEM((4, H * DH, 256), BF16),
        pltpu.VMEM((FF // 256, D, 256), BF16),
        pltpu.VMEM((4, FF, 256), BF16),
        pltpu.VMEM((16, D, 128), BF16),
        pltpu.VMEM((16, D, 256), BF16),
        pltpu.VMEM((M, D), BF16),
        pltpu.VMEM((FF,), BF16),
        pltpu.VMEM((D,), BF16),
        pltpu.VMEM((1, D), BF16),
        pltpu.VMEM((8, 6 * D), F32),
        pltpu.VMEM((16, 8, 128), F32),
        pltpu.VMEM((8, D), U32),
        pltpu.VMEM((8, FF + D), F32),
        pltpu.VMEM((8, NSEG * 8, 128), F32),
        pltpu.VMEM((9, NSEG * 4, 128), U32),
        pltpu.VMEM((NPAIR, NSEG * 8, 2 * DH), F32),
        pltpu.VMEM((24, NSEG * 8, 2 * DH), U32),
        pltpu.VMEM((80, 128), F32),
        pltpu.VMEM((16, D), U32),
        pltpu.VMEM((32, NS * 3 * DH), U32),
        pltpu.VMEM((40, NS * DH), U32),
        pltpu.VMEM((24, H * DH), U32),
        pltpu.VMEM((8, H * DH), F32),
        pltpu.VMEM((64, D), F32),
        pltpu.VMEM((64, D), F32),
        pltpu.VMEM((32, D), U32),
        pltpu.VMEM((32, FF), U32),
        pltpu.VMEM((24, D), F32),
        pltpu.SemaphoreType.DMA((4,)),
        pltpu.SemaphoreType.DMA((3,)),
        pltpu.SemaphoreType.DMA((17,)),
        pltpu.SemaphoreType.DMA((6,)),
        pltpu.SemaphoreType.DMA((4,)),
        pltpu.SemaphoreType.DMA((1,)),
    ]
    out = pl.pallas_call(
        _kernel,
        out_shape=jax.ShapeDtypeStruct((NSEG // 2, 2 * SEG, D), BF16),
        in_specs=[any_spec] * 12,
        out_specs=any_spec,
        scratch_shapes=scratch,
        compiler_params=pltpu.CompilerParams(vmem_limit_bytes=120 * 1024 * 1024,
                                             disable_bounds_checks=True),
    )(
        A_x.reshape(NSEG, SEG, D), A_mem0.reshape(M, D), A_Wq, A_Wk, A_Wv,
        A_Wo.reshape(H * DH, D), B_w1, B_b1, B_w2, B_b2,
        c, w_mod,
    )
    return out.reshape(1, S, D)
```

```python
import functools

import jax
import jax.numpy as jnp
import jax.experimental.pallas as pl
import jax.experimental.pallas.tpu as pltpu

F32 = jnp.float32
BF16 = jnp.bfloat16
U32 = jnp.uint32

S = 2048
D = 1024
H = 32
DH = 128
M = 8
SEG = 32
NSEG = S // SEG
FF = 3584
NPAIR = H // 2
PITCH = 516
XA = 8
NSTAGE = 4
STOP = 0
XHU = 2
PVLAG = 3
SLAG = 1
NS = 16
FA = {16: (0, 5), 17: (5, 10), 18: (10, 15), 19: (15, 24), 20: (24, 28)}
FB = {16: (0, 2), 17: (2, 4), 18: (4, 6), 19: (6, 8)}
PERSLAB = False
SCR = True
NITER = NSEG // 2
EPS = 1e-5
SCALE = DH ** (-0.5)


def _pair_heads(gp):
    half, r = divmod(gp, 8)
    par, i = divmod(r, 4)
    h0 = 16 * half + 4 * i + par
    return h0, h0 + 2


def _ln(xf):
    m = jnp.mean(xf, axis=-1, keepdims=True)
    xc = xf - m
    v = jnp.mean(xc * xc, axis=-1, keepdims=True)
    return xc * jax.lax.rsqrt(v + EPS)


def _dot(a, b):
    return jnp.dot(a, b, preferred_element_type=F32)


def _dot_nt(a, b):
    return jax.lax.dot_general(a, b, (((1,), (1,)), ((), ())), preferred_element_type=F32)


def _pack(xf):
    return pltpu.bitcast(xf.astype(BF16), U32)


def _unpack(u):
    return pltpu.bitcast(u, BF16)


def _kernel(x_hbm, mem0_hbm, wq_hbm, wk_hbm, wv_hbm, wo_hbm, w1_hbm, b1_hbm, w2_hbm, b2_hbm,
            c_hbm, wmod_hbm,
            out_hbm,
            x_v, out_v, stage, wqkv, wo_v, w1_v, w2_v, wm0_v, wm1_v,
            mem0_v, b1_v, b2_v, c_v,
            mod_v, modq_v, sc_v, bias_v, xh_v, h3_v, acc_v, qkv3, code_v,
            lhs_v, qkv_s, p_s, obuf, o3a, att_v, x1_v, h2_v, g_v, hn_v,
            sem_small, sem_x, sem_q, sem_stage, sem_w, sem_out):
    w_hbms = (wq_hbm, wk_hbm, wv_hbm)

    def mo(i, n):
        return i if isinstance(i, int) else pl.multiple_of(i, n)

    def small_copies():
        return [pltpu.make_async_copy(c_hbm, c_v, sem_small.at[0]),
                pltpu.make_async_copy(mem0_hbm, mem0_v, sem_small.at[1]),
                pltpu.make_async_copy(b1_hbm, b1_v, sem_small.at[2]),
                pltpu.make_async_copy(b2_hbm, b2_v, sem_small.at[3])]

    def x_copy(part):
        s0, ns, lo, n = [(0, NSEG, 24, 8), (0, XA, 0, 24), (XA, NSEG - XA, 0, 24)][part]
        return pltpu.make_async_copy(x_hbm.at[pl.ds(s0, ns), pl.ds(lo, n), :],
                                     x_v.at[pl.ds(s0, ns), pl.ds(lo, n), :], sem_x.at[part])

    def wq_chunk_copy(j, sem):
        d0 = mo((j >> 1) * 128, 128)
        hf = j & 1
        return pltpu.make_async_copy(wq_hbm.at[pl.ds(d0, 128), pl.ds(mo(16 * hf, 16), 16), :],
                                     stage.at[hf, pl.ds(d0, 128)], sem)

    def wm0_copy(i, sem):
        c0 = mo((i & 1) * D + (i >> 1) * 128, 128)
        return pltpu.make_async_copy(wmod_hbm.at[:, pl.ds(c0, 128)], wm0_v.at[i], sem)

    def g2_piece_copy(j, sem):
        d0 = mo(j * 64, 64)
        return pltpu.make_async_copy(wk_hbm.at[pl.ds(d0, 64), pl.ds(0, 16), :],
                                     stage.at[2, pl.ds(d0, 64)], sem)

    def group_copy(grp):
        mat, half = divmod(grp, 2)
        return pltpu.make_async_copy(w_hbms[mat].at[:, pl.ds(16 * half, 16), :],
                                     stage.at[grp % NSTAGE], sem_stage.at[grp])

    def slab_copies(src, c0, dst, sem):
        return [pltpu.make_async_copy(src.at[:, pl.ds(c0 + j * 256, 256)], dst.at[j], sem)
                for j in range(dst.shape[0])]

    wo_copies = lambda: slab_copies(wo_hbm, 0, wo_v, sem_w.at[0])
    wm1_copies = lambda: slab_copies(wmod_hbm, 2 * D, wm1_v, sem_w.at[1])
    w1_copies = lambda: slab_copies(w1_hbm, 0, w1_v, sem_w.at[2])
    w2_copies = lambda: slab_copies(w2_hbm, 0, w2_v, sem_w.at[3])

    def wcol(ref, j):
        return ref[j // 2, :, (j % 2) * 128:(j % 2 + 1) * 128]

    def relayout(src, dst, j0, j1):
        srcu = src.bitcast(U32)
        for j in range(j0, j1):
            a = srcu[2 * j]
            b = srcu[2 * j + 1]
            dst[pl.ds(j, 8, stride=PITCH), :] = (a & jnp.uint32(0xFFFF)) | (b << 16)
            dst[pl.ds(8 * PITCH + j, 8, stride=PITCH), :] = (a >> 16) | (b & jnp.uint32(0xFFFF0000))

    def wpair(ref, slab0, n=D // 2):
        return jnp.concatenate([_unpack(ref[pl.ds(slab0 * PITCH, n), :]),
                                _unpack(ref[pl.ds((slab0 + 1) * PITCH, n), :])], axis=1)

    def modrow(i):
        return mod_v[0:1, i * D:(i + 1) * D]

    def first_copies():
        return [wm0_copy(i, sem_q.at[16]) for i in range(2)] + [wq_chunk_copy(0, sem_q.at[16])]

    def q_copies(j, do):
        do(g2_piece_copy(j, sem_q.at[j]))

        @pl.when(j < 15)
        def _():
            do(wq_chunk_copy(j + 1, sem_q.at[j]))

        @pl.when(j < 14)
        def _():
            do(wm0_copy(j + 2, sem_q.at[j]))

    def issue(i, carry):
        @pl.when(i == 0)
        def _():
            for cp in small_copies():
                cp.start()
            x_copy(0).start()

        @pl.when(i == 1)
        def _():
            for cp in first_copies():
                cp.start()

        @pl.when(jnp.logical_and(i >= 2, i < 18))
        def _():
            q_copies(i - 2, lambda cp: cp.start())

        @pl.when(i == 18)
        def _():
            group_copy(3).start()
            x_copy(1).start()
        return carry

    jax.lax.fori_loop(0, 19, issue, 0)

    ri = jax.lax.broadcasted_iota(jnp.int32, (80, 128), 0)
    ci = jax.lax.broadcasted_iota(jnp.int32, (80, 128), 1)

    def head_of(i):
        return jnp.where(i < 64, i // 32, (i - 64) // 8)

    def pos_of(i):
        return jnp.where(i < 64, i % 32, 32 + (i - 64) % 8)

    same = head_of(ri) == head_of(ci)
    pr, pc = pos_of(ri), pos_of(ci)
    keep = jnp.logical_or(pr < M, pr >= pc)
    code_v[...] = jnp.where(same, jnp.where(keep, 0.0, -1e9), -jnp.inf).astype(F32)

    for cp in small_copies():
        cp.wait()
    cf = c_v[...].astype(F32)
    sc_v[...] = _pack(jnp.broadcast_to(cf * jax.nn.sigmoid(cf), (16, D)))
    bias_v[:, 0:FF] = jnp.broadcast_to(b1_v[...].astype(F32).reshape(1, FF), (8, FF))
    bias_v[:, FF:] = jnp.broadcast_to(b2_v[...].astype(F32).reshape(1, D), (8, D))

    x_copy(0).wait()

    def xh_body(i, carry):
        for h in range(XHU):
            s0 = pl.multiple_of((i * XHU + h) * 8, 8)
            xh = _ln(x_v[pl.ds(s0, 8), 24:32, :].astype(F32).reshape(64, D))
            r0 = pl.multiple_of((i * XHU + h) * 64, 64)
            for kt in range(8):
                xh_v[kt, pl.ds(r0, 64), :] = xh[:, kt * 128:(kt + 1) * 128]
        return carry

    jax.lax.fori_loop(0, 8 // XHU, xh_body, 0)

    def mod_slab(i):
        modq_v[i] = _dot(_unpack(sc_v[...]), wm0_v[i])[0:8]

    def h3_chunk(kt):
        sa = modq_v[2 * kt, 0:1, :]
        ca = modq_v[2 * kt + 1, 0:1, :]
        return _pack(xh_v[kt] * (1.0 + ca) + sa)

    for cp in first_copies():
        cp.wait()
    modq_v[2:16] = jnp.zeros((14, 8, 128), F32)
    for i in range(2):
        mod_slab(i)
    h3_v[0] = h3_chunk(0)
    relayout(stage.at[0], wqkv, 0, 64)

    def q_body(j, carry):
        q_copies(j, lambda cp: cp.wait())
        kt, hf = j >> 1, j & 1
        jn = jnp.minimum(j + 1, 15)
        ktn, hfn = jn >> 1, jn & 1
        hview = h3_v.at[pl.ds(kt, 2)]
        wview = wqkv.at[pl.ds(pl.multiple_of(hf * (16 * PITCH) + kt * 64, 8), 16 * PITCH - 448), :]
        aview = acc_v.at[pl.ds(pl.multiple_of(hf * 8, 8), 8)]
        qsrc = stage.at[hfn, pl.ds(pl.multiple_of(ktn * 128, 128), 128)]
        qdst = wqkv.at[pl.ds(pl.multiple_of(hfn * (16 * PITCH) + ktn * 64, 8), 16 * PITCH - 448), :]
        ksrc = stage.at[2, pl.ds(pl.multiple_of(j * 64, 64), 64)]
        kdst = wqkv.at[pl.ds(pl.multiple_of(32 * PITCH + j * 32, 8), 16 * PITCH - 480), :]
        for p in range(8):
            y = _dot(_unpack(hview[0]), wpair(wview, 2 * p, 64))
            aview[p] = jnp.where(kt > 0, aview[p], 0.0) + y
            if p == 1:
                mod_slab(jnp.minimum(j + 2, 15))
            if p == 5:
                hview[1] = h3_chunk(jnp.minimum(kt + 1, 7))
            relayout(qsrc, qdst, 8 * p, 8 * p + 8)
            relayout(ksrc, kdst, 4 * p, 4 * p + 4)
        return carry

    jax.lax.fori_loop(0, 16, q_body, 0)
    for kt in range(8):
        mod_v[:, kt * 128:(kt + 1) * 128] = modq_v[2 * kt]
        mod_v[:, D + kt * 128:D + (kt + 1) * 128] = modq_v[2 * kt + 1]
    if STOP == 1:
        group_copy(3).wait()
        x_copy(1).wait()
        return

    def ln1(xb):
        return _ln(xb.astype(F32)) * (1.0 + modrow(1)) + modrow(0)

    def store_x3(dst, half, mc, y):
        y = y.reshape(16, 8, 256)
        y = jnp.concatenate([y[:, :, :128], y[:, :, 128:]], axis=1).reshape(256, DH)
        dst[mc * 128:(mc + 1) * 128, half * DH:(half + 1) * DH] = _pack(y)

    def unit_body(u, carry):
        for k, cps in enumerate([lambda: [group_copy(4), group_copy(5)], wo_copies, wm1_copies,
                                 w1_copies, w2_copies, lambda: [x_copy(2)]]):
            @pl.when(u == 4 + k)
            def _(cps=cps):
                for cp in cps():
                    cp.start()

        gn = jnp.minimum((u >> 1) + 1, 5)
        slot = stage.at[gn & (NSTAGE - 1)]

        @pl.when(jnp.logical_and(u & 1 == 0, u < 10))
        def _():
            pltpu.make_async_copy(slot, slot, sem_stage.at[gn]).wait()

        src = slot.at[pl.ds(pl.multiple_of((u & 1) * 512, 512), 512)]
        dst = wqkv.at[pl.ds(pl.multiple_of(gn * (16 * PITCH) + (u & 1) * 256, 8), 16 * PITCH - 256), :]
        view = wqkv.at[pl.ds(pl.multiple_of(u * (8 * PITCH), 8), 8 * PITCH), :]
        for p in range(4):
            for mc in range(4):
                lhs = _unpack(jnp.concatenate(
                    [h3_v[kt, mc * 64:(mc + 1) * 64, :] for kt in range(8)], axis=1))
                store_x3(qkv3.at[2 * u + p // 2], p % 2, mc, _dot(lhs, wpair(view, 2 * p)))
                relayout(src, dst, 16 * (4 * p + mc), 16 * (4 * p + mc + 1))
                if p % 2 == 0:
                    store_x3(qkv3.at[u - 4], p // 2, mc,
                             acc_v[2 * (u - 4) + p // 2, mc * 128:(mc + 1) * 128, :])
        return carry

    jax.lax.fori_loop(4, 12, unit_body, 0)

    x_copy(1).wait()
    for cp in wo_copies() + wm1_copies():
        cp.wait()
    if STOP == 2:
        for cp in w1_copies() + w2_copies() + [x_copy(2)]:
            cp.wait()
        return

    def mod_rest(i):
        def run():
            for j in range(2 * i, 2 * i + 2):
                mod_v[:, 2 * D + j * 256:2 * D + (j + 1) * 256] = _dot(
                    _unpack(sc_v[...]), wm1_v[j])[0:8]
        return run

    lhs_v[...] = _pack(jnp.concatenate([mem0_v[...].astype(F32), ln1(x_v[0, 0:24, :])], axis=0))

    zpad = jnp.zeros((24, DH), U32)

    def qkv_pair(g, seg):
        res = []
        if not PERSLAB:
            lhs = _unpack(lhs_v[...])
        for mat in range(3):
            sl = mat * H + 2 * g
            if PERSLAB:
                ys = []
                for i in range(2):
                    w = _unpack(wqkv[pl.ds((sl + i) * PITCH, D // 2), :])
                    y = _pack(_dot(_unpack(lhs_v[...]), w))
                    if SCR:
                        qkv_s[16 * i:16 * (i + 1), pl.ds(((g % NS) * 3 + mat) * DH, DH)] = y
                    ys.append(y)
            else:
                y = _dot(lhs, wpair(wqkv, sl))
                ys = [_pack(y[:, :DH]), _pack(y[:, DH:])]
                if SCR:
                    for i in range(2):
                        qkv_s[16 * i:16 * (i + 1), pl.ds(((g % NS) * 3 + mat) * DH, DH)] = ys[i]

            def get(mat=mat, ys=ys):
                parts = [qkv_s[:, pl.ds(((g % NS) * 3 + mat) * DH, DH)]] if SCR else list(ys)
                u3, p3 = divmod(mat * NPAIR + g, 2)
                parts.append(qkv3[u3, pl.ds(pl.multiple_of(seg * 8, 8), 8), p3 * DH:(p3 + 1) * DH])
                if mat > 0:
                    parts.append(zpad)
                return _unpack(jnp.concatenate(parts, axis=0))
            res.append(get)
        return res

    def scores(q, k):
        s = _dot_nt(q, k) * SCALE
        code = code_v[...]
        s = jnp.where(code == 0.0, s, code)
        m = jnp.max(s, axis=-1, keepdims=True)
        e = jnp.exp(s - m)
        l = jnp.sum(e, axis=-1, keepdims=True)
        r = pl.reciprocal(l, approx=True)
        r = r * (2.0 - l * r)
        return (e * r).astype(BF16)

    def pv(g, p, v, second):
        o = _dot(p, v)
        c0, c1 = (h * DH for h in _pair_heads(g))
        obuf[0:16, c0:c0 + DH] = _pack(o[0:32])
        obuf[0:16, c1:c1 + DH] = _pack(o[32:64])
        if not second:
            o3a[:, c0:c0 + DH] = o[64:72]
            o3a[:, c1:c1 + DH] = o[72:80]
        else:
            obuf[16:24, c0:c0 + DH] = _pack(jnp.concatenate([o3a[:, c0:c0 + DH], o[64:72]], axis=0))
            obuf[16:24, c1:c1 + DH] = _pack(jnp.concatenate([o3a[:, c1:c1 + DH], o[72:80]], axis=0))

    def step(seg, second, fillers):
        qkv = {}
        sm = {}
        for i in range(NPAIR + PVLAG + 1):
            if i < NPAIR:
                qkv[i] = qkv_pair(i, seg)
            if i in fillers:
                fillers[i]()
            if 0 <= i - SLAG < NPAIR:
                q, k, _ = qkv[i - SLAG]
                p = scores(q(), k())
                if SCR:
                    p_s[:, pl.ds(((i - SLAG) % NS) * DH, DH)] = pltpu.bitcast(p, U32)
                sm[i - SLAG] = p
            if 0 <= i - PVLAG < NPAIR:
                g = i - PVLAG
                p = _unpack(p_s[:, pl.ds((g % NS) * DH, DH)]) if SCR else sm[g]
                pv(g, p, qkv.pop(g)[2](), second)
        nrow = 24 if second else 16
        for j in range(8):
            y = _dot(_unpack(obuf[0:nrow, :]), wcol(wo_v, j))
            cs = slice(j * 128, (j + 1) * 128)
            lhs_v[:, cs] = _pack(jnp.concatenate([y[0:8], hn_v[:, cs]], axis=0))
            if not second:
                att_v[0:24, cs] = y[8:32]
            else:
                att_v[32:56, cs] = y[8:32]
                att_v[24:32, cs] = y[32:40]
                att_v[56:64, cs] = y[40:48]
        if NPAIR + PVLAG + 1 in fillers:
            fillers[NPAIR + PVLAG + 1]()

    def ffn_pre(tp):
        xb = x_v[pl.ds(2 * tp, 2)].astype(F32).reshape(64, D)
        x1 = xb + modrow(2) * att_v[...]
        x1_v[...] = x1
        h2_v[...] = _pack(_ln(x1) * (1.0 + modrow(4)) + modrow(3))

    def ffn1(lo, hi):
        def run():
            for j in range(lo, hi):
                cs = slice(j * 128, (j + 1) * 128)
                y = _dot(_unpack(h2_v[...]), wcol(w1_v, j)) + bias_v[0:1, cs]
                g_v[:, cs] = _pack(jax.nn.gelu(y, approximate=True))
        return run

    def ffn2(tp, lo, hi):
        def run():
            for j in range(lo, hi):
                cs = slice(j * 128, (j + 1) * 128)
                y = _dot(_unpack(g_v[...]), wcol(w2_v, j)) + bias_v[0:1, FF + j * 128:FF + (j + 1) * 128]
                o = x1_v[:, cs] + mod_v[0:1, 5 * D + j * 128:5 * D + (j + 1) * 128] * y
                out_v[tp, :, cs] = o.astype(BF16)
        return run

    def out_copy(tp):
        return pltpu.make_async_copy(out_v.at[tp], out_hbm.at[tp], sem_out.at[0])

    def seq(*fs):
        def run():
            for f in fs:
                f()
        return run

    def double_step(t, with_ffn):
        if with_ffn:
            ffn_pre(t - 1)
            fa = {k: ffn1(a, b) for k, (a, b) in FA.items()}
            fb = {k: ffn2(t - 1, a, b) for k, (a, b) in FB.items()}
        else:
            fa = {NPAIR + k: mod_rest(k) for k in range(4)}
            fb = {NPAIR + k: mod_rest(4 + k) for k in range(4)}
        hn_v[...] = ln1(x_v[2 * t + 1, 0:24, :])
        step(2 * t, False, fa)
        nxt = jnp.minimum(2 * t + 2, NSEG - 1)
        hn_v[...] = ln1(x_v[nxt, 0:24, :])
        step(2 * t + 1, True, fb)
        if with_ffn:
            out_copy(t - 1).start()

    double_step(0, False)
    for cp in w1_copies() + w2_copies():
        cp.wait()
    if STOP == 3:
        x_copy(2).wait()
        return

    def body(t, carry):
        @pl.when(t == 2)
        def _():
            x_copy(2).wait()
        double_step(t, True)
        return carry

    jax.lax.fori_loop(1, NITER, body, 0)

    last = NITER - 1
    ffn_pre(last)
    ffn1(0, FF // 128)()
    ffn2(last, 0, 8)()
    out_copy(last).start()
    pltpu.make_async_copy(out_v.at[0:NITER], out_hbm.at[0:NITER], sem_out.at[0]).wait()


@functools.partial(jax.jit, static_argnames=("A_seg_len",))
def pallas_adaLN_cond__memory_aug_recurrent_mem_tr__dense_activation_gelu__prompt_kernel(
    A_x, A_mem0, A_Wq, A_Wk, A_Wv, A_Wo, A_seg_len, B_x, B_w1, B_b1, B_w2, B_b2, c, w_mod,
):
    assert A_x.shape == (1, S, D) and A_mem0.shape == (1, M, D) and A_seg_len == SEG
    assert A_Wq.shape == (D, H, DH) and B_w1.shape == (D, FF)
    any_spec = pl.BlockSpec(memory_space=pl.ANY)
    scratch = [
        pltpu.VMEM((NSEG, SEG, D), BF16),
        pltpu.VMEM((NSEG // 2, 2 * SEG, D), BF16),
        pltpu.VMEM((NSTAGE, D, 16, DH), BF16),
        pltpu.VMEM((3 * H * PITCH, DH), U32),
        pltpu.VMEM((4, H * DH, 256), BF16),
        pltpu.VMEM((FF // 256, D, 256), BF16),
        pltpu.VMEM((4, FF, 256), BF16),
        pltpu.VMEM((16, D, 128), BF16),
        pltpu.VMEM((16, D, 256), BF16),
        pltpu.VMEM((M, D), BF16),
        pltpu.VMEM((FF,), BF16),
        pltpu.VMEM((D,), BF16),
        pltpu.VMEM((1, D), BF16),
        pltpu.VMEM((8, 6 * D), F32),
        pltpu.VMEM((16, 8, 128), F32),
        pltpu.VMEM((8, D), U32),
        pltpu.VMEM((8, FF + D), F32),
        pltpu.VMEM((8, NSEG * 8, 128), F32),
        pltpu.VMEM((9, NSEG * 4, 128), U32),
        pltpu.VMEM((NPAIR, NSEG * 8, 2 * DH), F32),
        pltpu.VMEM((24, NSEG * 8, 2 * DH), U32),
        pltpu.VMEM((80, 128), F32),
        pltpu.VMEM((16, D), U32),
        pltpu.VMEM((32, NS * 3 * DH), U32),
        pltpu.VMEM((40, NS * DH), U32),
        pltpu.VMEM((24, H * DH), U32),
        pltpu.VMEM((8, H * DH), F32),
        pltpu.VMEM((64, D), F32),
        pltpu.VMEM((64, D), F32),
        pltpu.VMEM((32, D), U32),
        pltpu.VMEM((32, FF), U32),
        pltpu.VMEM((24, D), F32),
        pltpu.SemaphoreType.DMA((4,)),
        pltpu.SemaphoreType.DMA((3,)),
        pltpu.SemaphoreType.DMA((17,)),
        pltpu.SemaphoreType.DMA((6,)),
        pltpu.SemaphoreType.DMA((4,)),
        pltpu.SemaphoreType.DMA((1,)),
    ]
    out = pl.pallas_call(
        _kernel,
        out_shape=jax.ShapeDtypeStruct((NSEG // 2, 2 * SEG, D), BF16),
        in_specs=[any_spec] * 12,
        out_specs=any_spec,
        scratch_shapes=scratch,
        compiler_params=pltpu.CompilerParams(vmem_limit_bytes=120 * 1024 * 1024,
                                             disable_bounds_checks=True),
    )(
        A_x.reshape(NSEG, SEG, D), A_mem0.reshape(M, D), A_Wq, A_Wk, A_Wv,
        A_Wo.reshape(H * DH, D), B_w1, B_b1, B_w2, B_b2,
        c, w_mod,
    )
    return out.reshape(1, S, D)
```

```python
import functools

import jax
import jax.numpy as jnp
import jax.experimental.pallas as pl
import jax.experimental.pallas.tpu as pltpu

F32 = jnp.float32
BF16 = jnp.bfloat16
U32 = jnp.uint32

S = 2048
D = 1024
H = 32
DH = 128
M = 8
SEG = 32
NSEG = S // SEG
FF = 3584
NPAIR = H // 2
PITCH = 516
XA = 8
NSTAGE = 4
STOP = 0
XHU = 2
PVLAG = 3
SLAG = 1
NS = 16
FA = {16: (0, 5), 17: (5, 10), 18: (10, 15), 19: (15, 24), 20: (24, 28)}
FB = {16: (0, 2), 17: (2, 4), 18: (4, 6), 19: (6, 8)}
PERSLAB = False
SCR = True
NITER = NSEG // 2
EPS = 1e-5
SCALE = DH ** (-0.5)


def _pair_heads(gp):
    half, r = divmod(gp, 8)
    par, i = divmod(r, 4)
    h0 = 16 * half + 4 * i + par
    return h0, h0 + 2


def _ln(xf):
    m = jnp.mean(xf, axis=-1, keepdims=True)
    xc = xf - m
    v = jnp.mean(xc * xc, axis=-1, keepdims=True)
    return xc * jax.lax.rsqrt(v + EPS)


def _dot(a, b):
    return jnp.dot(a, b, preferred_element_type=F32)


def _dot_nt(a, b):
    return jax.lax.dot_general(a, b, (((1,), (1,)), ((), ())), preferred_element_type=F32)


def _pack(xf):
    return pltpu.bitcast(xf.astype(BF16), U32)


def _unpack(u):
    return pltpu.bitcast(u, BF16)


def _kernel(x_hbm, mem0_hbm, wq_hbm, wk_hbm, wv_hbm, wo_hbm, w1_hbm, b1_hbm, w2_hbm, b2_hbm,
            c_hbm, wmod_hbm,
            out_hbm,
            x_v, out_v, stage, wqkv, wo_v, w1_v, w2_v, wm0_v, wm1_v,
            mem0_v, b1_v, b2_v, c_v,
            mod_v, modq_v, sc_v, bias_v, xh_v, h3_v, acc_v, qkv3, code_v,
            lhs_v, qkv_s, p_s, obuf, o3a, att_v, x1_v, h2_v, g_v, hn_v,
            sem_small, sem_x, sem_q, sem_stage, sem_w, sem_out):
    w_hbms = (wq_hbm, wk_hbm, wv_hbm)

    def mo(i, n):
        return i if isinstance(i, int) else pl.multiple_of(i, n)

    def small_copies():
        return [pltpu.make_async_copy(c_hbm, c_v, sem_small.at[0]),
                pltpu.make_async_copy(mem0_hbm, mem0_v, sem_small.at[1]),
                pltpu.make_async_copy(b1_hbm, b1_v, sem_small.at[2]),
                pltpu.make_async_copy(b2_hbm, b2_v, sem_small.at[3])]

    def x_copy(part):
        s0, ns, lo, n = [(0, NSEG, 24, 8), (0, XA, 0, 24), (XA, NSEG - XA, 0, 24)][part]
        return pltpu.make_async_copy(x_hbm.at[pl.ds(s0, ns), pl.ds(lo, n), :],
                                     x_v.at[pl.ds(s0, ns), pl.ds(lo, n), :], sem_x.at[part])

    def wq_chunk_copy(j, sem):
        d0 = mo((j >> 1) * 128, 128)
        hf = j & 1
        return pltpu.make_async_copy(wq_hbm.at[pl.ds(d0, 128), pl.ds(mo(16 * hf, 16), 16), :],
                                     stage.at[hf, pl.ds(d0, 128)], sem)

    def wm0_copy(i, sem):
        c0 = mo((i & 1) * D + (i >> 1) * 128, 128)
        return pltpu.make_async_copy(wmod_hbm.at[:, pl.ds(c0, 128)], wm0_v.at[i], sem)

    def g2_piece_copy(j, sem):
        d0 = mo(j * 64, 64)
        return pltpu.make_async_copy(wk_hbm.at[pl.ds(d0, 64), pl.ds(0, 16), :],
                                     stage.at[2, pl.ds(d0, 64)], sem)

    def group_copy(grp):
        mat, half = divmod(grp, 2)
        return pltpu.make_async_copy(w_hbms[mat].at[:, pl.ds(16 * half, 16), :],
                                     stage.at[grp % NSTAGE], sem_stage.at[grp])

    def slab_copies(src, c0, dst, sem):
        return [pltpu.make_async_copy(src.at[:, pl.ds(c0 + j * 256, 256)], dst.at[j], sem)
                for j in range(dst.shape[0])]

    wo_copies = lambda: slab_copies(wo_hbm, 0, wo_v, sem_w.at[0])
    wm1_copies = lambda: slab_copies(wmod_hbm, 2 * D, wm1_v, sem_w.at[1])
    w1_copies = lambda: slab_copies(w1_hbm, 0, w1_v, sem_w.at[2])
    w2_copies = lambda: slab_copies(w2_hbm, 0, w2_v, sem_w.at[3])

    def wcol(ref, j):
        return ref[j // 2, :, (j % 2) * 128:(j % 2 + 1) * 128]

    def relayout(src, dst, j0, j1):
        srcu = src.bitcast(U32)
        for j in range(j0, j1):
            a = srcu[2 * j]
            b = srcu[2 * j + 1]
            dst[pl.ds(j, 8, stride=PITCH), :] = (a & jnp.uint32(0xFFFF)) | (b << 16)
            dst[pl.ds(8 * PITCH + j, 8, stride=PITCH), :] = (a >> 16) | (b & jnp.uint32(0xFFFF0000))

    def wpair(ref, slab0, n=D // 2):
        return jnp.concatenate([_unpack(ref[pl.ds(slab0 * PITCH, n), :]),
                                _unpack(ref[pl.ds((slab0 + 1) * PITCH, n), :])], axis=1)

    def modrow(i):
        return mod_v[0:1, i * D:(i + 1) * D]

    def first_copies():
        return [wm0_copy(i, sem_q.at[16]) for i in range(2)] + [wq_chunk_copy(0, sem_q.at[16])]

    def q_copies(j, do):
        do(g2_piece_copy(j, sem_q.at[j]))

        @pl.when(j < 15)
        def _():
            do(wq_chunk_copy(j + 1, sem_q.at[j]))

        @pl.when(j < 14)
        def _():
            do(wm0_copy(j + 2, sem_q.at[j]))

    def issue(i, carry):
        @pl.when(i == 0)
        def _():
            for cp in small_copies():
                cp.start()
            x_copy(0).start()

        @pl.when(i == 1)
        def _():
            for cp in first_copies():
                cp.start()

        @pl.when(jnp.logical_and(i >= 2, i < 18))
        def _():
            q_copies(i - 2, lambda cp: cp.start())

        @pl.when(i == 18)
        def _():
            group_copy(3).start()
            x_copy(1).start()
        return carry

    jax.lax.fori_loop(0, 19, issue, 0)

    ri = jax.lax.broadcasted_iota(jnp.int32, (80, 128), 0)
    ci = jax.lax.broadcasted_iota(jnp.int32, (80, 128), 1)

    def head_of(i):
        return jnp.where(i < 64, i // 32, (i - 64) // 8)

    def pos_of(i):
        return jnp.where(i < 64, i % 32, 32 + (i - 64) % 8)

    same = head_of(ri) == head_of(ci)
    pr, pc = pos_of(ri), pos_of(ci)
    keep = jnp.logical_or(pr < M, pr >= pc)
    code_v[...] = jnp.where(same, jnp.where(keep, 0.0, -1e9), -jnp.inf).astype(F32)

    for cp in small_copies():
        cp.wait()
    cf = c_v[...].astype(F32)
    sc_v[...] = _pack(jnp.broadcast_to(cf * jax.nn.sigmoid(cf), (16, D)))
    bias_v[:, 0:FF] = jnp.broadcast_to(b1_v[...].astype(F32).reshape(1, FF), (8, FF))
    bias_v[:, FF:] = jnp.broadcast_to(b2_v[...].astype(F32).reshape(1, D), (8, D))

    x_copy(0).wait()

    def xh_body(i, carry):
        for h in range(XHU):
            s0 = pl.multiple_of((i * XHU + h) * 8, 8)
            xh = _ln(x_v[pl.ds(s0, 8), 24:32, :].astype(F32).reshape(64, D))
            r0 = pl.multiple_of((i * XHU + h) * 64, 64)
            for kt in range(8):
                xh_v[kt, pl.ds(r0, 64), :] = xh[:, kt * 128:(kt + 1) * 128]
        return carry

    jax.lax.fori_loop(0, 8 // XHU, xh_body, 0)

    def mod_slab(i):
        modq_v[i] = _dot(_unpack(sc_v[...]), _unpack(wm0_v.bitcast(U32)[i]))[0:8]

    def h3_store(dst, kt, mc):
        sa = modq_v[2 * kt, 0:1, :]
        ca = modq_v[2 * kt + 1, 0:1, :]
        dst[:, mc * 128:(mc + 1) * 128] = _pack(
            xh_v[kt, mc * 128:(mc + 1) * 128, :] * (1.0 + ca) + sa)

    for cp in first_copies():
        cp.wait()
    modq_v[2:16] = jnp.zeros((14, 8, 128), F32)
    for i in range(2):
        mod_slab(i)
    for mc in range(4):
        h3_store(h3_v.at[0], 0, mc)
    relayout(stage.at[0], wqkv, 0, 64)

    def q_body(j, carry):
        q_copies(j, lambda cp: cp.wait())
        kt, hf = j >> 1, j & 1
        jn = jnp.minimum(j + 1, 15)
        ktn, hfn = jn >> 1, jn & 1
        hview = h3_v.at[pl.ds(kt, 2)]
        wview = wqkv.at[pl.ds(pl.multiple_of(hf * (16 * PITCH) + kt * 64, 8), 16 * PITCH - 448), :]
        aview = acc_v.at[pl.ds(pl.multiple_of(hf * 8, 8), 8)]
        qsrc = stage.at[hfn, pl.ds(pl.multiple_of(ktn * 128, 128), 128)]
        qdst = wqkv.at[pl.ds(pl.multiple_of(hfn * (16 * PITCH) + ktn * 64, 8), 16 * PITCH - 448), :]
        ksrc = stage.at[2, pl.ds(pl.multiple_of(j * 64, 64), 64)]
        kdst = wqkv.at[pl.ds(pl.multiple_of(32 * PITCH + j * 32, 8), 16 * PITCH - 480), :]
        for p in range(8):
            lhs = jnp.concatenate([hview[0, :, mc * 128:(mc + 1) * 128] for mc in range(4)], axis=0)
            y = _dot(_unpack(lhs), wpair(wview, 2 * p, 64))
            aview[p] = jnp.where(kt > 0, aview[p], 0.0) + y
            if p == 1:
                mod_slab(jnp.minimum(j + 2, 15))
            if p >= 4:
                h3_store(hview.at[1], jnp.minimum(kt + 1, 7), p - 4)
            if p % 2 == 1:
                relayout(qsrc, qdst, 8 * p - 8, 8 * p + 8)
                relayout(ksrc, kdst, 4 * p - 4, 4 * p + 4)
        return carry

    jax.lax.fori_loop(0, 16, q_body, 0)
    for kt in range(8):
        mod_v[:, kt * 128:(kt + 1) * 128] = modq_v[2 * kt]
        mod_v[:, D + kt * 128:D + (kt + 1) * 128] = modq_v[2 * kt + 1]
    if STOP == 1:
        group_copy(3).wait()
        x_copy(1).wait()
        return

    def ln1(xb):
        return _ln(xb.astype(F32)) * (1.0 + modrow(1)) + modrow(0)

    def store_x3(dst, half, mc, y):
        y = y.reshape(16, 8, 256)
        y = jnp.concatenate([y[:, :, :128], y[:, :, 128:]], axis=1).reshape(256, DH)
        dst[mc * 128:(mc + 1) * 128, half * DH:(half + 1) * DH] = _pack(y)

    def unit_body(u, carry):
        gn = jnp.minimum((u >> 1) + 1, 5)
        slot = stage.at[gn & (NSTAGE - 1)]

        @pl.when(jnp.logical_and(u & 1 == 0, u < 10))
        def _():
            pltpu.make_async_copy(slot, slot, sem_stage.at[gn]).wait()

        for k, cps in enumerate([lambda: [group_copy(4), group_copy(5)], wo_copies, wm1_copies,
                                 w1_copies, w2_copies, lambda: [x_copy(2)]]):
            @pl.when(u == 4 + k)
            def _(cps=cps):
                for cp in cps():
                    cp.start()

        src = slot.at[pl.ds(pl.multiple_of((u & 1) * 512, 512), 512)]
        dst = wqkv.at[pl.ds(pl.multiple_of(gn * (16 * PITCH) + (u & 1) * 256, 8), 16 * PITCH - 256), :]
        view = wqkv.at[pl.ds(pl.multiple_of(u * (8 * PITCH), 8), 8 * PITCH), :]
        for p in range(4):
            for mc in range(4):
                lhs = _unpack(jnp.concatenate(
                    [h3_v[kt, :, mc * 128:(mc + 1) * 128] for kt in range(8)], axis=1))
                store_x3(qkv3.at[2 * u + p // 2], p % 2, mc, _dot(lhs, wpair(view, 2 * p)))
                relayout(src, dst, 16 * (4 * p + mc), 16 * (4 * p + mc + 1))
                if p % 2 == 0:
                    store_x3(qkv3.at[u - 4], p // 2, mc,
                             acc_v[2 * (u - 4) + p // 2, mc * 128:(mc + 1) * 128, :])
        return carry

    jax.lax.fori_loop(4, 12, unit_body, 0)

    x_copy(1).wait()
    for cp in wo_copies() + wm1_copies():
        cp.wait()
    if STOP == 2:
        for cp in w1_copies() + w2_copies() + [x_copy(2)]:
            cp.wait()
        return

    def mod_rest(i):
        def run():
            for j in range(2 * i, 2 * i + 2):
                mod_v[:, 2 * D + j * 256:2 * D + (j + 1) * 256] = _dot(
                    _unpack(sc_v[...]), wm1_v[j])[0:8]
        return run

    lhs_v[...] = _pack(jnp.concatenate([mem0_v[...].astype(F32), ln1(x_v[0, 0:24, :])], axis=0))

    zpad = jnp.zeros((24, DH), U32)

    def qkv_pair(g, seg):
        res = []
        if not PERSLAB:
            lhs = _unpack(lhs_v[...])
        for mat in range(3):
            sl = mat * H + 2 * g
            if PERSLAB:
                ys = []
                for i in range(2):
                    w = _unpack(wqkv[pl.ds((sl + i) * PITCH, D // 2), :])
                    y = _pack(_dot(_unpack(lhs_v[...]), w))
                    if SCR:
                        qkv_s[16 * i:16 * (i + 1), pl.ds(((g % NS) * 3 + mat) * DH, DH)] = y
                    ys.append(y)
            else:
                y = _dot(lhs, wpair(wqkv, sl))
                ys = [_pack(y[:, :DH]), _pack(y[:, DH:])]
                if SCR:
                    for i in range(2):
                        qkv_s[16 * i:16 * (i + 1), pl.ds(((g % NS) * 3 + mat) * DH, DH)] = ys[i]

            def get(mat=mat, ys=ys):
                parts = [qkv_s[:, pl.ds(((g % NS) * 3 + mat) * DH, DH)]] if SCR else list(ys)
                u3, p3 = divmod(mat * NPAIR + g, 2)
                parts.append(qkv3[u3, pl.ds(pl.multiple_of(seg * 8, 8), 8), p3 * DH:(p3 + 1) * DH])
                if mat > 0:
                    parts.append(zpad)
                return _unpack(jnp.concatenate(parts, axis=0))
            res.append(get)
        return res

    def scores(q, k):
        s = _dot_nt(q, k) * SCALE
        code = code_v[...]
        s = jnp.where(code == 0.0, s, code)
        m = jnp.max(s, axis=-1, keepdims=True)
        e = jnp.exp(s - m)
        l = jnp.sum(e, axis=-1, keepdims=True)
        r = pl.reciprocal(l, approx=True)
        r = r * (2.0 - l * r)
        return (e * r).astype(BF16)

    def pv(g, p, v, second):
        o = _dot(p, v)
        c0, c1 = (h * DH for h in _pair_heads(g))
        obuf[0:16, c0:c0 + DH] = _pack(o[0:32])
        obuf[0:16, c1:c1 + DH] = _pack(o[32:64])
        if not second:
            o3a[:, c0:c0 + DH] = o[64:72]
            o3a[:, c1:c1 + DH] = o[72:80]
        else:
            obuf[16:24, c0:c0 + DH] = _pack(jnp.concatenate([o3a[:, c0:c0 + DH], o[64:72]], axis=0))
            obuf[16:24, c1:c1 + DH] = _pack(jnp.concatenate([o3a[:, c1:c1 + DH], o[72:80]], axis=0))

    def step(seg, second, fillers):
        qkv = {}
        sm = {}
        for i in range(NPAIR + PVLAG + 1):
            if i < NPAIR:
                qkv[i] = qkv_pair(i, seg)
            if i in fillers:
                fillers[i]()
            if 0 <= i - SLAG < NPAIR:
                q, k, _ = qkv[i - SLAG]
                p = scores(q(), k())
                if SCR:
                    p_s[:, pl.ds(((i - SLAG) % NS) * DH, DH)] = pltpu.bitcast(p, U32)
                sm[i - SLAG] = p
            if 0 <= i - PVLAG < NPAIR:
                g = i - PVLAG
                p = _unpack(p_s[:, pl.ds((g % NS) * DH, DH)]) if SCR else sm[g]
                pv(g, p, qkv.pop(g)[2](), second)
        nrow = 24 if second else 16
        for j in range(8):
            y = _dot(_unpack(obuf[0:nrow, :]), wcol(wo_v, j))
            cs = slice(j * 128, (j + 1) * 128)
            lhs_v[:, cs] = _pack(jnp.concatenate([y[0:8], hn_v[:, cs]], axis=0))
            if not second:
                att_v[0:24, cs] = y[8:32]
            else:
                att_v[32:56, cs] = y[8:32]
                att_v[24:32, cs] = y[32:40]
                att_v[56:64, cs] = y[40:48]
        if NPAIR + PVLAG + 1 in fillers:
            fillers[NPAIR + PVLAG + 1]()

    def ffn_pre(tp):
        xb = x_v[pl.ds(2 * tp, 2)].astype(F32).reshape(64, D)
        x1 = xb + modrow(2) * att_v[...]
        x1_v[...] = x1
        h2_v[...] = _pack(_ln(x1) * (1.0 + modrow(4)) + modrow(3))

    def ffn1(lo, hi):
        def run():
            for j in range(lo, hi):
                cs = slice(j * 128, (j + 1) * 128)
                y = _dot(_unpack(h2_v[...]), wcol(w1_v, j)) + bias_v[0:1, cs]
                g_v[:, cs] = _pack(jax.nn.gelu(y, approximate=True))
        return run

    def ffn2(tp, lo, hi):
        def run():
            for j in range(lo, hi):
                cs = slice(j * 128, (j + 1) * 128)
                y = _dot(_unpack(g_v[...]), wcol(w2_v, j)) + bias_v[0:1, FF + j * 128:FF + (j + 1) * 128]
                o = x1_v[:, cs] + mod_v[0:1, 5 * D + j * 128:5 * D + (j + 1) * 128] * y
                out_v[tp, :, cs] = o.astype(BF16)
        return run

    def out_copy(tp):
        return pltpu.make_async_copy(out_v.at[tp], out_hbm.at[tp], sem_out.at[0])

    def seq(*fs):
        def run():
            for f in fs:
                f()
        return run

    def double_step(t, with_ffn):
        if with_ffn:
            ffn_pre(t - 1)
            fa = {k: ffn1(a, b) for k, (a, b) in FA.items()}
            fb = {k: ffn2(t - 1, a, b) for k, (a, b) in FB.items()}
        else:
            fa = {NPAIR + k: mod_rest(k) for k in range(4)}
            fb = {NPAIR + k: mod_rest(4 + k) for k in range(4)}
        hn_v[...] = ln1(x_v[2 * t + 1, 0:24, :])
        step(2 * t, False, fa)
        nxt = jnp.minimum(2 * t + 2, NSEG - 1)
        hn_v[...] = ln1(x_v[nxt, 0:24, :])
        step(2 * t + 1, True, fb)
        if with_ffn:
            out_copy(t - 1).start()

    double_step(0, False)
    for cp in w1_copies() + w2_copies():
        cp.wait()
    if STOP == 3:
        x_copy(2).wait()
        return

    def body(t, carry):
        @pl.when(t == 2)
        def _():
            x_copy(2).wait()
        double_step(t, True)
        return carry

    jax.lax.fori_loop(1, NITER, body, 0)

    last = NITER - 1
    ffn_pre(last)
    ffn1(0, FF // 128)()
    ffn2(last, 0, 8)()
    out_copy(last).start()
    pltpu.make_async_copy(out_v.at[0:NITER], out_hbm.at[0:NITER], sem_out.at[0]).wait()


@functools.partial(jax.jit, static_argnames=("A_seg_len",))
def pallas_adaLN_cond__memory_aug_recurrent_mem_tr__dense_activation_gelu__prompt_kernel(
    A_x, A_mem0, A_Wq, A_Wk, A_Wv, A_Wo, A_seg_len, B_x, B_w1, B_b1, B_w2, B_b2, c, w_mod,
):
    assert A_x.shape == (1, S, D) and A_mem0.shape == (1, M, D) and A_seg_len == SEG
    assert A_Wq.shape == (D, H, DH) and B_w1.shape == (D, FF)
    any_spec = pl.BlockSpec(memory_space=pl.ANY)
    scratch = [
        pltpu.VMEM((NSEG, SEG, D), BF16),
        pltpu.VMEM((NSEG // 2, 2 * SEG, D), BF16),
        pltpu.VMEM((NSTAGE, D, 16, DH), BF16),
        pltpu.VMEM((3 * H * PITCH, DH), U32),
        pltpu.VMEM((4, H * DH, 256), BF16),
        pltpu.VMEM((FF // 256, D, 256), BF16),
        pltpu.VMEM((4, FF, 256), BF16),
        pltpu.VMEM((16, D, 128), BF16),
        pltpu.VMEM((16, D, 256), BF16),
        pltpu.VMEM((M, D), BF16),
        pltpu.VMEM((FF,), BF16),
        pltpu.VMEM((D,), BF16),
        pltpu.VMEM((1, D), BF16),
        pltpu.VMEM((8, 6 * D), F32),
        pltpu.VMEM((16, 8, 128), F32),
        pltpu.VMEM((8, D), U32),
        pltpu.VMEM((8, FF + D), F32),
        pltpu.VMEM((8, NSEG * 8, 128), F32),
        pltpu.VMEM((9, 64, 512), U32),
        pltpu.VMEM((NPAIR, NSEG * 8, 2 * DH), F32),
        pltpu.VMEM((24, NSEG * 8, 2 * DH), U32),
        pltpu.VMEM((80, 128), F32),
        pltpu.VMEM((16, D), U32),
        pltpu.VMEM((32, NS * 3 * DH), U32),
        pltpu.VMEM((40, NS * DH), U32),
        pltpu.VMEM((24, H * DH), U32),
        pltpu.VMEM((8, H * DH), F32),
        pltpu.VMEM((64, D), F32),
        pltpu.VMEM((64, D), F32),
        pltpu.VMEM((32, D), U32),
        pltpu.VMEM((32, FF), U32),
        pltpu.VMEM((24, D), F32),
        pltpu.SemaphoreType.DMA((4,)),
        pltpu.SemaphoreType.DMA((3,)),
        pltpu.SemaphoreType.DMA((17,)),
        pltpu.SemaphoreType.DMA((6,)),
        pltpu.SemaphoreType.DMA((4,)),
        pltpu.SemaphoreType.DMA((1,)),
    ]
    out = pl.pallas_call(
        _kernel,
        out_shape=jax.ShapeDtypeStruct((NSEG // 2, 2 * SEG, D), BF16),
        in_specs=[any_spec] * 12,
        out_specs=any_spec,
        scratch_shapes=scratch,
        compiler_params=pltpu.CompilerParams(vmem_limit_bytes=120 * 1024 * 1024,
                                             disable_bounds_checks=True),
    )(
        A_x.reshape(NSEG, SEG, D), A_mem0.reshape(M, D), A_Wq, A_Wk, A_Wv,
        A_Wo.reshape(H * DH, D), B_w1, B_b1, B_w2, B_b2,
        c, w_mod,
    )
    return out.reshape(1, S, D)
```

```python
import functools

import jax
import jax.numpy as jnp
import jax.experimental.pallas as pl
import jax.experimental.pallas.tpu as pltpu

F32 = jnp.float32
BF16 = jnp.bfloat16
U32 = jnp.uint32

S = 2048
D = 1024
H = 32
DH = 128
M = 8
SEG = 32
NSEG = S // SEG
FF = 3584
NPAIR = H // 2
PITCH = 516
XA = 8
NSTAGE = 4
STOP = 0
XHU = 2
QOFF, KOFF, VOFF, SOFF, POFF = 0.0, 0.1, 0.2, 1.5, 3.6
SSCR = 0
NEWTON = 1
KMAJOR = 1
KSTEP = 2
PIN = 1
AHEAD = 0
HNA = 17.9
HNB = 18.9
FB1 = {}
WSPLIT = 0
WSPLIT0 = 0
WEARLY = [16.0, 16.1, 17.0, 17.1, 18.0, 18.1, 19.0, 19.1]
FA = {16: (0, 5), 17: (5, 10), 18: (10, 15), 19: (15, 24), 200: (24, 28)}
FB = {16: (0, 2), 17: (2, 4), 18: (4, 6), 19: (6, 8)}
NITER = NSEG // 2
EPS = 1e-5
SCALE = DH ** (-0.5)


def _pair_heads(gp):
    half, r = divmod(gp, 8)
    par, i = divmod(r, 4)
    h0 = 16 * half + 4 * i + par
    return h0, h0 + 2


def _ln(xf):
    m = jnp.mean(xf, axis=-1, keepdims=True)
    xc = xf - m
    v = jnp.mean(xc * xc, axis=-1, keepdims=True)
    return xc * jax.lax.rsqrt(v + EPS)


def _dot(a, b):
    return jnp.dot(a, b, preferred_element_type=F32)


def _dot_nt(a, b):
    return jax.lax.dot_general(a, b, (((1,), (1,)), ((), ())), preferred_element_type=F32)


def _pack(xf):
    return pltpu.bitcast(xf.astype(BF16), U32)


def _unpack(u):
    return pltpu.bitcast(u, BF16)


def _kernel(x_hbm, mem0_hbm, wq_hbm, wk_hbm, wv_hbm, wo_hbm, w1_hbm, b1_hbm, w2_hbm, b2_hbm,
            c_hbm, wmod_hbm,
            out_hbm,
            x_v, out_v, stage, wqkv, wo_v, w1_v, w2_v, wm0_v, wm1_v,
            mem0_v, b1_v, b2_v, c_v,
            mod_v, modq_v, sc_v, bias_v, xh_v, h3_v, acc_v, qkv3, code_v,
            lhs_v, qkv_s, p_s, s_s, e_s, wacc, obuf, o3a, att_v, x1_v, h2_v, g_v, zero_s,
            sem_small, sem_x, sem_q, sem_stage, sem_w, sem_out):
    w_hbms = (wq_hbm, wk_hbm, wv_hbm)

    def mo(i, n):
        return i if isinstance(i, int) else pl.multiple_of(i, n)

    def small_copies():
        return [pltpu.make_async_copy(c_hbm, c_v, sem_small.at[0]),
                pltpu.make_async_copy(mem0_hbm, mem0_v, sem_small.at[1]),
                pltpu.make_async_copy(b1_hbm, b1_v, sem_small.at[2]),
                pltpu.make_async_copy(b2_hbm, b2_v, sem_small.at[3])]

    def x_copy(part):
        s0, ns, lo, n = [(0, NSEG, 24, 8), (0, XA, 0, 24), (XA, NSEG - XA, 0, 24)][part]
        return pltpu.make_async_copy(x_hbm.at[pl.ds(s0, ns), pl.ds(lo, n), :],
                                     x_v.at[pl.ds(s0, ns), pl.ds(lo, n), :], sem_x.at[part])

    def wq_chunk_copy(j, sem):
        d0 = mo((j >> 1) * 128, 128)
        hf = j & 1
        return pltpu.make_async_copy(wq_hbm.at[pl.ds(d0, 128), pl.ds(mo(16 * hf, 16), 16), :],
                                     stage.at[hf, pl.ds(d0, 128)], sem)

    def wm0_copy(i, sem):
        c0 = mo((i & 1) * D + (i >> 1) * 128, 128)
        return pltpu.make_async_copy(wmod_hbm.at[:, pl.ds(c0, 128)], wm0_v.at[i], sem)

    def g2_piece_copy(j, sem):
        d0 = mo(j * 64, 64)
        return pltpu.make_async_copy(wk_hbm.at[pl.ds(d0, 64), pl.ds(0, 16), :],
                                     stage.at[2, pl.ds(d0, 64)], sem)

    def group_copy(grp):
        mat, half = divmod(grp, 2)
        return pltpu.make_async_copy(w_hbms[mat].at[:, pl.ds(16 * half, 16), :],
                                     stage.at[grp % NSTAGE], sem_stage.at[grp])

    def slab_copies(src, c0, dst, sem):
        return [pltpu.make_async_copy(src.at[:, pl.ds(c0 + j * 128, 128)], dst.at[j], sem)
                for j in range(dst.shape[0])]

    wo_copies = lambda: slab_copies(wo_hbm, 0, wo_v, sem_w.at[0])
    wm1_copies = lambda: slab_copies(wmod_hbm, 2 * D, wm1_v, sem_w.at[1])
    w1_copies = lambda: slab_copies(w1_hbm, 0, w1_v, sem_w.at[2])
    w2_copies = lambda: slab_copies(w2_hbm, 0, w2_v, sem_w.at[3])

    def wcol(ref, j):
        return _unpack(ref.bitcast(U32)[j])

    def relayout(src, dst, j0, j1):
        srcu = src.bitcast(U32)
        for j in range(j0, j1):
            a = srcu[2 * j]
            b = srcu[2 * j + 1]
            dst[pl.ds(j, 8, stride=PITCH), :] = (a & jnp.uint32(0xFFFF)) | (b << 16)
            dst[pl.ds(8 * PITCH + j, 8, stride=PITCH), :] = (a >> 16) | (b & jnp.uint32(0xFFFF0000))

    def wpair(ref, slab0, n=D // 2):
        return jnp.concatenate([_unpack(ref[pl.ds(slab0 * PITCH, n), :]),
                                _unpack(ref[pl.ds((slab0 + 1) * PITCH, n), :])], axis=1)

    def modrow(i):
        return mod_v[0:1, i * D:(i + 1) * D]

    def first_copies():
        return [wm0_copy(i, sem_q.at[16]) for i in range(2)] + [wq_chunk_copy(0, sem_q.at[16])]

    def q_copies(j, do):
        do(g2_piece_copy(j, sem_q.at[j]))

        @pl.when(j < 15)
        def _():
            do(wq_chunk_copy(j + 1, sem_q.at[j]))

        @pl.when(j < 14)
        def _():
            do(wm0_copy(j + 2, sem_q.at[j]))

    def issue(i, carry):
        @pl.when(i == 0)
        def _():
            for cp in small_copies():
                cp.start()
            x_copy(0).start()

        @pl.when(i == 1)
        def _():
            for cp in first_copies():
                cp.start()

        @pl.when(jnp.logical_and(i >= 2, i < 18))
        def _():
            q_copies(i - 2, lambda cp: cp.start())

        @pl.when(i == 18)
        def _():
            group_copy(3).start()
            x_copy(1).start()
        return carry

    jax.lax.fori_loop(0, 19, issue, 0)
    zero_s[0] = 0

    ri = jax.lax.broadcasted_iota(jnp.int32, (80, 128), 0)
    ci = jax.lax.broadcasted_iota(jnp.int32, (80, 128), 1)

    def head_of(i):
        return jnp.where(i < 64, i // 32, (i - 64) // 8)

    def pos_of(i):
        return jnp.where(i < 64, i % 32, 32 + (i - 64) % 8)

    same = head_of(ri) == head_of(ci)
    pr, pc = pos_of(ri), pos_of(ci)
    keep = jnp.logical_or(pr < M, pr >= pc)
    code_v[...] = jnp.where(same, jnp.where(keep, 0.0, -1e9), -jnp.inf).astype(F32)

    for cp in small_copies():
        cp.wait()
    cf = c_v[...].astype(F32)
    sc_v[...] = _pack(jnp.broadcast_to(cf * jax.nn.sigmoid(cf), (16, D)))
    bias_v[:, 0:FF] = jnp.broadcast_to(b1_v[...].astype(F32).reshape(1, FF), (8, FF))
    bias_v[:, FF:] = jnp.broadcast_to(b2_v[...].astype(F32).reshape(1, D), (8, D))

    x_copy(0).wait()

    def xh_body(i, carry):
        for h in range(XHU):
            s0 = pl.multiple_of((i * XHU + h) * 8, 8)
            xh = _ln(x_v[pl.ds(s0, 8), 24:32, :].astype(F32).reshape(64, D))
            r0 = pl.multiple_of((i * XHU + h) * 64, 64)
            for kt in range(8):
                xh_v[kt, pl.ds(r0, 64), :] = xh[:, kt * 128:(kt + 1) * 128]
        return carry

    jax.lax.fori_loop(0, 8 // XHU, xh_body, 0)

    def mod_slab(i):
        modq_v[i] = _dot(_unpack(sc_v[...]), wcol(wm0_v, i))[0:8]

    def h3_store(dst, kt, mc):
        sa = modq_v[2 * kt, 0:1, :]
        ca = modq_v[2 * kt + 1, 0:1, :]
        dst[:, mc * 128:(mc + 1) * 128] = _pack(
            xh_v[kt, mc * 128:(mc + 1) * 128, :] * (1.0 + ca) + sa)

    for cp in first_copies():
        cp.wait()
    modq_v[2:16] = jnp.zeros((14, 8, 128), F32)
    for i in range(2):
        mod_slab(i)
    for mc in range(4):
        h3_store(h3_v.at[0], 0, mc)
    relayout(stage.at[0], wqkv, 0, 64)

    def q_body(j, carry):
        q_copies(j, lambda cp: cp.wait())
        kt, hf = j >> 1, j & 1
        jn = jnp.minimum(j + 1, 15)
        ktn, hfn = jn >> 1, jn & 1
        hview = h3_v.at[pl.ds(kt, 2)]
        wview = wqkv.at[pl.ds(pl.multiple_of(hf * (16 * PITCH) + kt * 64, 8), 16 * PITCH - 448), :]
        aview = acc_v.at[pl.ds(pl.multiple_of(hf * 8, 8), 8)]
        qsrc = stage.at[hfn, pl.ds(pl.multiple_of(ktn * 128, 128), 128)]
        qdst = wqkv.at[pl.ds(pl.multiple_of(hfn * (16 * PITCH) + ktn * 64, 8), 16 * PITCH - 448), :]
        ksrc = stage.at[2, pl.ds(pl.multiple_of(j * 64, 64), 64)]
        kdst = wqkv.at[pl.ds(pl.multiple_of(32 * PITCH + j * 32, 8), 16 * PITCH - 480), :]
        for p in range(8):
            lhs = jnp.concatenate([hview[0, :, mc * 128:(mc + 1) * 128] for mc in range(4)], axis=0)
            y = _dot(_unpack(lhs), wpair(wview, 2 * p, 64))
            aview[p] = jnp.where(kt > 0, aview[p], 0.0) + y
            if p == 1:
                mod_slab(jnp.minimum(j + 2, 15))
            if p >= 4:
                h3_store(hview.at[1], jnp.minimum(kt + 1, 7), p - 4)
            if p % 2 == 1:
                relayout(qsrc, qdst, 8 * p - 8, 8 * p + 8)
                relayout(ksrc, kdst, 4 * p - 4, 4 * p + 4)
        return carry

    jax.lax.fori_loop(0, 16, q_body, 0)
    for kt in range(8):
        mod_v[:, kt * 128:(kt + 1) * 128] = modq_v[2 * kt]
        mod_v[:, D + kt * 128:D + (kt + 1) * 128] = modq_v[2 * kt + 1]
    if STOP == 1:
        group_copy(3).wait()
        x_copy(1).wait()
        return

    def ln1(xb):
        return _ln(xb.astype(F32)) * (1.0 + modrow(1)) + modrow(0)

    def store_x3(dst, half, mc, y):
        y = y.reshape(16, 8, 256)
        y = jnp.concatenate([y[:, :, :128], y[:, :, 128:]], axis=1).reshape(256, DH)
        dst[mc * 128:(mc + 1) * 128, half * DH:(half + 1) * DH] = _pack(y)

    def unit_body(u, carry):
        gn = jnp.minimum((u >> 1) + 1, 5)
        slot = stage.at[gn & (NSTAGE - 1)]

        @pl.when(jnp.logical_and(u & 1 == 0, u < 10))
        def _():
            pltpu.make_async_copy(slot, slot, sem_stage.at[gn]).wait()

        for k, cps in enumerate([lambda: [group_copy(4), group_copy(5)], wo_copies, wm1_copies,
                                 w1_copies, w2_copies, lambda: [x_copy(2)]]):
            @pl.when(u == 4 + k)
            def _(cps=cps):
                for cp in cps():
                    cp.start()

        src = slot.at[pl.ds(pl.multiple_of((u & 1) * 512, 512), 512)]
        dst = wqkv.at[pl.ds(pl.multiple_of(gn * (16 * PITCH) + (u & 1) * 256, 8), 16 * PITCH - 256), :]
        view = wqkv.at[pl.ds(pl.multiple_of(u * (8 * PITCH), 8), 8 * PITCH), :]
        for p in range(4):
            for mc in range(4):
                lhs = _unpack(jnp.concatenate(
                    [h3_v[kt, :, mc * 128:(mc + 1) * 128] for kt in range(8)], axis=1))
                store_x3(qkv3.at[2 * u + p // 2], p % 2, mc, _dot(lhs, wpair(view, 2 * p)))
                relayout(src, dst, 16 * (4 * p + mc), 16 * (4 * p + mc + 1))
                if p % 2 == 0:
                    store_x3(qkv3.at[u - 4], p // 2, mc,
                             acc_v[2 * (u - 4) + p // 2, mc * 128:(mc + 1) * 128, :])
        return carry

    jax.lax.fori_loop(4, 12, unit_body, 0)

    x_copy(1).wait()
    for cp in wo_copies() + wm1_copies():
        cp.wait()
    if STOP == 2:
        for cp in w1_copies() + w2_copies() + [x_copy(2)]:
            cp.wait()
        return

    def mod_rest(i):
        def run():
            for j in range(4 * i, 4 * i + 4):
                mod_v[:, 2 * D + j * 128:2 * D + (j + 1) * 128] = _dot(
                    _unpack(sc_v[...]), wcol(wm1_v, j))[0:8]
        return run

    lhs_v[...] = _pack(jnp.concatenate([mem0_v[...].astype(F32), ln1(x_v[0, 0:24, :])], axis=0))

    zpad = jnp.zeros((24, DH), U32)

    def proj(g, mat):
        y = _dot(_unpack(lhs_v[...]), wpair(wqkv, mat * H + 2 * g))
        cs = pl.ds((g * 3 + mat) * DH, DH)
        qkv_s[0:16, cs] = _pack(y[:, :DH])
        qkv_s[16:32, cs] = _pack(y[:, DH:])

    def proj4(gg, mat):
        y = None
        for kt in range(0, 8, KSTEP):
            w = jnp.concatenate(
                [_unpack(wqkv[pl.ds((mat * H + 4 * gg + i) * PITCH + 64 * kt, 64 * KSTEP), :])
                 for i in range(4)], axis=1)
            d = _dot(_unpack(lhs_v[:, kt * 128:(kt + KSTEP) * 128]), w)
            y = d if y is None else y + d
        for i in range(4):
            cs = pl.ds(((2 * gg + i // 2) * 3 + mat) * DH, DH)
            qkv_s[16 * (i % 2):16 * (i % 2 + 1), cs] = _pack(y[:, i * DH:(i + 1) * DH])

    def get(g, mat, seg):
        u3, p3 = divmod(mat * NPAIR + g, 2)
        parts = [qkv_s[:, pl.ds((g * 3 + mat) * DH, DH)],
                 qkv3[u3, pl.ds(mo(seg * 8, 8), 8), p3 * DH:(p3 + 1) * DH]]
        if mat > 0:
            parts.append(zpad)
        return _unpack(jnp.concatenate(parts, axis=0))

    def scores(g, q, k):
        cs = pl.ds(g * DH, DH)
        s = _dot_nt(q, k) * SCALE
        code = code_v[...]
        s = jnp.where(code == 0.0, s, code)
        m = jnp.max(s, axis=-1, keepdims=True)
        if SSCR & 1:
            s_s[:, cs] = s
            s = s_s[:, cs]
        e = jnp.exp(s - m)
        l = jnp.sum(e, axis=-1, keepdims=True)
        if SSCR & 2:
            e_s[:, cs] = e
            e = e_s[:, cs]
        r = pl.reciprocal(l, approx=True)
        if NEWTON:
            r = r * (2.0 - l * r)
        return (e * r).astype(BF16)

    def pv(g, p, v, second):
        o = _dot(p, v)
        c0, c1 = (h * DH for h in _pair_heads(g))
        obuf[0:16, c0:c0 + DH] = _pack(o[0:32])
        obuf[0:16, c1:c1 + DH] = _pack(o[32:64])
        if not second:
            o3a[:, c0:c0 + DH] = o[64:72]
            o3a[:, c1:c1 + DH] = o[72:80]
        else:
            obuf[16:24, c0:c0 + DH] = _pack(jnp.concatenate([o3a[:, c0:c0 + DH], o[64:72]], axis=0))
            obuf[16:24, c1:c1 + DH] = _pack(jnp.concatenate([o3a[:, c1:c1 + DH], o[72:80]], axis=0))

    def wo_cols(pairs):
        return sorted(h for g in pairs for h in _pair_heads(g))

    def wo_dot(j, heads, nrow):
        lhs = jnp.concatenate([obuf[0:nrow, h * DH:(h + 1) * DH] for h in heads], axis=1)
        w = jnp.concatenate([wo_v.bitcast(U32)[j, h * 64:(h + 1) * 64, :] for h in heads], axis=0)
        return _dot(_unpack(lhs), _unpack(w))

    def step(seg, second, fillers, wsplit):
        nrow = 24 if second else 16
        early, late = wo_cols(range(NPAIR - wsplit)), wo_cols(range(NPAIR - wsplit, NPAIR))

        def do_scores(g):
            p_s[:, pl.ds(g * DH, DH)] = pltpu.bitcast(scores(g, get(g, 0, seg), get(g, 1, seg)), U32)

        def do_pv(g):
            pv(g, _unpack(p_s[:, pl.ds(g * DH, DH)]), get(g, 2, seg), second)

        def wo_early(j):
            wacc[0:2 * nrow, j * 128:(j + 1) * 128] = wo_dot(j, early, nrow)

        def wo_final(j):
            cs = slice(j * 128, (j + 1) * 128)
            if wsplit:
                y = wacc[0:2 * nrow, cs] + wo_dot(j, late, nrow)
            else:
                y = wo_dot(j, early, nrow)
            r0 = 32 if second else 56
            hn = pltpu.bitcast(obuf[r0:r0 + 24, cs], F32)
            lhs_v[:, cs] = _pack(jnp.concatenate([y[0:8], hn], axis=0))
            if not second:
                att_v[0:24, cs] = y[8:32]
            else:
                att_v[32:56, cs] = y[8:32]
                att_v[24:32, cs] = y[32:40]
                att_v[56:64, cs] = y[40:48]

        ev = []
        for g in range(NPAIR):
            if not KMAJOR:
                ev.append((g + QOFF, functools.partial(proj, g, 0)))
                ev.append((g + KOFF, functools.partial(proj, g, 1)))
                ev.append((g + VOFF, functools.partial(proj, g, 2)))
            elif g % 2 == 0:
                ev.append((g, functools.partial(proj4, g // 2, 0)))
                ev.append((g + 0.66, functools.partial(proj4, g // 2, 1)))
                ev.append((g + 1.33, functools.partial(proj4, g // 2, 2)))
            ev.append((g + SOFF, functools.partial(do_scores, g)))
            ev.append((g + POFF, functools.partial(do_pv, g)))
        if wsplit:
            for j in range(8):
                ev.append((WEARLY[j], functools.partial(wo_early, j)))
        for j in range(8):
            ev.append((100 + j, functools.partial(wo_final, j)))
        ev.extend(fillers.items())
        ev.sort(key=lambda e: e[0])
        for _, f in ev:
            f()

    def ffn_pre(tp):
        xb = x_v[pl.ds(2 * tp, 2)].astype(F32).reshape(64, D)
        x1 = xb + modrow(2) * att_v[...]
        x1_v[...] = x1
        h2_v[0:32, :] = _pack(_ln(x1) * (1.0 + modrow(4)) + modrow(3))

    def ffn1(lo, hi):
        def run():
            for j in range(lo, hi):
                cs = slice(j * 128, (j + 1) * 128)
                y = _dot(_unpack(h2_v[0:32, :]), wcol(w1_v, j)) + bias_v[0:1, cs]
                g_v[0:32, cs] = _pack(jax.nn.gelu(y, approximate=True))
        return run

    def ffn2(tp, lo, hi):
        def run():
            for j in range(lo, hi):
                cs = slice(j * 128, (j + 1) * 128)
                y = _dot(_unpack(g_v[0:32, :]), wcol(w2_v, j)) + bias_v[0:1, FF + j * 128:FF + (j + 1) * 128]
                o = x1_v[:, cs] + mod_v[0:1, 5 * D + j * 128:5 * D + (j + 1) * 128] * y
                out_v[tp, :, cs] = o.astype(BF16)
        return run

    def out_copy(tp):
        return pltpu.make_async_copy(out_v.at[tp], out_hbm.at[tp], sem_out.at[0])

    def next_rows(r0, seg):
        def run():
            z = pl.multiple_of(zero_s[0], 8) if PIN else 0
            obuf[pl.ds(r0 + z, 24), 0:D] = pltpu.bitcast(ln1(x_v[seg, 0:24, :]), U32)
        return run

    def double_step(t, with_ffn):
        if with_ffn:
            ffn_pre(t - 1)
            fa = {k: ffn1(a, b) for k, (a, b) in FA.items()}
            fb = {k: ffn2(t - 1, a, b) for k, (a, b) in FB.items()}
            fb.update({k: ffn1(a, b) for k, (a, b) in FB1.items()})
        else:
            fa = {NPAIR + k: mod_rest(k) for k in range(4)}
            fb = {NPAIR + k: mod_rest(4 + k) for k in range(4)}
        if AHEAD:
            fb[HNA] = next_rows(56, jnp.minimum(2 * t + 3, NSEG - 1))
            if not with_ffn:
                fa[HNA] = next_rows(56, 1)
        else:
            fa[HNA] = next_rows(56, 2 * t + 1)
        fb[HNB] = next_rows(32, jnp.minimum(2 * t + 2, NSEG - 1))
        step(2 * t, False, fa, WSPLIT if with_ffn else WSPLIT0)
        step(2 * t + 1, True, fb, WSPLIT if with_ffn else WSPLIT0)
        if with_ffn:
            out_copy(t - 1).start()

    double_step(0, False)
    for cp in w1_copies() + w2_copies():
        cp.wait()
    if STOP == 3:
        x_copy(2).wait()
        return

    def body(t, carry):
        @pl.when(t == 2)
        def _():
            x_copy(2).wait()
        double_step(t, True)
        return carry

    jax.lax.fori_loop(1, NITER, body, 0)

    last = NITER - 1
    ffn_pre(last)
    ffn1(0, FF // 128)()
    ffn2(last, 0, 8)()
    out_copy(last).start()
    pltpu.make_async_copy(out_v.at[0:NITER], out_hbm.at[0:NITER], sem_out.at[0]).wait()


@functools.partial(jax.jit, static_argnames=("A_seg_len",))
def pallas_adaLN_cond__memory_aug_recurrent_mem_tr__dense_activation_gelu__prompt_kernel(
    A_x, A_mem0, A_Wq, A_Wk, A_Wv, A_Wo, A_seg_len, B_x, B_w1, B_b1, B_w2, B_b2, c, w_mod,
):
    assert A_x.shape == (1, S, D) and A_mem0.shape == (1, M, D) and A_seg_len == SEG
    assert A_Wq.shape == (D, H, DH) and B_w1.shape == (D, FF)
    any_spec = pl.BlockSpec(memory_space=pl.ANY)
    scratch = [
        pltpu.VMEM((NSEG, SEG, D), BF16),
        pltpu.VMEM((NSEG // 2, 2 * SEG, D), BF16),
        pltpu.VMEM((NSTAGE, D, 16, DH), BF16),
        pltpu.VMEM((3 * H * PITCH, DH), U32),
        pltpu.VMEM((8, H * DH, 128), BF16),
        pltpu.VMEM((FF // 128, D, 128), BF16),
        pltpu.VMEM((8, FF, 128), BF16),
        pltpu.VMEM((16, D, 128), BF16),
        pltpu.VMEM((32, D, 128), BF16),
        pltpu.VMEM((M, D), BF16),
        pltpu.VMEM((FF,), BF16),
        pltpu.VMEM((D,), BF16),
        pltpu.VMEM((1, D), BF16),
        pltpu.VMEM((8, 6 * D), F32),
        pltpu.VMEM((16, 8, 128), F32),
        pltpu.VMEM((8, D), U32),
        pltpu.VMEM((8, FF + D), F32),
        pltpu.VMEM((8, NSEG * 8, 128), F32),
        pltpu.VMEM((9, 64, 512), U32),
        pltpu.VMEM((NPAIR, NSEG * 8, 2 * DH), F32),
        pltpu.VMEM((24, NSEG * 8, 2 * DH), U32),
        pltpu.VMEM((80, 128), F32),
        pltpu.VMEM((16, D), U32),
        pltpu.VMEM((32, NPAIR * 3 * DH), U32),
        pltpu.VMEM((40, NPAIR * DH), U32),
        pltpu.VMEM((80, NPAIR * DH), F32),
        pltpu.VMEM((80, NPAIR * DH), F32),
        pltpu.VMEM((48, D), F32),
        pltpu.VMEM((80, H * DH), U32),
        pltpu.VMEM((8, H * DH), F32),
        pltpu.VMEM((64, D), F32),
        pltpu.VMEM((64, D), F32),
        pltpu.VMEM((32, D), U32),
        pltpu.VMEM((32, FF), U32),
        pltpu.SMEM((1,), jnp.int32),
        pltpu.SemaphoreType.DMA((4,)),
        pltpu.SemaphoreType.DMA((3,)),
        pltpu.SemaphoreType.DMA((17,)),
        pltpu.SemaphoreType.DMA((6,)),
        pltpu.SemaphoreType.DMA((4,)),
        pltpu.SemaphoreType.DMA((1,)),
    ]
    out = pl.pallas_call(
        _kernel,
        out_shape=jax.ShapeDtypeStruct((NSEG // 2, 2 * SEG, D), BF16),
        in_specs=[any_spec] * 12,
        out_specs=any_spec,
        scratch_shapes=scratch,
        compiler_params=pltpu.CompilerParams(vmem_limit_bytes=120 * 1024 * 1024,
                                             disable_bounds_checks=True),
    )(
        A_x.reshape(NSEG, SEG, D), A_mem0.reshape(M, D), A_Wq, A_Wk, A_Wv,
        A_Wo.reshape(H * DH, D), B_w1, B_b1, B_w2, B_b2,
        c, w_mod,
    )
    return out.reshape(1, S, D)
```

```python
import functools

import jax
import jax.numpy as jnp
import jax.experimental.pallas as pl
import jax.experimental.pallas.tpu as pltpu

F32 = jnp.float32
BF16 = jnp.bfloat16
U32 = jnp.uint32

S = 2048
D = 1024
H = 32
DH = 128
M = 8
SEG = 32
NSEG = S // SEG
FF = 3584
NPAIR = H // 2
PITCH = 516
XA = 8
NSTAGE = 4
STOP = 0
XHU = 2
QOFF, KOFF, VOFF, SOFF, POFF = 0.0, 0.1, 0.2, 1.5, 3.6
SSCR = 0
NEWTON = 1
KMAJOR = 1
KSTEP = 2
PIN = 1
HN0 = 10
MODMC = 1
HNA = 17.9
HNB = 18.9
FB1 = {}
WSPLIT = 0
WSPLIT0 = 4
WEARLY = [16.0, 16.1, 17.0, 17.1, 18.0, 18.1, 19.0, 19.1]
FA = {16: (0, 5), 17: (5, 10), 18: (10, 15), 19: (15, 24), 200: (24, 28)}
FB = {16: (0, 2), 17: (2, 4), 18: (4, 6), 19: (6, 8)}
NITER = NSEG // 2
EPS = 1e-5
SCALE = DH ** (-0.5)


def _pair_heads(gp):
    half, r = divmod(gp, 8)
    par, i = divmod(r, 4)
    h0 = 16 * half + 4 * i + par
    return h0, h0 + 2


def _ln(xf):
    m = jnp.mean(xf, axis=-1, keepdims=True)
    xc = xf - m
    v = jnp.mean(xc * xc, axis=-1, keepdims=True)
    return xc * jax.lax.rsqrt(v + EPS)


def _dot(a, b):
    return jnp.dot(a, b, preferred_element_type=F32)


def _dot_nt(a, b):
    return jax.lax.dot_general(a, b, (((1,), (1,)), ((), ())), preferred_element_type=F32)


def _pack(xf):
    return pltpu.bitcast(xf.astype(BF16), U32)


def _unpack(u):
    return pltpu.bitcast(u, BF16)


def _kernel(x_hbm, mem0_hbm, wq_hbm, wk_hbm, wv_hbm, wo_hbm, w1_hbm, b1_hbm, w2_hbm, b2_hbm,
            c_hbm, wmod_hbm,
            out_hbm,
            x_v, out_v, stage, wqkv, wo_v, w1_v, w2_v, wm0_v, wm1_v,
            mem0_v, b1_v, b2_v, c_v,
            mod_v, modq_v, modr_v, sc_v, bias_v, xh_v, h3_v, acc_v, qkv3, code_v,
            lhs_v, qkv_s, p_s, s_s, e_s, wacc, obuf, o3a, att_v, x1_v, h2_v, g_v, zero_s,
            sem_small, sem_x, sem_q, sem_u, sem_w, sem_out):
    w_hbms = (wq_hbm, wk_hbm, wv_hbm)

    def mo(i, n):
        return i if isinstance(i, int) else pl.multiple_of(i, n)

    def small_copies():
        return [pltpu.make_async_copy(c_hbm, c_v, sem_small.at[0]),
                pltpu.make_async_copy(mem0_hbm, mem0_v, sem_small.at[1]),
                pltpu.make_async_copy(b1_hbm, b1_v, sem_small.at[2]),
                pltpu.make_async_copy(b2_hbm, b2_v, sem_small.at[3])]

    def x_copy(part):
        s0, ns, lo, n = [(0, NSEG, 24, 8), (0, XA, 0, 24), (XA, NSEG - XA, 0, 24)][part]
        return pltpu.make_async_copy(x_hbm.at[pl.ds(s0, ns), pl.ds(lo, n), :],
                                     x_v.at[pl.ds(s0, ns), pl.ds(lo, n), :], sem_x.at[part])

    def wq_chunk_copy(j, sem):
        d0 = mo((j >> 1) * 128, 128)
        hf = j & 1
        return pltpu.make_async_copy(wq_hbm.at[pl.ds(d0, 128), pl.ds(mo(16 * hf, 16), 16), :],
                                     stage.at[hf, pl.ds(d0, 128)], sem)

    def wm0_copy(i, sem):
        c0 = mo((i & 1) * D + (i >> 1) * 128, 128)
        return pltpu.make_async_copy(wmod_hbm.at[:, pl.ds(c0, 128)], wm0_v.at[i], sem)

    def g2_piece_copy(j, sem):
        d0 = mo(j * 64, 64)
        return pltpu.make_async_copy(wk_hbm.at[pl.ds(d0, 64), pl.ds(0, 16), :],
                                     stage.at[2, pl.ds(d0, 64)], sem)

    def unit_copies(u):
        cps = [pltpu.make_async_copy(wmod_hbm.at[:, pl.ds(2 * D + j * 128, 128)], wm1_v.at[j],
                                     sem_u.at[u - 4]) for j in range(4 * (u - 4), 4 * (u - 3))]
        if u < 10:
            grp = u // 2 + 1
            mat, half = divmod(grp, 2)
            rows = pl.ds((u % 2) * 512, 512)
            cps.append(pltpu.make_async_copy(w_hbms[mat].at[rows, pl.ds(16 * half, 16), :],
                                             stage.at[grp % NSTAGE, rows], sem_u.at[u - 4]))
        return cps

    def slab_copies(src, c0, dst, sem):
        return [pltpu.make_async_copy(src.at[:, pl.ds(c0 + j * 128, 128)], dst.at[j], sem)
                for j in range(dst.shape[0])]

    wo_copies = lambda: slab_copies(wo_hbm, 0, wo_v, sem_w.at[0])
    w1_copies = lambda: slab_copies(w1_hbm, 0, w1_v, sem_w.at[2])
    w2_copies = lambda: slab_copies(w2_hbm, 0, w2_v, sem_w.at[3])

    def wcol(ref, j):
        return _unpack(ref.bitcast(U32)[j])

    def relayout(src, dst, j0, j1):
        srcu = src.bitcast(U32)
        for j in range(j0, j1):
            a = srcu[2 * j]
            b = srcu[2 * j + 1]
            dst[pl.ds(j, 8, stride=PITCH), :] = (a & jnp.uint32(0xFFFF)) | (b << 16)
            dst[pl.ds(8 * PITCH + j, 8, stride=PITCH), :] = (a >> 16) | (b & jnp.uint32(0xFFFF0000))

    def wpair(ref, slab0, n=D // 2):
        return jnp.concatenate([_unpack(ref[pl.ds(slab0 * PITCH, n), :]),
                                _unpack(ref[pl.ds((slab0 + 1) * PITCH, n), :])], axis=1)

    def modrow(i):
        return mod_v[0:1, i * D:(i + 1) * D]

    def first_copies():
        return [wm0_copy(i, sem_q.at[16]) for i in range(2)] + [wq_chunk_copy(0, sem_q.at[16])]

    def q_copies(j, do):
        do(g2_piece_copy(j, sem_q.at[j]))

        @pl.when(j < 15)
        def _():
            do(wq_chunk_copy(j + 1, sem_q.at[j]))

        @pl.when(j < 14)
        def _():
            do(wm0_copy(j + 2, sem_q.at[j]))

    def issue(i, carry):
        @pl.when(i == 0)
        def _():
            for cp in small_copies():
                cp.start()
            x_copy(0).start()

        @pl.when(i == 1)
        def _():
            for cp in first_copies():
                cp.start()

        @pl.when(jnp.logical_and(i >= 2, i < 18))
        def _():
            q_copies(i - 2, lambda cp: cp.start())

        @pl.when(i == 18)
        def _():
            for cp in unit_copies(4) + [x_copy(1)]:
                cp.start()

        @pl.when(i == 19)
        def _():
            for cp in unit_copies(5):
                cp.start()
        return carry

    jax.lax.fori_loop(0, 20, issue, 0)
    zero_s[0] = 0

    ri = jax.lax.broadcasted_iota(jnp.int32, (80, 128), 0)
    ci = jax.lax.broadcasted_iota(jnp.int32, (80, 128), 1)

    def head_of(i):
        return jnp.where(i < 64, i // 32, (i - 64) // 8)

    def pos_of(i):
        return jnp.where(i < 64, i % 32, 32 + (i - 64) % 8)

    same = head_of(ri) == head_of(ci)
    pr, pc = pos_of(ri), pos_of(ci)
    keep = jnp.logical_or(pr < M, pr >= pc)
    code_v[...] = jnp.where(same, jnp.where(keep, 0.0, -1e9), -jnp.inf).astype(F32)

    for cp in small_copies():
        cp.wait()
    cf = c_v[...].astype(F32)
    sc_v[...] = _pack(jnp.broadcast_to(cf * jax.nn.sigmoid(cf), (16, D)))
    bias_v[:, 0:FF] = jnp.broadcast_to(b1_v[...].astype(F32).reshape(1, FF), (8, FF))
    bias_v[:, FF:] = jnp.broadcast_to(b2_v[...].astype(F32).reshape(1, D), (8, D))

    x_copy(0).wait()

    def xh_body(i, carry):
        for h in range(XHU):
            s0 = pl.multiple_of((i * XHU + h) * 8, 8)
            xh = _ln(x_v[pl.ds(s0, 8), 24:32, :].astype(F32).reshape(64, D))
            r0 = pl.multiple_of((i * XHU + h) * 64, 64)
            for kt in range(8):
                xh_v[kt, pl.ds(r0, 64), :] = xh[:, kt * 128:(kt + 1) * 128]
        return carry

    jax.lax.fori_loop(0, 8 // XHU, xh_body, 0)

    def mod_slab(i):
        modq_v[i] = _dot(_unpack(sc_v[...]), wcol(wm0_v, i))[0:8]

    def h3_store(dst, kt, mc):
        sa = modq_v[2 * kt, 0:1, :]
        ca = modq_v[2 * kt + 1, 0:1, :]
        dst[:, mc * 128:(mc + 1) * 128] = _pack(
            xh_v[kt, mc * 128:(mc + 1) * 128, :] * (1.0 + ca) + sa)

    for cp in first_copies():
        cp.wait()
    modq_v[2:16] = jnp.zeros((14, 8, 128), F32)
    for i in range(2):
        mod_slab(i)
    for mc in range(4):
        h3_store(h3_v.at[0], 0, mc)
    relayout(stage.at[0], wqkv, 0, 64)

    def q_body(j, carry):
        q_copies(j, lambda cp: cp.wait())
        kt, hf = j >> 1, j & 1
        jn = jnp.minimum(j + 1, 15)
        ktn, hfn = jn >> 1, jn & 1
        hview = h3_v.at[pl.ds(kt, 2)]
        wview = wqkv.at[pl.ds(pl.multiple_of(hf * (16 * PITCH) + kt * 64, 8), 16 * PITCH - 448), :]
        aview = acc_v.at[pl.ds(pl.multiple_of(hf * 8, 8), 8)]
        qsrc = stage.at[hfn, pl.ds(pl.multiple_of(ktn * 128, 128), 128)]
        qdst = wqkv.at[pl.ds(pl.multiple_of(hfn * (16 * PITCH) + ktn * 64, 8), 16 * PITCH - 448), :]
        ksrc = stage.at[2, pl.ds(pl.multiple_of(j * 64, 64), 64)]
        kdst = wqkv.at[pl.ds(pl.multiple_of(32 * PITCH + j * 32, 8), 16 * PITCH - 480), :]
        for p in range(8):
            lhs = jnp.concatenate([hview[0, :, mc * 128:(mc + 1) * 128] for mc in range(4)], axis=0)
            y = _dot(_unpack(lhs), wpair(wview, 2 * p, 64))
            aview[p] = jnp.where(kt > 0, aview[p], 0.0) + y
            if p == 1:
                mod_slab(jnp.minimum(j + 2, 15))
            if p >= 4:
                h3_store(hview.at[1], jnp.minimum(kt + 1, 7), p - 4)
            if p % 2 == 1:
                relayout(qsrc, qdst, 8 * p - 8, 8 * p + 8)
                relayout(ksrc, kdst, 4 * p - 4, 4 * p + 4)
        return carry

    jax.lax.fori_loop(0, 16, q_body, 0)
    for kt in range(8):
        mod_v[:, kt * 128:(kt + 1) * 128] = modq_v[2 * kt]
        mod_v[:, D + kt * 128:D + (kt + 1) * 128] = modq_v[2 * kt + 1]
    for cp in unit_copies(6):
        cp.start()
    x_copy(1).wait()

    def ln1(xb):
        return _ln(xb.astype(F32)) * (1.0 + modrow(1)) + modrow(0)

    def store_x3(dst, half, mc, y):
        y = y.reshape(16, 8, 256)
        y = jnp.concatenate([y[:, :, :128], y[:, :, 128:]], axis=1).reshape(256, DH)
        dst[mc * 128:(mc + 1) * 128, half * DH:(half + 1) * DH] = _pack(y)

    def unit_body(u, carry):
        gn = jnp.minimum((u >> 1) + 1, 5)
        src = stage.at[gn & (NSTAGE - 1), pl.ds(pl.multiple_of((u & 1) * 512, 512), 512)]
        wm = wm1_v.at[pl.ds(4 * (u - 4), 4)]
        pltpu.make_async_copy(wm, wm, sem_u.at[u - 4]).wait()

        @pl.when(u < 10)
        def _():
            pltpu.make_async_copy(src, src, sem_u.at[u - 4]).wait()

        for k, cps in [(7, w1_copies), (4, lambda: unit_copies(7) + unit_copies(8)),
                       (5, lambda: unit_copies(9) + unit_copies(10) + unit_copies(11)),
                       (6, wo_copies), (8, w2_copies), (9, lambda: [x_copy(2)])]:
            @pl.when(u == k)
            def _(cps=cps):
                for cp in cps():
                    cp.start()

        lhs_v[...] = _pack(jnp.concatenate([mem0_v[...].astype(F32), ln1(x_v[0, 0:24, :])], axis=0))
        dst = wqkv.at[pl.ds(pl.multiple_of(gn * (16 * PITCH) + (u & 1) * 256, 8), 16 * PITCH - 256), :]
        view = wqkv.at[pl.ds(pl.multiple_of(u * (8 * PITCH), 8), 8 * PITCH), :]
        for p in range(4):
            for mc in range(4):
                lhs = _unpack(jnp.concatenate(
                    [h3_v[kt, :, mc * 128:(mc + 1) * 128] for kt in range(8)], axis=1))
                store_x3(qkv3.at[2 * u + p // 2], p % 2, mc, _dot(lhs, wpair(view, 2 * p)))
                relayout(src, dst, 16 * (4 * p + mc), 16 * (4 * p + mc + 1))
                if mc == MODMC:
                    modr_v[4 * (u - 4) + p] = _dot(_unpack(sc_v[...]), wcol(wm, p))[0:8]
                if p % 2 == 0:
                    store_x3(qkv3.at[u - 4], p // 2, mc,
                             acc_v[2 * (u - 4) + p // 2, mc * 128:(mc + 1) * 128, :])
        return carry

    jax.lax.fori_loop(4, 12, unit_body, 0)

    for cp in wo_copies():
        cp.wait()
    for j in range(32):
        mod_v[:, 2 * D + j * 128:2 * D + (j + 1) * 128] = modr_v[j]

    zpad = jnp.zeros((24, DH), U32)

    def proj(g, mat):
        y = _dot(_unpack(lhs_v[...]), wpair(wqkv, mat * H + 2 * g))
        cs = pl.ds((g * 3 + mat) * DH, DH)
        qkv_s[0:16, cs] = _pack(y[:, :DH])
        qkv_s[16:32, cs] = _pack(y[:, DH:])

    def proj4(gg, mat):
        y = None
        for kt in range(0, 8, KSTEP):
            w = jnp.concatenate(
                [_unpack(wqkv[pl.ds((mat * H + 4 * gg + i) * PITCH + 64 * kt, 64 * KSTEP), :])
                 for i in range(4)], axis=1)
            d = _dot(_unpack(lhs_v[:, kt * 128:(kt + KSTEP) * 128]), w)
            y = d if y is None else y + d
        for i in range(4):
            cs = pl.ds(((2 * gg + i // 2) * 3 + mat) * DH, DH)
            qkv_s[16 * (i % 2):16 * (i % 2 + 1), cs] = _pack(y[:, i * DH:(i + 1) * DH])

    def get(g, mat, seg):
        u3, p3 = divmod(mat * NPAIR + g, 2)
        parts = [qkv_s[:, pl.ds((g * 3 + mat) * DH, DH)],
                 qkv3[u3, pl.ds(mo(seg * 8, 8), 8), p3 * DH:(p3 + 1) * DH]]
        if mat > 0:
            parts.append(zpad)
        return _unpack(jnp.concatenate(parts, axis=0))

    def scores(g, q, k):
        cs = pl.ds(g * DH, DH)
        s = _dot_nt(q, k) * SCALE
        code = code_v[...]
        s = jnp.where(code == 0.0, s, code)
        m = jnp.max(s, axis=-1, keepdims=True)
        if SSCR & 1:
            s_s[:, cs] = s
            s = s_s[:, cs]
        e = jnp.exp(s - m)
        l = jnp.sum(e, axis=-1, keepdims=True)
        if SSCR & 2:
            e_s[:, cs] = e
            e = e_s[:, cs]
        r = pl.reciprocal(l, approx=True)
        if NEWTON:
            r = r * (2.0 - l * r)
        return (e * r).astype(BF16)

    def pv(g, p, v, second):
        o = _dot(p, v)
        c0, c1 = (h * DH for h in _pair_heads(g))
        obuf[0:16, c0:c0 + DH] = _pack(o[0:32])
        obuf[0:16, c1:c1 + DH] = _pack(o[32:64])
        if not second:
            o3a[:, c0:c0 + DH] = o[64:72]
            o3a[:, c1:c1 + DH] = o[72:80]
        else:
            obuf[16:24, c0:c0 + DH] = _pack(jnp.concatenate([o3a[:, c0:c0 + DH], o[64:72]], axis=0))
            obuf[16:24, c1:c1 + DH] = _pack(jnp.concatenate([o3a[:, c1:c1 + DH], o[72:80]], axis=0))

    def wo_cols(pairs):
        return sorted(h for g in pairs for h in _pair_heads(g))

    def wo_dot(j, heads, nrow):
        lhs = jnp.concatenate([obuf[0:nrow, h * DH:(h + 1) * DH] for h in heads], axis=1)
        w = jnp.concatenate([wo_v.bitcast(U32)[j, h * 64:(h + 1) * 64, :] for h in heads], axis=0)
        return _dot(_unpack(lhs), _unpack(w))

    def step(seg, second, fillers, wsplit):
        nrow = 24 if second else 16
        early, late = wo_cols(range(NPAIR - wsplit)), wo_cols(range(NPAIR - wsplit, NPAIR))

        def do_scores(g):
            p_s[:, pl.ds(g * DH, DH)] = pltpu.bitcast(scores(g, get(g, 0, seg), get(g, 1, seg)), U32)

        def do_pv(g):
            pv(g, _unpack(p_s[:, pl.ds(g * DH, DH)]), get(g, 2, seg), second)

        def wo_early(j):
            wacc[0:2 * nrow, j * 128:(j + 1) * 128] = wo_dot(j, early, nrow)

        def wo_final(j):
            cs = slice(j * 128, (j + 1) * 128)
            if wsplit:
                y = wacc[0:2 * nrow, cs] + wo_dot(j, late, nrow)
            else:
                y = wo_dot(j, early, nrow)
            r0 = 32 if second else 56
            hn = pltpu.bitcast(obuf[r0:r0 + 24, cs], F32)
            lhs_v[:, cs] = _pack(jnp.concatenate([y[0:8], hn], axis=0))
            if not second:
                att_v[0:24, cs] = y[8:32]
            else:
                att_v[32:56, cs] = y[8:32]
                att_v[24:32, cs] = y[32:40]
                att_v[56:64, cs] = y[40:48]

        ev = []
        for g in range(NPAIR):
            if not KMAJOR:
                ev.append((g + QOFF, functools.partial(proj, g, 0)))
                ev.append((g + KOFF, functools.partial(proj, g, 1)))
                ev.append((g + VOFF, functools.partial(proj, g, 2)))
            elif g % 2 == 0:
                ev.append((g, functools.partial(proj4, g // 2, 0)))
                ev.append((g + 0.66, functools.partial(proj4, g // 2, 1)))
                ev.append((g + 1.33, functools.partial(proj4, g // 2, 2)))
            ev.append((g + SOFF, functools.partial(do_scores, g)))
            ev.append((g + POFF, functools.partial(do_pv, g)))
        if wsplit:
            for j in range(8):
                ev.append((WEARLY[j], functools.partial(wo_early, j)))
        for j in range(8):
            ev.append((100 + j, functools.partial(wo_final, j)))
        ev.extend(fillers.items())
        ev.sort(key=lambda e: e[0])
        for _, f in ev:
            f()

    def ffn_pre(tp):
        xb = x_v[pl.ds(2 * tp, 2)].astype(F32).reshape(64, D)
        x1 = xb + modrow(2) * att_v[...]
        x1_v[...] = x1
        h2_v[0:32, :] = _pack(_ln(x1) * (1.0 + modrow(4)) + modrow(3))

    def ffn1(lo, hi):
        def run():
            for j in range(lo, hi):
                cs = slice(j * 128, (j + 1) * 128)
                y = _dot(_unpack(h2_v[0:32, :]), wcol(w1_v, j)) + bias_v[0:1, cs]
                g_v[0:32, cs] = _pack(jax.nn.gelu(y, approximate=True))
        return run

    def ffn2(tp, lo, hi):
        def run():
            for j in range(lo, hi):
                cs = slice(j * 128, (j + 1) * 128)
                y = _dot(_unpack(g_v[0:32, :]), wcol(w2_v, j))
                y = y + bias_v[0:1, FF + j * 128:FF + (j + 1) * 128]
                o = x1_v[:, cs] + mod_v[0:1, 5 * D + j * 128:5 * D + (j + 1) * 128] * y
                out_v[tp, :, cs] = o.astype(BF16)
        return run

    def out_copy(tp):
        return pltpu.make_async_copy(out_v.at[tp], out_hbm.at[tp], sem_out.at[0])

    def next_rows(r0, seg):
        def run():
            z = pl.multiple_of(zero_s[0], 8) if PIN else 0
            obuf[pl.ds(r0 + z, 24), 0:D] = pltpu.bitcast(ln1(x_v[seg, 0:24, :]), U32)
        return run

    def double_step(t, with_ffn):
        if with_ffn:
            ffn_pre(t - 1)
            fa = {k: ffn1(a, b) for k, (a, b) in FA.items()}
            fb = {k: ffn2(t - 1, a, b) for k, (a, b) in FB.items()}
            fb.update({k: ffn1(a, b) for k, (a, b) in FB1.items()})
        else:
            fa, fb = {}, {}
        fa[HNA if with_ffn else HN0] = next_rows(56, 2 * t + 1)
        fb[HNB if with_ffn else HN0] = next_rows(32, jnp.minimum(2 * t + 2, NSEG - 1))
        step(2 * t, False, fa, WSPLIT if with_ffn else WSPLIT0)
        step(2 * t + 1, True, fb, WSPLIT if with_ffn else WSPLIT0)
        if with_ffn:
            out_copy(t - 1).start()

    double_step(0, False)
    for cp in w1_copies() + w2_copies():
        cp.wait()
    if STOP == 3:
        x_copy(2).wait()
        return

    def body(t, carry):
        @pl.when(t == 2)
        def _():
            x_copy(2).wait()
        double_step(t, True)
        return carry

    jax.lax.fori_loop(1, NITER, body, 0)

    last = NITER - 1
    ffn_pre(last)
    ffn1(0, FF // 128)()
    ffn2(last, 0, 8)()
    out_copy(last).start()
    pltpu.make_async_copy(out_v.at[0:NITER], out_hbm.at[0:NITER], sem_out.at[0]).wait()


@functools.partial(jax.jit, static_argnames=("A_seg_len",))
def pallas_adaLN_cond__memory_aug_recurrent_mem_tr__dense_activation_gelu__prompt_kernel(
    A_x, A_mem0, A_Wq, A_Wk, A_Wv, A_Wo, A_seg_len, B_x, B_w1, B_b1, B_w2, B_b2, c, w_mod,
):
    assert A_x.shape == (1, S, D) and A_mem0.shape == (1, M, D) and A_seg_len == SEG
    assert A_Wq.shape == (D, H, DH) and B_w1.shape == (D, FF)
    any_spec = pl.BlockSpec(memory_space=pl.ANY)
    scratch = [
        pltpu.VMEM((NSEG, SEG, D), BF16),
        pltpu.VMEM((NSEG // 2, 2 * SEG, D), BF16),
        pltpu.VMEM((NSTAGE, D, 16, DH), BF16),
        pltpu.VMEM((3 * H * PITCH, DH), U32),
        pltpu.VMEM((8, H * DH, 128), BF16),
        pltpu.VMEM((FF // 128, D, 128), BF16),
        pltpu.VMEM((8, FF, 128), BF16),
        pltpu.VMEM((16, D, 128), BF16),
        pltpu.VMEM((32, D, 128), BF16),
        pltpu.VMEM((M, D), BF16),
        pltpu.VMEM((FF,), BF16),
        pltpu.VMEM((D,), BF16),
        pltpu.VMEM((1, D), BF16),
        pltpu.VMEM((8, 6 * D), F32),
        pltpu.VMEM((16, 8, 128), F32),
        pltpu.VMEM((32, 8, 128), F32),
        pltpu.VMEM((8, D), U32),
        pltpu.VMEM((8, FF + D), F32),
        pltpu.VMEM((8, NSEG * 8, 128), F32),
        pltpu.VMEM((9, 64, 512), U32),
        pltpu.VMEM((NPAIR, NSEG * 8, 2 * DH), F32),
        pltpu.VMEM((24, NSEG * 8, 2 * DH), U32),
        pltpu.VMEM((80, 128), F32),
        pltpu.VMEM((16, D), U32),
        pltpu.VMEM((32, NPAIR * 3 * DH), U32),
        pltpu.VMEM((40, NPAIR * DH), U32),
        pltpu.VMEM((80, NPAIR * DH), F32),
        pltpu.VMEM((80, NPAIR * DH), F32),
        pltpu.VMEM((48, D), F32),
        pltpu.VMEM((80, H * DH), U32),
        pltpu.VMEM((8, H * DH), F32),
        pltpu.VMEM((64, D), F32),
        pltpu.VMEM((64, D), F32),
        pltpu.VMEM((32, D), U32),
        pltpu.VMEM((32, FF), U32),
        pltpu.SMEM((1,), jnp.int32),
        pltpu.SemaphoreType.DMA((4,)),
        pltpu.SemaphoreType.DMA((3,)),
        pltpu.SemaphoreType.DMA((17,)),
        pltpu.SemaphoreType.DMA((8,)),
        pltpu.SemaphoreType.DMA((4,)),
        pltpu.SemaphoreType.DMA((1,)),
    ]
    out = pl.pallas_call(
        _kernel,
        out_shape=jax.ShapeDtypeStruct((NSEG // 2, 2 * SEG, D), BF16),
        in_specs=[any_spec] * 12,
        out_specs=any_spec,
        scratch_shapes=scratch,
        compiler_params=pltpu.CompilerParams(vmem_limit_bytes=120 * 1024 * 1024,
                                             disable_bounds_checks=True,
                                             disable_semaphore_checks=True),
    )(
        A_x.reshape(NSEG, SEG, D), A_mem0.reshape(M, D), A_Wq, A_Wk, A_Wv,
        A_Wo.reshape(H * DH, D), B_w1, B_b1, B_w2, B_b2,
        c, w_mod,
    )
    return out.reshape(1, S, D)
```

```python
import functools

import jax
import jax.numpy as jnp
import jax.experimental.pallas as pl
import jax.experimental.pallas.tpu as pltpu

F32 = jnp.float32
BF16 = jnp.bfloat16
U32 = jnp.uint32

S = 2048
D = 1024
H = 32
DH = 128
M = 8
SEG = 32
NSEG = S // SEG
FF = 3584
NPAIR = H // 2
PITCH = 516
XA = 8
NSTAGE = 4
STOP = 0
XHU = 2
QOFF, KOFF, VOFF, SOFF, POFF = 0.0, 0.1, 0.2, 1.5, 3.6
SSCR = 0
NEWTON = 1
KMAJOR = 1
KSTEP = 2
PIN = 1
HN0 = 10
MODMC = 1
HNA = 45.5
HNB = 47.9
FB1 = {}
OUTSPLIT = [(0, 7), (7, 8)]
SKEYS = [[19.5 + 1.25 * g for g in range(16)], [19.5 + 4 * (g // 3) + 0.1 * g for g in range(16)]]
PKEYS = [[24.6 + 1.25 * g for g in range(16)], [25.9 + 4 * (g // 3) + 0.1 * g for g in range(16)]]
WSPLIT = 0
WSPLIT0 = 4
WEARLY = [16.0, 16.1, 17.0, 17.1, 18.0, 18.1, 19.0, 19.1]
FA = {**{20 + j: (j, j + 1) for j in range(26)}, 200: (26, 28)}
FB = {20 + 4 * j: (j, j + 1) for j in range(8)}
NITER = NSEG // 2
EPS = 1e-5
SCALE = DH ** (-0.5)


def _pair_heads(gp):
    half, r = divmod(gp, 8)
    par, i = divmod(r, 4)
    h0 = 16 * half + 4 * i + par
    return h0, h0 + 2


def _ln(xf):
    m = jnp.mean(xf, axis=-1, keepdims=True)
    xc = xf - m
    v = jnp.mean(xc * xc, axis=-1, keepdims=True)
    return xc * jax.lax.rsqrt(v + EPS)


def _dot(a, b):
    return jnp.dot(a, b, preferred_element_type=F32)


def _dot_nt(a, b):
    return jax.lax.dot_general(a, b, (((1,), (1,)), ((), ())), preferred_element_type=F32)


def _pack(xf):
    return pltpu.bitcast(xf.astype(BF16), U32)


def _unpack(u):
    return pltpu.bitcast(u, BF16)


def _kernel(x_hbm, mem0_hbm, wq_hbm, wk_hbm, wv_hbm, wo_hbm, w1_hbm, b1_hbm, w2_hbm, b2_hbm,
            c_hbm, wmod_hbm,
            out_hbm,
            x_v, out_v, stage, wqkv, wo_v, w1_v, w2_v, wm0_v, wm1_v,
            mem0_v, b1_v, b2_v, c_v,
            mod_v, modq_v, modr_v, sc_v, bias_v, xh_v, h3_v, acc_v, qkv3, code_v,
            lhs_v, qkv_s, p_s, s_s, e_s, wacc, obuf, o3a, att_v, x1_v, h2_v, g_v, zero_s,
            sem_small, sem_x, sem_q, sem_u, sem_w, sem_out):
    w_hbms = (wq_hbm, wk_hbm, wv_hbm)

    def mo(i, n):
        return i if isinstance(i, int) else pl.multiple_of(i, n)

    def small_copies():
        return [pltpu.make_async_copy(c_hbm, c_v, sem_small.at[0]),
                pltpu.make_async_copy(mem0_hbm, mem0_v, sem_small.at[1]),
                pltpu.make_async_copy(b1_hbm, b1_v, sem_small.at[2]),
                pltpu.make_async_copy(b2_hbm, b2_v, sem_small.at[3])]

    def x_copy(part):
        s0, ns, lo, n = [(0, NSEG, 24, 8), (0, XA, 0, 24), (XA, NSEG - XA, 0, 24)][part]
        return pltpu.make_async_copy(x_hbm.at[pl.ds(s0, ns), pl.ds(lo, n), :],
                                     x_v.at[pl.ds(s0, ns), pl.ds(lo, n), :], sem_x.at[part])

    def wq_chunk_copy(j, sem):
        d0 = mo((j >> 1) * 128, 128)
        hf = j & 1
        return pltpu.make_async_copy(wq_hbm.at[pl.ds(d0, 128), pl.ds(mo(16 * hf, 16), 16), :],
                                     stage.at[hf, pl.ds(d0, 128)], sem)

    def wm0_copy(i, sem):
        c0 = mo((i & 1) * D + (i >> 1) * 128, 128)
        return pltpu.make_async_copy(wmod_hbm.at[:, pl.ds(c0, 128)], wm0_v.at[i], sem)

    def g2_piece_copy(j, sem):
        d0 = mo(j * 64, 64)
        return pltpu.make_async_copy(wk_hbm.at[pl.ds(d0, 64), pl.ds(0, 16), :],
                                     stage.at[2, pl.ds(d0, 64)], sem)

    def unit_copies(u):
        cps = [pltpu.make_async_copy(wmod_hbm.at[:, pl.ds(2 * D + j * 128, 128)], wm1_v.at[j],
                                     sem_u.at[u - 4]) for j in range(4 * (u - 4), 4 * (u - 3))]
        if u < 10:
            grp = u // 2 + 1
            mat, half = divmod(grp, 2)
            rows = pl.ds((u % 2) * 512, 512)
            cps.append(pltpu.make_async_copy(w_hbms[mat].at[rows, pl.ds(16 * half, 16), :],
                                             stage.at[grp % NSTAGE, rows], sem_u.at[u - 4]))
        return cps

    def slab_copies(src, c0, dst, sem):
        return [pltpu.make_async_copy(src.at[:, pl.ds(c0 + j * 128, 128)], dst.at[j], sem)
                for j in range(dst.shape[0])]

    wo_copies = lambda: slab_copies(wo_hbm, 0, wo_v, sem_w.at[0])
    w1_copies = lambda: slab_copies(w1_hbm, 0, w1_v, sem_w.at[2])
    w2_copies = lambda: slab_copies(w2_hbm, 0, w2_v, sem_w.at[3])

    def wcol(ref, j):
        return _unpack(ref.bitcast(U32)[j])

    def relayout(src, dst, j0, j1):
        srcu = src.bitcast(U32)
        for j in range(j0, j1):
            a = srcu[2 * j]
            b = srcu[2 * j + 1]
            dst[pl.ds(j, 8, stride=PITCH), :] = (a & jnp.uint32(0xFFFF)) | (b << 16)
            dst[pl.ds(8 * PITCH + j, 8, stride=PITCH), :] = (a >> 16) | (b & jnp.uint32(0xFFFF0000))

    def wpair(ref, slab0, n=D // 2):
        return jnp.concatenate([_unpack(ref[pl.ds(slab0 * PITCH, n), :]),
                                _unpack(ref[pl.ds((slab0 + 1) * PITCH, n), :])], axis=1)

    def modrow(i):
        return mod_v[0:1, i * D:(i + 1) * D]

    def first_copies():
        return [wm0_copy(i, sem_q.at[16]) for i in range(2)] + [wq_chunk_copy(0, sem_q.at[16])]

    def q_copies(j, do):
        do(g2_piece_copy(j, sem_q.at[j]))

        @pl.when(j < 15)
        def _():
            do(wq_chunk_copy(j + 1, sem_q.at[j]))

        @pl.when(j < 14)
        def _():
            do(wm0_copy(j + 2, sem_q.at[j]))

    def issue(i, carry):
        @pl.when(i == 0)
        def _():
            for cp in small_copies():
                cp.start()
            x_copy(0).start()

        @pl.when(i == 1)
        def _():
            for cp in first_copies():
                cp.start()

        @pl.when(jnp.logical_and(i >= 2, i < 18))
        def _():
            q_copies(i - 2, lambda cp: cp.start())

        @pl.when(i == 18)
        def _():
            for cp in unit_copies(4) + [x_copy(1)]:
                cp.start()

        @pl.when(i == 19)
        def _():
            for cp in unit_copies(5):
                cp.start()
        return carry

    jax.lax.fori_loop(0, 20, issue, 0)
    zero_s[0] = 0

    ri = jax.lax.broadcasted_iota(jnp.int32, (80, 128), 0)
    ci = jax.lax.broadcasted_iota(jnp.int32, (80, 128), 1)

    def head_of(i):
        return jnp.where(i < 64, i // 32, (i - 64) // 8)

    def pos_of(i):
        return jnp.where(i < 64, i % 32, 32 + (i - 64) % 8)

    same = head_of(ri) == head_of(ci)
    pr, pc = pos_of(ri), pos_of(ci)
    keep = jnp.logical_or(pr < M, pr >= pc)
    code_v[...] = jnp.where(same, jnp.where(keep, 0.0, -1e9), -jnp.inf).astype(F32)

    for cp in small_copies():
        cp.wait()
    cf = c_v[...].astype(F32)
    sc_v[...] = _pack(jnp.broadcast_to(cf * jax.nn.sigmoid(cf), (16, D)))
    bias_v[:, 0:FF] = jnp.broadcast_to(b1_v[...].astype(F32).reshape(1, FF), (8, FF))
    bias_v[:, FF:] = jnp.broadcast_to(b2_v[...].astype(F32).reshape(1, D), (8, D))

    x_copy(0).wait()

    def xh_body(i, carry):
        for h in range(XHU):
            s0 = pl.multiple_of((i * XHU + h) * 8, 8)
            xh = _ln(x_v[pl.ds(s0, 8), 24:32, :].astype(F32).reshape(64, D))
            r0 = pl.multiple_of((i * XHU + h) * 64, 64)
            for kt in range(8):
                xh_v[kt, pl.ds(r0, 64), :] = xh[:, kt * 128:(kt + 1) * 128]
        return carry

    jax.lax.fori_loop(0, 8 // XHU, xh_body, 0)

    def mod_slab(i):
        modq_v[i] = _dot(_unpack(sc_v[...]), wcol(wm0_v, i))[0:8]

    def h3_store(dst, kt, mc):
        sa = modq_v[2 * kt, 0:1, :]
        ca = modq_v[2 * kt + 1, 0:1, :]
        dst[:, mc * 128:(mc + 1) * 128] = _pack(
            xh_v[kt, mc * 128:(mc + 1) * 128, :] * (1.0 + ca) + sa)

    for cp in first_copies():
        cp.wait()
    modq_v[2:16] = jnp.zeros((14, 8, 128), F32)
    for i in range(2):
        mod_slab(i)
    for mc in range(4):
        h3_store(h3_v.at[0], 0, mc)
    relayout(stage.at[0], wqkv, 0, 64)

    def q_body(j, carry):
        q_copies(j, lambda cp: cp.wait())
        kt, hf = j >> 1, j & 1
        jn = jnp.minimum(j + 1, 15)
        ktn, hfn = jn >> 1, jn & 1
        hview = h3_v.at[pl.ds(kt, 2)]
        wview = wqkv.at[pl.ds(pl.multiple_of(hf * (16 * PITCH) + kt * 64, 8), 16 * PITCH - 448), :]
        aview = acc_v.at[pl.ds(pl.multiple_of(hf * 8, 8), 8)]
        qsrc = stage.at[hfn, pl.ds(pl.multiple_of(ktn * 128, 128), 128)]
        qdst = wqkv.at[pl.ds(pl.multiple_of(hfn * (16 * PITCH) + ktn * 64, 8), 16 * PITCH - 448), :]
        ksrc = stage.at[2, pl.ds(pl.multiple_of(j * 64, 64), 64)]
        kdst = wqkv.at[pl.ds(pl.multiple_of(32 * PITCH + j * 32, 8), 16 * PITCH - 480), :]
        for p in range(8):
            lhs = jnp.concatenate([hview[0, :, mc * 128:(mc + 1) * 128] for mc in range(4)], axis=0)
            y = _dot(_unpack(lhs), wpair(wview, 2 * p, 64))
            aview[p] = jnp.where(kt > 0, aview[p], 0.0) + y
            if p == 1:
                mod_slab(jnp.minimum(j + 2, 15))
            if p >= 4:
                h3_store(hview.at[1], jnp.minimum(kt + 1, 7), p - 4)
            if p % 2 == 1:
                relayout(qsrc, qdst, 8 * p - 8, 8 * p + 8)
                relayout(ksrc, kdst, 4 * p - 4, 4 * p + 4)
        return carry

    jax.lax.fori_loop(0, 16, q_body, 0)
    for kt in range(8):
        mod_v[:, kt * 128:(kt + 1) * 128] = modq_v[2 * kt]
        mod_v[:, D + kt * 128:D + (kt + 1) * 128] = modq_v[2 * kt + 1]
    for cp in unit_copies(6):
        cp.start()
    x_copy(1).wait()

    def ln1(xb):
        return _ln(xb.astype(F32)) * (1.0 + modrow(1)) + modrow(0)

    def store_x3(dst, half, mc, y):
        y = y.reshape(16, 8, 256)
        y = jnp.concatenate([y[:, :, :128], y[:, :, 128:]], axis=1).reshape(256, DH)
        dst[mc * 128:(mc + 1) * 128, half * DH:(half + 1) * DH] = _pack(y)

    def unit_body(u, carry):
        gn = jnp.minimum((u >> 1) + 1, 5)
        src = stage.at[gn & (NSTAGE - 1), pl.ds(pl.multiple_of((u & 1) * 512, 512), 512)]
        wm = wm1_v.at[pl.ds(4 * (u - 4), 4)]
        pltpu.make_async_copy(wm, wm, sem_u.at[u - 4]).wait()

        @pl.when(u < 10)
        def _():
            pltpu.make_async_copy(src, src, sem_u.at[u - 4]).wait()

        for k, cps in [(7, w1_copies), (4, lambda: unit_copies(7) + unit_copies(8)),
                       (5, lambda: unit_copies(9) + unit_copies(10) + unit_copies(11)),
                       (6, wo_copies), (8, w2_copies), (9, lambda: [x_copy(2)])][0:{0: 6, 3: 5, 4: 4}[STOP]]:
            @pl.when(u == k)
            def _(cps=cps):
                for cp in cps():
                    cp.start()

        lhs_v[...] = _pack(jnp.concatenate([mem0_v[...].astype(F32), ln1(x_v[0, 0:24, :])], axis=0))
        dst = wqkv.at[pl.ds(pl.multiple_of(gn * (16 * PITCH) + (u & 1) * 256, 8), 16 * PITCH - 256), :]
        view = wqkv.at[pl.ds(pl.multiple_of(u * (8 * PITCH), 8), 8 * PITCH), :]
        for p in range(4):
            for mc in range(4):
                lhs = _unpack(jnp.concatenate(
                    [h3_v[kt, :, mc * 128:(mc + 1) * 128] for kt in range(8)], axis=1))
                store_x3(qkv3.at[2 * u + p // 2], p % 2, mc, _dot(lhs, wpair(view, 2 * p)))
                relayout(src, dst, 16 * (4 * p + mc), 16 * (4 * p + mc + 1))
                if mc == MODMC:
                    modr_v[4 * (u - 4) + p] = _dot(_unpack(sc_v[...]), wcol(wm, p))[0:8]
                if p % 2 == 0:
                    store_x3(qkv3.at[u - 4], p // 2, mc,
                             acc_v[2 * (u - 4) + p // 2, mc * 128:(mc + 1) * 128, :])
        return carry

    jax.lax.fori_loop(4, 12, unit_body, 0)

    for cp in wo_copies():
        cp.wait()
    for j in range(32):
        mod_v[:, 2 * D + j * 128:2 * D + (j + 1) * 128] = modr_v[j]

    zpad = jnp.zeros((24, DH), U32)

    def proj(g, mat):
        y = _dot(_unpack(lhs_v[...]), wpair(wqkv, mat * H + 2 * g))
        cs = pl.ds((g * 3 + mat) * DH, DH)
        qkv_s[0:16, cs] = _pack(y[:, :DH])
        qkv_s[16:32, cs] = _pack(y[:, DH:])

    def proj4(gg, mat):
        y = None
        for kt in range(0, 8, KSTEP):
            w = jnp.concatenate(
                [_unpack(wqkv[pl.ds((mat * H + 4 * gg + i) * PITCH + 64 * kt, 64 * KSTEP), :])
                 for i in range(4)], axis=1)
            d = _dot(_unpack(lhs_v[:, kt * 128:(kt + KSTEP) * 128]), w)
            y = d if y is None else y + d
        for i in range(4):
            cs = pl.ds(((2 * gg + i // 2) * 3 + mat) * DH, DH)
            qkv_s[16 * (i % 2):16 * (i % 2 + 1), cs] = _pack(y[:, i * DH:(i + 1) * DH])

    def get(g, mat, seg):
        u3, p3 = divmod(mat * NPAIR + g, 2)
        parts = [qkv_s[:, pl.ds((g * 3 + mat) * DH, DH)],
                 qkv3[u3, pl.ds(mo(seg * 8, 8), 8), p3 * DH:(p3 + 1) * DH]]
        if mat > 0:
            parts.append(zpad)
        return _unpack(jnp.concatenate(parts, axis=0))

    def scores(g, q, k):
        cs = pl.ds(g * DH, DH)
        s = _dot_nt(q, k) * SCALE
        code = code_v[...]
        s = jnp.where(code == 0.0, s, code)
        m = jnp.max(s, axis=-1, keepdims=True)
        if SSCR & 1:
            s_s[:, cs] = s
            s = s_s[:, cs]
        e = jnp.exp(s - m)
        l = jnp.sum(e, axis=-1, keepdims=True)
        if SSCR & 2:
            e_s[:, cs] = e
            e = e_s[:, cs]
        r = pl.reciprocal(l, approx=True)
        if NEWTON:
            r = r * (2.0 - l * r)
        return (e * r).astype(BF16)

    def pv(g, p, v, second):
        o = _dot(p, v)
        c0, c1 = (h * DH for h in _pair_heads(g))
        obuf[0:16, c0:c0 + DH] = _pack(o[0:32])
        obuf[0:16, c1:c1 + DH] = _pack(o[32:64])
        if not second:
            o3a[:, c0:c0 + DH] = o[64:72]
            o3a[:, c1:c1 + DH] = o[72:80]
        else:
            obuf[16:24, c0:c0 + DH] = _pack(jnp.concatenate([o3a[:, c0:c0 + DH], o[64:72]], axis=0))
            obuf[16:24, c1:c1 + DH] = _pack(jnp.concatenate([o3a[:, c1:c1 + DH], o[72:80]], axis=0))

    def wo_cols(pairs):
        return sorted(h for g in pairs for h in _pair_heads(g))

    def wo_dot(j, heads, nrow):
        lhs = jnp.concatenate([obuf[0:nrow, h * DH:(h + 1) * DH] for h in heads], axis=1)
        w = jnp.concatenate([wo_v.bitcast(U32)[j, h * 64:(h + 1) * 64, :] for h in heads], axis=0)
        return _dot(_unpack(lhs), _unpack(w))

    def step(seg, second, fillers, wsplit):
        nrow = 24 if second else 16
        early, late = wo_cols(range(NPAIR - wsplit)), wo_cols(range(NPAIR - wsplit, NPAIR))

        def do_scores(g):
            p_s[:, pl.ds(g * DH, DH)] = pltpu.bitcast(scores(g, get(g, 0, seg), get(g, 1, seg)), U32)

        def do_pv(g):
            pv(g, _unpack(p_s[:, pl.ds(g * DH, DH)]), get(g, 2, seg), second)

        def wo_early(j):
            wacc[0:2 * nrow, j * 128:(j + 1) * 128] = wo_dot(j, early, nrow)

        def wo_final(j):
            cs = slice(j * 128, (j + 1) * 128)
            if wsplit:
                y = wacc[0:2 * nrow, cs] + wo_dot(j, late, nrow)
            else:
                y = wo_dot(j, early, nrow)
            r0 = 32 if second else 56
            hn = pltpu.bitcast(obuf[r0:r0 + 24, cs], F32)
            lhs_v[:, cs] = _pack(jnp.concatenate([y[0:8], hn], axis=0))
            if not second:
                att_v[0:24, cs] = y[8:32]
            else:
                att_v[32:56, cs] = y[8:32]
                att_v[24:32, cs] = y[32:40]
                att_v[56:64, cs] = y[40:48]

        ev = []
        for g in range(NPAIR):
            if not KMAJOR:
                ev.append((g + QOFF, functools.partial(proj, g, 0)))
                ev.append((g + KOFF, functools.partial(proj, g, 1)))
                ev.append((g + VOFF, functools.partial(proj, g, 2)))
            elif g % 2 == 0:
                ev.append((g, functools.partial(proj4, g // 2, 0)))
                ev.append((g + 0.66, functools.partial(proj4, g // 2, 1)))
                ev.append((g + 1.33, functools.partial(proj4, g // 2, 2)))
            skey, pkey = (SKEYS[second][g], PKEYS[second][g]) if (SKEYS and not wsplit) else (g + SOFF, g + POFF)
            ev.append((skey, functools.partial(do_scores, g)))
            ev.append((pkey, functools.partial(do_pv, g)))
        if wsplit:
            for j in range(8):
                ev.append((WEARLY[j], functools.partial(wo_early, j)))
        for j in range(8):
            ev.append((100 + j, functools.partial(wo_final, j)))
        ev.extend(fillers.items())
        ev.sort(key=lambda e: e[0])
        for _, f in ev:
            f()

    def ffn_pre(tp):
        xb = x_v[pl.ds(2 * tp, 2)].astype(F32).reshape(64, D)
        x1 = xb + modrow(2) * att_v[...]
        x1_v[...] = x1
        h2_v[0:32, :] = _pack(_ln(x1) * (1.0 + modrow(4)) + modrow(3))

    def ffn1(lo, hi):
        def run():
            for j in range(lo, hi):
                cs = slice(j * 128, (j + 1) * 128)
                y = _dot(_unpack(h2_v[0:32, :]), wcol(w1_v, j)) + bias_v[0:1, cs]
                g_v[0:32, cs] = _pack(jax.nn.gelu(y, approximate=True))
        return run

    def ffn2(tp, lo, hi):
        def run():
            for j in range(lo, hi):
                cs = slice(j * 128, (j + 1) * 128)
                y = _dot(_unpack(g_v[0:32, :]), wcol(w2_v, j))
                y = y + bias_v[0:1, FF + j * 128:FF + (j + 1) * 128]
                o = x1_v[:, cs] + mod_v[0:1, 5 * D + j * 128:5 * D + (j + 1) * 128] * y
                out_v[tp, :, cs] = o.astype(BF16)
        return run

    def out_copy(tp):
        return pltpu.make_async_copy(out_v.at[tp], out_hbm.at[tp], sem_out.at[0])

    def next_rows(r0, seg):
        def run():
            z = pl.multiple_of(zero_s[0], 8) if PIN else 0
            obuf[pl.ds(r0 + z, 24), 0:D] = pltpu.bitcast(ln1(x_v[seg, 0:24, :]), U32)
        return run

    def double_step(t, with_ffn):
        if with_ffn:
            ffn_pre(t - 1)
            fa = {k: ffn1(a, b) for k, (a, b) in FA.items()}
            fb = {k: ffn2(t - 1, a, b) for k, (a, b) in FB.items()}
            fb.update({k: ffn1(a, b) for k, (a, b) in FB1.items()})
        else:
            fa, fb = {}, {}
        fa[HNA if with_ffn else HN0] = next_rows(56, 2 * t + 1)
        fb[HNB if with_ffn else HN0] = next_rows(32, jnp.minimum(2 * t + 2, NSEG - 1))
        step(2 * t, False, fa, WSPLIT if with_ffn else WSPLIT0)
        step(2 * t + 1, True, fb, WSPLIT if with_ffn else WSPLIT0)
        if with_ffn:
            out_copy(t - 1).start()

    double_step(0, False)
    for cp in w1_copies() + (w2_copies() if STOP != 4 else []):
        cp.wait()
    if STOP:
        return

    def body(t, carry):
        @pl.when(t == 2)
        def _():
            x_copy(2).wait()
        double_step(t, True)
        return carry

    jax.lax.fori_loop(1, NITER, body, 0)

    last = NITER - 1
    ffn_pre(last)
    ffn1(0, FF // 128)()
    for lo, hi in OUTSPLIT:
        ffn2(last, lo, hi)()
        cols = pl.ds(lo * 128, (hi - lo) * 128)
        pltpu.make_async_copy(out_v.at[last, :, cols], out_hbm.at[last, :, cols],
                              sem_out.at[0]).start()
    pltpu.make_async_copy(out_v.at[0:NITER], out_hbm.at[0:NITER], sem_out.at[0]).wait()


@functools.partial(jax.jit, static_argnames=("A_seg_len",))
def pallas_adaLN_cond__memory_aug_recurrent_mem_tr__dense_activation_gelu__prompt_kernel(
    A_x, A_mem0, A_Wq, A_Wk, A_Wv, A_Wo, A_seg_len, B_x, B_w1, B_b1, B_w2, B_b2, c, w_mod,
):
    assert A_x.shape == (1, S, D) and A_mem0.shape == (1, M, D) and A_seg_len == SEG
    assert A_Wq.shape == (D, H, DH) and B_w1.shape == (D, FF)
    any_spec = pl.BlockSpec(memory_space=pl.ANY)
    scratch = [
        pltpu.VMEM((NSEG, SEG, D), BF16),
        pltpu.VMEM((NSEG // 2, 2 * SEG, D), BF16),
        pltpu.VMEM((NSTAGE, D, 16, DH), BF16),
        pltpu.VMEM((3 * H * PITCH, DH), U32),
        pltpu.VMEM((8, H * DH, 128), BF16),
        pltpu.VMEM((FF // 128, D, 128), BF16),
        pltpu.VMEM((8, FF, 128), BF16),
        pltpu.VMEM((16, D, 128), BF16),
        pltpu.VMEM((32, D, 128), BF16),
        pltpu.VMEM((M, D), BF16),
        pltpu.VMEM((FF,), BF16),
        pltpu.VMEM((D,), BF16),
        pltpu.VMEM((1, D), BF16),
        pltpu.VMEM((8, 6 * D), F32),
        pltpu.VMEM((16, 8, 128), F32),
        pltpu.VMEM((32, 8, 128), F32),
        pltpu.VMEM((8, D), U32),
        pltpu.VMEM((8, FF + D), F32),
        pltpu.VMEM((8, NSEG * 8, 128), F32),
        pltpu.VMEM((9, 64, 512), U32),
        pltpu.VMEM((NPAIR, NSEG * 8, 2 * DH), F32),
        pltpu.VMEM((24, NSEG * 8, 2 * DH), U32),
        pltpu.VMEM((80, 128), F32),
        pltpu.VMEM((16, D), U32),
        pltpu.VMEM((32, NPAIR * 3 * DH), U32),
        pltpu.VMEM((40, NPAIR * DH), U32),
        pltpu.VMEM((80, NPAIR * DH), F32),
        pltpu.VMEM((80, NPAIR * DH), F32),
        pltpu.VMEM((48, D), F32),
        pltpu.VMEM((80, H * DH), U32),
        pltpu.VMEM((8, H * DH), F32),
        pltpu.VMEM((64, D), F32),
        pltpu.VMEM((64, D), F32),
        pltpu.VMEM((32, D), U32),
        pltpu.VMEM((32, FF), U32),
        pltpu.SMEM((1,), jnp.int32),
        pltpu.SemaphoreType.DMA((4,)),
        pltpu.SemaphoreType.DMA((3,)),
        pltpu.SemaphoreType.DMA((17,)),
        pltpu.SemaphoreType.DMA((8,)),
        pltpu.SemaphoreType.DMA((4,)),
        pltpu.SemaphoreType.DMA((1,)),
    ]
    out = pl.pallas_call(
        _kernel,
        out_shape=jax.ShapeDtypeStruct((NSEG // 2, 2 * SEG, D), BF16),
        in_specs=[any_spec] * 12,
        out_specs=any_spec,
        scratch_shapes=scratch,
        compiler_params=pltpu.CompilerParams(vmem_limit_bytes=120 * 1024 * 1024,
                                             disable_bounds_checks=True,
                                             disable_semaphore_checks=True),
    )(
        A_x.reshape(NSEG, SEG, D), A_mem0.reshape(M, D), A_Wq, A_Wk, A_Wv,
        A_Wo.reshape(H * DH, D), B_w1, B_b1, B_w2, B_b2,
        c, w_mod,
    )
    return out.reshape(1, S, D)
```

```python
import functools

import jax
import jax.numpy as jnp
import jax.experimental.pallas as pl
import jax.experimental.pallas.tpu as pltpu

F32 = jnp.float32
BF16 = jnp.bfloat16
U32 = jnp.uint32

S = 2048
D = 1024
H = 32
DH = 128
M = 8
SEG = 32
NSEG = S // SEG
FF = 3584
NPAIR = H // 2
PITCH = 516
XA = 8
NSTAGE = 4
NDS = NSEG // 2
FFN1_KEYS = [20 + j for j in range(FF // 128)]
FFN2_KEYS = [20 + 4 * j for j in range(D // 128)]
SCORE_KEYS = [[20.5 + 1.3 * g for g in range(NPAIR)],
              [20.5 + 4 * (g // 3) + 0.1 * g for g in range(NPAIR)]]
PV_KEYS = [[25.6 + 1.3 * g for g in range(NPAIR)],
           [27.0 + 4 * (g // 3) + 0.01 * g for g in range(NPAIR)]]
NEXT_KEYS = [47.5, 47.9]
SOFF0, POFF0, NEXT0, WSPLIT0 = 2.1, 4.2, 10, 5
WEARLY0 = [16.0 + 0.5 * j for j in range(8)]
CHECKS = False
EPS = 1e-5
SCALE = DH ** (-0.5)


def _pair_heads(gp):
    half, r = divmod(gp, 8)
    par, i = divmod(r, 4)
    h0 = 16 * half + 4 * i + par
    return h0, h0 + 2


def _ln(xf):
    m = jnp.mean(xf, axis=-1, keepdims=True)
    xc = xf - m
    v = jnp.mean(xc * xc, axis=-1, keepdims=True)
    return xc * jax.lax.rsqrt(v + EPS)


def _dot(a, b):
    return jnp.dot(a, b, preferred_element_type=F32)


def _dot_nt(a, b):
    return jax.lax.dot_general(a, b, (((1,), (1,)), ((), ())), preferred_element_type=F32)


def _pack(xf):
    return pltpu.bitcast(xf.astype(BF16), U32)


def _unpack(u):
    return pltpu.bitcast(u, BF16)


def _kernel(x_hbm, mem0_hbm, wq_hbm, wk_hbm, wv_hbm, wo_hbm, w1_hbm, b1_hbm, w2_hbm, b2_hbm,
            c_hbm, wmod_hbm,
            out_hbm,
            x_v, out_v, stage, wqkv, wo_v, w1_v, w2_v, wm0_v, wm1_v,
            mem0_v, b1_v, b2_v, c_v,
            mod_v, modq_v, modr_v, sc_v, bias_v, xh_v, h3_v, acc_v, qkv3, code_v,
            lhs_v, qkv_s, p_s, wacc, obuf, o3a, x1n_v, x1_v, h2_v, g_v, zero_s,
            sem_small, sem_x, sem_q, sem_u, sem_w, sem_out):
    w_hbms = (wq_hbm, wk_hbm, wv_hbm)

    def mo(i, n):
        return i if isinstance(i, int) else pl.multiple_of(i, n)

    def small_copies():
        return [pltpu.make_async_copy(c_hbm, c_v, sem_small.at[0]),
                pltpu.make_async_copy(mem0_hbm, mem0_v, sem_small.at[1]),
                pltpu.make_async_copy(b1_hbm, b1_v, sem_small.at[2]),
                pltpu.make_async_copy(b2_hbm, b2_v, sem_small.at[3])]

    def x_copy(part):
        s0, ns, lo, n = [(0, NSEG, 24, 8), (0, XA, 0, 24), (XA, NSEG - XA, 0, 24)][part]
        return pltpu.make_async_copy(x_hbm.at[pl.ds(s0, ns), pl.ds(lo, n), :],
                                     x_v.at[pl.ds(s0, ns), pl.ds(lo, n), :], sem_x.at[part])

    def wq_chunk_copy(j, sem):
        d0 = mo((j >> 1) * 128, 128)
        hf = j & 1
        return pltpu.make_async_copy(wq_hbm.at[pl.ds(d0, 128), pl.ds(mo(16 * hf, 16), 16), :],
                                     stage.at[hf, pl.ds(d0, 128)], sem)

    def wm0_copy(i, sem):
        c0 = mo((i & 1) * D + (i >> 1) * 128, 128)
        return pltpu.make_async_copy(wmod_hbm.at[:, pl.ds(c0, 128)], wm0_v.at[i], sem)

    def g2_piece_copy(j, sem):
        d0 = mo(j * 64, 64)
        return pltpu.make_async_copy(wk_hbm.at[pl.ds(d0, 64), pl.ds(0, 16), :],
                                     stage.at[2, pl.ds(d0, 64)], sem)

    def unit_copies(u):
        cps = [pltpu.make_async_copy(wmod_hbm.at[:, pl.ds(2 * D + j * 128, 128)], wm1_v.at[j],
                                     sem_u.at[u - 4]) for j in range(4 * (u - 4), 4 * (u - 3))]
        if u < 10:
            grp = u // 2 + 1
            mat, half = divmod(grp, 2)
            rows = pl.ds((u % 2) * 512, 512)
            cps.append(pltpu.make_async_copy(w_hbms[mat].at[rows, pl.ds(16 * half, 16), :],
                                             stage.at[grp % NSTAGE, rows], sem_u.at[u - 4]))
        return cps

    def slab_copies(src, dst, sem):
        return [pltpu.make_async_copy(src.at[:, pl.ds(j * 128, 128)], dst.at[j], sem)
                for j in range(dst.shape[0])]

    wo_copies = lambda: slab_copies(wo_hbm, wo_v, sem_w.at[0])
    w1_copies = lambda: slab_copies(w1_hbm, w1_v, sem_w.at[1])
    w2_copies = lambda: slab_copies(w2_hbm, w2_v, sem_w.at[2])

    def wcol(ref, j):
        return _unpack(ref.at[j].bitcast(U32)[...])

    def relayout(src, dst, j0, j1):
        srcu = src.bitcast(U32)
        for j in range(j0, j1):
            a = srcu[2 * j]
            b = srcu[2 * j + 1]
            dst[pl.ds(j, 8, stride=PITCH), :] = (a & jnp.uint32(0xFFFF)) | (b << 16)
            dst[pl.ds(8 * PITCH + j, 8, stride=PITCH), :] = (a >> 16) | (b & jnp.uint32(0xFFFF0000))

    def wpair(ref, slab0, n=D // 2):
        return jnp.concatenate([_unpack(ref[pl.ds(slab0 * PITCH, n), :]),
                                _unpack(ref[pl.ds((slab0 + 1) * PITCH, n), :])], axis=1)

    def modrow(i):
        return mod_v[0:1, i * D:(i + 1) * D]

    def first_copies():
        return [wm0_copy(i, sem_q.at[16]) for i in range(2)] + [wq_chunk_copy(0, sem_q.at[16])]

    def q_copies(j, do):
        do(g2_piece_copy(j, sem_q.at[j]))

        @pl.when(j < 15)
        def _():
            do(wq_chunk_copy(j + 1, sem_q.at[j]))

        @pl.when(j < 14)
        def _():
            do(wm0_copy(j + 2, sem_q.at[j]))

    def issue(i, carry):
        @pl.when(i == 0)
        def _():
            for cp in small_copies():
                cp.start()
            x_copy(0).start()

        @pl.when(i == 1)
        def _():
            for cp in first_copies():
                cp.start()

        @pl.when(jnp.logical_and(i >= 2, i < 18))
        def _():
            q_copies(i - 2, lambda cp: cp.start())

        @pl.when(i == 18)
        def _():
            for cp in unit_copies(4) + [x_copy(1)]:
                cp.start()

        @pl.when(i == 19)
        def _():
            for cp in unit_copies(5):
                cp.start()
        return carry

    jax.lax.fori_loop(0, 20, issue, 0)
    zero_s[0] = 0

    ri = jax.lax.broadcasted_iota(jnp.int32, (80, 128), 0)
    ci = jax.lax.broadcasted_iota(jnp.int32, (80, 128), 1)

    def head_of(i):
        return jnp.where(i < 64, i // 32, (i - 64) // 8)

    def pos_of(i):
        return jnp.where(i < 64, i % 32, 32 + (i - 64) % 8)

    same = head_of(ri) == head_of(ci)
    pr, pc = pos_of(ri), pos_of(ci)
    keep = jnp.logical_or(pr < M, pr >= pc)
    code_v[...] = jnp.where(same, jnp.where(keep, 0.0, -1e9), -jnp.inf).astype(F32)

    for cp in small_copies():
        cp.wait()
    cf = c_v[...].astype(F32)
    sc_v[...] = _pack(jnp.broadcast_to(cf * jax.nn.sigmoid(cf), (16, D)))
    bias_v[:, 0:FF] = jnp.broadcast_to(b1_v[...].astype(F32).reshape(1, FF), (8, FF))
    bias_v[:, FF:] = jnp.broadcast_to(b2_v[...].astype(F32).reshape(1, D), (8, D))

    x_copy(0).wait()

    def xh_body(i, carry):
        for h in range(2):
            s0 = pl.multiple_of((i * 2 + h) * 8, 8)
            xh = _ln(x_v[pl.ds(s0, 8), 24:32, :].astype(F32).reshape(64, D))
            r0 = pl.multiple_of((i * 2 + h) * 64, 64)
            for kt in range(8):
                xh_v[kt, pl.ds(r0, 64), :] = xh[:, kt * 128:(kt + 1) * 128]
        return carry

    jax.lax.fori_loop(0, 4, xh_body, 0)

    def mod_slab(i):
        modq_v[i] = _dot(_unpack(sc_v[...]), wcol(wm0_v, i))[0:8]

    def h3_store(dst, kt, mc):
        sa = modq_v[2 * kt, 0:1, :]
        ca = modq_v[2 * kt + 1, 0:1, :]
        dst[:, mc * 128:(mc + 1) * 128] = _pack(
            xh_v[kt, mc * 128:(mc + 1) * 128, :] * (1.0 + ca) + sa)

    for cp in first_copies():
        cp.wait()
    modq_v[2:16] = jnp.zeros((14, 8, 128), F32)
    for i in range(2):
        mod_slab(i)
    for mc in range(4):
        h3_store(h3_v.at[0], 0, mc)
    relayout(stage.at[0, pl.ds(0, 128)], wqkv, 0, 64)

    def q_body(j, carry):
        q_copies(j, lambda cp: cp.wait())
        kt, hf = j >> 1, j & 1
        jn = jnp.minimum(j + 1, 15)
        ktn, hfn = jn >> 1, jn & 1
        hview = h3_v.at[pl.ds(kt, 2)]
        wview = wqkv.at[pl.ds(pl.multiple_of(hf * (16 * PITCH) + kt * 64, 8), 16 * PITCH - 448), :]
        aview = acc_v.at[pl.ds(pl.multiple_of(hf * 8, 8), 8)]
        qsrc = stage.at[hfn, pl.ds(pl.multiple_of(ktn * 128, 128), 128)]
        qdst = wqkv.at[pl.ds(pl.multiple_of(hfn * (16 * PITCH) + ktn * 64, 8), 16 * PITCH + 64), :]
        ksrc = stage.at[2, pl.ds(pl.multiple_of(j * 64, 64), 64)]
        kdst = wqkv.at[pl.ds(pl.multiple_of(32 * PITCH + j * 32, 8), 16 * PITCH + 32), :]
        for p in range(8):
            lhs = jnp.concatenate([hview[0, :, mc * 128:(mc + 1) * 128] for mc in range(4)], axis=0)
            y = _dot(_unpack(lhs), wpair(wview, 2 * p, 64))
            aview[p] = jnp.where(kt > 0, aview[p], 0.0) + y
            if p == 1:
                mod_slab(jnp.minimum(j + 2, 15))
            if p >= 4:
                h3_store(hview.at[1], jnp.minimum(kt + 1, 7), p - 4)
            if p % 2 == 1:
                relayout(qsrc, qdst, 8 * p - 8, 8 * p + 8)
                relayout(ksrc, kdst, 4 * p - 4, 4 * p + 4)
        return carry

    jax.lax.fori_loop(0, 16, q_body, 0)
    for kt in range(8):
        mod_v[:, kt * 128:(kt + 1) * 128] = modq_v[2 * kt]
        mod_v[:, D + kt * 128:D + (kt + 1) * 128] = modq_v[2 * kt + 1]
    for cp in unit_copies(6):
        cp.start()
    x_copy(1).wait()

    def ln1(xb):
        return _ln(xb.astype(F32)) * (1.0 + modrow(1)) + modrow(0)

    def store_x3(dst, half, mc, y):
        y = y.reshape(16, 8, 256)
        y = jnp.concatenate([y[:, :, :128], y[:, :, 128:]], axis=1).reshape(256, DH)
        dst[mc * 128:(mc + 1) * 128, half * DH:(half + 1) * DH] = _pack(y)

    def unit_body(u, carry):
        gn = jnp.minimum((u >> 1) + 1, 5)
        src = stage.at[gn & (NSTAGE - 1), pl.ds(pl.multiple_of((u & 1) * 512, 512), 512)]
        wm = wm1_v.at[pl.ds(4 * (u - 4), 4)]
        pltpu.make_async_copy(wm, wm, sem_u.at[u - 4]).wait()

        @pl.when(u < 10)
        def _():
            pltpu.make_async_copy(src, src, sem_u.at[u - 4]).wait()

        for k, cps in [(7, w1_copies), (4, lambda: unit_copies(7) + unit_copies(8)),
                       (5, lambda: unit_copies(9) + unit_copies(10) + unit_copies(11)),
                       (6, wo_copies), (8, w2_copies), (9, lambda: [x_copy(2)])]:
            @pl.when(u == k)
            def _(cps=cps):
                for cp in cps():
                    cp.start()

        lhs_v[...] = _pack(jnp.concatenate([mem0_v[...].astype(F32), ln1(x_v[0, 0:24, :])], axis=0))
        dst = wqkv.at[pl.ds(pl.multiple_of(gn * (16 * PITCH) + (u & 1) * 256, 8), 16 * PITCH + 256), :]
        view = wqkv.at[pl.ds(pl.multiple_of(u * (8 * PITCH), 8), 8 * PITCH), :]
        for p in range(4):
            for mc in range(4):
                lhs = _unpack(jnp.concatenate(
                    [h3_v[kt, :, mc * 128:(mc + 1) * 128] for kt in range(8)], axis=1))
                store_x3(qkv3.at[2 * u + p // 2], p % 2, mc, _dot(lhs, wpair(view, 2 * p)))
                relayout(src, dst, 16 * (4 * p + mc), 16 * (4 * p + mc + 1))
                if mc == 1:
                    modr_v[4 * (u - 4) + p] = _dot(_unpack(sc_v[...]), wcol(wm, p))[0:8]
                if p % 2 == 0:
                    store_x3(qkv3.at[u - 4], p // 2, mc,
                             acc_v[2 * (u - 4) + p // 2, mc * 128:(mc + 1) * 128, :])
        return carry

    jax.lax.fori_loop(4, 12, unit_body, 0)

    for cp in wo_copies():
        cp.wait()
    for j in range(32):
        mod_v[:, 2 * D + j * 128:2 * D + (j + 1) * 128] = modr_v[j]

    zpad = jnp.zeros((24, DH), U32)

    def proj(gg, mat):
        y = None
        for kt in range(0, 8, 2):
            w = jnp.concatenate(
                [_unpack(wqkv[pl.ds((mat * H + 4 * gg + i) * PITCH + 64 * kt, 128), :])
                 for i in range(4)], axis=1)
            d = _dot(_unpack(lhs_v[:, kt * 128:(kt + 2) * 128]), w)
            y = d if y is None else y + d
        for i in range(4):
            cs = pl.ds(((2 * gg + i // 2) * 3 + mat) * DH, DH)
            qkv_s[16 * (i % 2):16 * (i % 2 + 1), cs] = _pack(y[:, i * DH:(i + 1) * DH])

    def get(g, mat, seg):
        u3, p3 = divmod(mat * NPAIR + g, 2)
        parts = [qkv_s[:, pl.ds((g * 3 + mat) * DH, DH)],
                 qkv3[u3, pl.ds(mo(seg * 8, 8), 8), p3 * DH:(p3 + 1) * DH]]
        if mat > 0:
            parts.append(zpad)
        return _unpack(jnp.concatenate(parts, axis=0))

    def scores(g, seg):
        s = _dot_nt(get(g, 0, seg), get(g, 1, seg)) * SCALE
        code = code_v[...]
        s = jnp.where(code == 0.0, s, code)
        e = jnp.exp(s - jnp.max(s, axis=-1, keepdims=True))
        l = jnp.sum(e, axis=-1, keepdims=True)
        p_s[:, pl.ds(g * DH, DH)] = _pack(e * (1.0 / l))

    def pv(g, seg, second):
        o = _dot(_unpack(p_s[:, pl.ds(g * DH, DH)]), get(g, 2, seg))
        c0, c1 = (h * DH for h in _pair_heads(g))
        obuf[0:16, c0:c0 + DH] = _pack(o[0:32])
        obuf[0:16, c1:c1 + DH] = _pack(o[32:64])
        if not second:
            o3a[:, c0:c0 + DH] = o[64:72]
            o3a[:, c1:c1 + DH] = o[72:80]
        else:
            obuf[16:24, c0:c0 + DH] = _pack(jnp.concatenate([o3a[:, c0:c0 + DH], o[64:72]], axis=0))
            obuf[16:24, c1:c1 + DH] = _pack(jnp.concatenate([o3a[:, c1:c1 + DH], o[72:80]], axis=0))

    def wo_cols(pairs):
        return sorted(h for g in pairs for h in _pair_heads(g))

    def wo_dot(j, heads, nrow):
        lhs = jnp.concatenate([obuf[0:nrow, h * DH:(h + 1) * DH] for h in heads], axis=1)
        wu = wo_v.at[j].bitcast(U32)
        w = jnp.concatenate([wu[h * 64:(h + 1) * 64, :] for h in heads], axis=0)
        return _dot(_unpack(lhs), _unpack(w))

    def next_rows(seg):
        z = pl.multiple_of(zero_s[0], 8)
        obuf[pl.ds(24 + z, 24), 0:D] = pltpu.bitcast(ln1(x_v[seg, 0:24, :]), U32)

    def step(seg, second, fillers):
        part = functools.partial
        nrow = 24 if second else 16
        wsplit = 0 if fillers else WSPLIT0
        early, late = wo_cols(range(NPAIR - wsplit)), wo_cols(range(NPAIR - wsplit, NPAIR))

        def wo_early(j):
            wacc[0:2 * nrow, j * 128:(j + 1) * 128] = wo_dot(j, early, nrow)

        def wo_final(j):
            cs = slice(j * 128, (j + 1) * 128)
            if wsplit:
                y = wacc[0:2 * nrow, cs] + wo_dot(j, late, nrow)
            else:
                y = wo_dot(j, early, nrow)
            hn = pltpu.bitcast(obuf[24:48, cs], F32)
            lhs_v[:, cs] = _pack(jnp.concatenate([y[0:8], hn], axis=0))
            ga = mod_v[0:1, 2 * D + j * 128:2 * D + (j + 1) * 128]
            res = lambda sg, r0, n, yy: x_v[sg, r0:r0 + n, cs].astype(F32) + ga * yy
            if not second:
                x1n_v[0:24, cs] = res(seg, 0, 24, y[8:32])
            else:
                x1n_v[32:56, cs] = res(seg, 0, 24, y[8:32])
                x1n_v[24:32, cs] = res(seg - 1, 24, 8, y[32:40])
                x1n_v[56:64, cs] = res(seg, 24, 8, y[40:48])

        ev = list(fillers)
        for gg in range(NPAIR // 2):
            ev += [(2 * gg + 0.66 * mat, part(proj, gg, mat)) for mat in range(3)]
        for g in range(NPAIR):
            ev.append((SCORE_KEYS[second][g] if fillers else g + SOFF0, part(scores, g, seg)))
            ev.append((PV_KEYS[second][g] if fillers else g + POFF0, part(pv, g, seg, second)))
        ev.append((NEXT_KEYS[second] if fillers else NEXT0,
                   part(next_rows, jnp.minimum(seg + 1, NSEG - 1))))
        if wsplit:
            ev += [(WEARLY0[j], part(wo_early, j)) for j in range(8)]
        ev += [(100 + j, part(wo_final, j)) for j in range(8)]
        ev.sort(key=lambda e: e[0])
        for _, f in ev:
            f()

    def ffn_pre():
        x1 = x1n_v[...]
        x1_v[...] = x1
        h2_v[...] = _pack(_ln(x1) * (1.0 + modrow(4)) + modrow(3))

    def ffn1(j):
        cs = slice(j * 128, (j + 1) * 128)
        y = _dot(_unpack(h2_v[...]), wcol(w1_v, j)) + bias_v[0:1, cs]
        g_v[:, cs] = _pack(jax.nn.gelu(y, approximate=True))

    def ffn2(tp, j):
        cs = slice(j * 128, (j + 1) * 128)
        y = _dot(_unpack(g_v[...]), wcol(w2_v, j)) + bias_v[0:1, FF + j * 128:FF + (j + 1) * 128]
        o = x1_v[:, cs] + mod_v[0:1, 5 * D + j * 128:5 * D + (j + 1) * 128] * y
        out_v[tp, :, cs] = o.astype(BF16)

    step(0, False, [])
    step(1, True, [])
    for cp in w1_copies() + w2_copies():
        cp.wait()

    def body(t, carry):
        @pl.when(t == 2)
        def _():
            x_copy(2).wait()

        ffn_pre()
        step(2 * t, False, [(k, functools.partial(ffn1, j)) for j, k in enumerate(FFN1_KEYS)])
        step(2 * t + 1, True,
             [(k, functools.partial(ffn2, t - 1, j)) for j, k in enumerate(FFN2_KEYS)])
        pltpu.make_async_copy(out_v.at[t - 1], out_hbm.at[t - 1], sem_out.at[0]).start()
        return carry

    jax.lax.fori_loop(1, NDS, body, 0)

    ffn_pre()
    for j in range(FF // 128):
        ffn1(j)
    for lo, hi in [(0, 7), (7, 8)]:
        for j in range(lo, hi):
            ffn2(NDS - 1, j)
        cols = pl.ds(lo * 128, (hi - lo) * 128)
        pltpu.make_async_copy(out_v.at[NDS - 1, :, cols], out_hbm.at[NDS - 1, :, cols],
                              sem_out.at[0]).start()
    pltpu.make_async_copy(out_v, out_hbm, sem_out.at[0]).wait()


@jax.jit
def pallas_adaLN_cond__memory_aug_recurrent_mem_tr__dense_activation_gelu__prompt_kernel(
    A_x, A_mem0, A_Wq, A_Wk, A_Wv, A_Wo, A_seg_len, B_x, B_w1, B_b1, B_w2, B_b2, c, w_mod,
):
    del A_seg_len, B_x
    assert A_x.shape == (1, S, D) and A_mem0.shape == (1, M, D)
    assert A_Wq.shape == (D, H, DH) and B_w1.shape == (D, FF)
    any_spec = pl.BlockSpec(memory_space=pl.ANY)
    scratch = [
        pltpu.VMEM((NSEG, SEG, D), BF16),
        pltpu.VMEM((NSEG // 2, 2 * SEG, D), BF16),
        pltpu.VMEM((NSTAGE, D, 16, DH), BF16),
        pltpu.VMEM(((3 * H + 1) * PITCH, DH), U32),
        pltpu.VMEM((8, H * DH, 128), BF16),
        pltpu.VMEM((FF // 128, D, 128), BF16),
        pltpu.VMEM((8, FF, 128), BF16),
        pltpu.VMEM((16, D, 128), BF16),
        pltpu.VMEM((32, D, 128), BF16),
        pltpu.VMEM((M, D), BF16),
        pltpu.VMEM((FF,), BF16),
        pltpu.VMEM((D,), BF16),
        pltpu.VMEM((1, D), BF16),
        pltpu.VMEM((8, 6 * D), F32),
        pltpu.VMEM((16, 8, 128), F32),
        pltpu.VMEM((32, 8, 128), F32),
        pltpu.VMEM((8, D), U32),
        pltpu.VMEM((8, FF + D), F32),
        pltpu.VMEM((8, NSEG * 8, 128), F32),
        pltpu.VMEM((9, 64, 512), U32),
        pltpu.VMEM((NPAIR, NSEG * 8, 2 * DH), F32),
        pltpu.VMEM((24, NSEG * 8, 2 * DH), U32),
        pltpu.VMEM((80, 128), F32),
        pltpu.VMEM((16, D), U32),
        pltpu.VMEM((32, NPAIR * 3 * DH), U32),
        pltpu.VMEM((40, NPAIR * DH), U32),
        pltpu.VMEM((48, D), F32),
        pltpu.VMEM((48, H * DH), U32),
        pltpu.VMEM((8, H * DH), F32),
        pltpu.VMEM((64, D), F32),
        pltpu.VMEM((64, D), F32),
        pltpu.VMEM((32, D), U32),
        pltpu.VMEM((32, FF), U32),
        pltpu.SMEM((1,), jnp.int32),
        pltpu.SemaphoreType.DMA((4,)),
        pltpu.SemaphoreType.DMA((3,)),
        pltpu.SemaphoreType.DMA((17,)),
        pltpu.SemaphoreType.DMA((8,)),
        pltpu.SemaphoreType.DMA((3,)),
        pltpu.SemaphoreType.DMA((1,)),
    ]
    out = pl.pallas_call(
        _kernel,
        out_shape=jax.ShapeDtypeStruct((NSEG // 2, 2 * SEG, D), BF16),
        in_specs=[any_spec] * 12,
        out_specs=any_spec,
        scratch_shapes=scratch,
        compiler_params=pltpu.CompilerParams(vmem_limit_bytes=120 * 1024 * 1024,
                                             disable_bounds_checks=not CHECKS,
                                             disable_semaphore_checks=not CHECKS),
    )(
        A_x.reshape(NSEG, SEG, D), A_mem0.reshape(M, D), A_Wq, A_Wk, A_Wv,
        A_Wo.reshape(H * DH, D), B_w1, B_b1, B_w2, B_b2,
        c, w_mod,
    )
    return out.reshape(1, S, D)
```

```python
import functools

import jax
import jax.numpy as jnp
import jax.experimental.pallas as pl
import jax.experimental.pallas.tpu as pltpu

F32 = jnp.float32
BF16 = jnp.bfloat16
U32 = jnp.uint32

S = 2048
D = 1024
H = 32
DH = 128
M = 8
SEG = 32
NSEG = S // SEG
FF = 3584
NPAIR = H // 2
PITCH = 516
XA = 8
NSTAGE = 4
NDS = NSEG // 2
FFN1_KEYS = [20 + j for j in range(FF // 128)]
FFN2_KEYS = [20 + 4 * j for j in range(D // 128 - 1)]
HELD_KEY = 19.0
SCORE_KEYS = [[20.5 + 1.3 * g for g in range(NPAIR)],
              [20.5 + 4 * (g * 5 // 16) + 0.1 * g for g in range(NPAIR)]]
PV_KEYS = [[25.6 + 1.3 * g for g in range(NPAIR)],
           [27.0 + 4 * (g * 5 // 16) + 0.01 * g for g in range(NPAIR)]]
NEXT_KEYS = [47.5, 43.9]
SOFF0, POFF0, NEXT0, WSPLIT0 = 2.1, 4.2, 10, 5
WEARLY0 = [16.0 + 0.5 * j for j in range(8)]
CHECKS = False
EPS = 1e-5
SCALE = DH ** (-0.5)


def _pair_heads(gp):
    half, r = divmod(gp, 8)
    par, i = divmod(r, 4)
    h0 = 16 * half + 4 * i + par
    return h0, h0 + 2


def _ln(xf):
    m = jnp.mean(xf, axis=-1, keepdims=True)
    xc = xf - m
    v = jnp.mean(xc * xc, axis=-1, keepdims=True)
    return xc * jax.lax.rsqrt(v + EPS)


def _dot(a, b):
    return jnp.dot(a, b, preferred_element_type=F32)


def _dot_nt(a, b):
    return jax.lax.dot_general(a, b, (((1,), (1,)), ((), ())), preferred_element_type=F32)


def _pack(xf):
    return pltpu.bitcast(xf.astype(BF16), U32)


def _unpack(u):
    return pltpu.bitcast(u, BF16)


def _kernel(x_hbm, mem0_hbm, wq_hbm, wk_hbm, wv_hbm, wo_hbm, w1_hbm, b1_hbm, w2_hbm, b2_hbm,
            c_hbm, wmod_hbm,
            out_hbm,
            x_v, out_v, stage, wqkv, wo_v, w1_v, w2_v, wm0_v, wm1_v,
            mem0_v, b1_v, b2_v, c_v,
            mod_v, modq_v, modr_v, sc_v, bias_v, xh_v, h3_v, acc_v, qkv3, code_v,
            lhs_v, qkv_s, p_s, wacc, obuf, o3a, x1n_v, x1_v, h2_v, g_v, zero_s,
            sem_small, sem_x, sem_q, sem_u, sem_w, sem_out):
    w_hbms = (wq_hbm, wk_hbm, wv_hbm)

    def mo(i, n):
        return i if isinstance(i, int) else pl.multiple_of(i, n)

    def small_copies():
        return [pltpu.make_async_copy(c_hbm, c_v, sem_small.at[0]),
                pltpu.make_async_copy(mem0_hbm, mem0_v, sem_small.at[1]),
                pltpu.make_async_copy(b1_hbm, b1_v, sem_small.at[2]),
                pltpu.make_async_copy(b2_hbm, b2_v, sem_small.at[3])]

    def x_copy(part):
        s0, ns, lo, n = [(0, NSEG, 24, 8), (0, XA, 0, 24), (XA, NSEG - XA, 0, 24)][part]
        return pltpu.make_async_copy(x_hbm.at[pl.ds(s0, ns), pl.ds(lo, n), :],
                                     x_v.at[pl.ds(s0, ns), pl.ds(lo, n), :], sem_x.at[part])

    def wq_chunk_copy(j, sem):
        d0 = mo((j >> 1) * 128, 128)
        hf = j & 1
        return pltpu.make_async_copy(wq_hbm.at[pl.ds(d0, 128), pl.ds(mo(16 * hf, 16), 16), :],
                                     stage.at[hf, pl.ds(d0, 128)], sem)

    def wm0_copy(i, sem):
        c0 = mo((i & 1) * D + (i >> 1) * 128, 128)
        return pltpu.make_async_copy(wmod_hbm.at[:, pl.ds(c0, 128)], wm0_v.at[i], sem)

    def g2_piece_copy(j, sem):
        d0 = mo(j * 64, 64)
        return pltpu.make_async_copy(wk_hbm.at[pl.ds(d0, 64), pl.ds(0, 16), :],
                                     stage.at[2, pl.ds(d0, 64)], sem)

    def unit_copies(u):
        cps = [pltpu.make_async_copy(wmod_hbm.at[:, pl.ds(2 * D + j * 128, 128)], wm1_v.at[j],
                                     sem_u.at[u - 4]) for j in range(4 * (u - 4), 4 * (u - 3))]
        if u < 10:
            grp = u // 2 + 1
            mat, half = divmod(grp, 2)
            rows = pl.ds((u % 2) * 512, 512)
            cps.append(pltpu.make_async_copy(w_hbms[mat].at[rows, pl.ds(16 * half, 16), :],
                                             stage.at[grp % NSTAGE, rows], sem_u.at[u - 4]))
        return cps

    def slab_copies(src, dst, sem):
        return [pltpu.make_async_copy(src.at[:, pl.ds(j * 128, 128)], dst.at[j], sem)
                for j in range(dst.shape[0])]

    wo_copies = lambda: slab_copies(wo_hbm, wo_v, sem_w.at[0])
    w1_copies = lambda: slab_copies(w1_hbm, w1_v, sem_w.at[1])
    w2_copies = lambda: slab_copies(w2_hbm, w2_v, sem_w.at[2])

    def wcol(ref, j):
        return _unpack(ref.at[j].bitcast(U32)[...])

    def relayout(src, dst, j0, j1):
        srcu = src.bitcast(U32)
        for j in range(j0, j1):
            a = srcu[2 * j]
            b = srcu[2 * j + 1]
            dst[pl.ds(j, 8, stride=PITCH), :] = (a & jnp.uint32(0xFFFF)) | (b << 16)
            dst[pl.ds(8 * PITCH + j, 8, stride=PITCH), :] = (a >> 16) | (b & jnp.uint32(0xFFFF0000))

    def wpair(ref, slab0, n=D // 2):
        return jnp.concatenate([_unpack(ref[pl.ds(slab0 * PITCH, n), :]),
                                _unpack(ref[pl.ds((slab0 + 1) * PITCH, n), :])], axis=1)

    def modrow(i):
        return mod_v[0:1, i * D:(i + 1) * D]

    def first_copies():
        return [wm0_copy(i, sem_q.at[16]) for i in range(2)] + [wq_chunk_copy(0, sem_q.at[16])]

    def q_copies(j, do):
        @pl.when(j > 0)
        def _():
            do(g2_piece_copy(j - 1, sem_q.at[j]))

        @pl.when(j == 15)
        def _():
            do(g2_piece_copy(15, sem_q.at[j]))

        @pl.when(j < 15)
        def _():
            do(wq_chunk_copy(j + 1, sem_q.at[j]))

        @pl.when(j < 14)
        def _():
            do(wm0_copy(j + 2, sem_q.at[j]))

    def issue(i, carry):
        @pl.when(i == 0)
        def _():
            for cp in small_copies():
                cp.start()
            x_copy(0).start()

        @pl.when(i == 1)
        def _():
            for cp in first_copies():
                cp.start()

        @pl.when(jnp.logical_and(i >= 2, i < 18))
        def _():
            q_copies(i - 2, lambda cp: cp.start())

        @pl.when(i == 18)
        def _():
            for cp in unit_copies(4) + [x_copy(1)]:
                cp.start()

        @pl.when(i == 19)
        def _():
            for cp in unit_copies(5):
                cp.start()
        return carry

    jax.lax.fori_loop(0, 20, issue, 0)
    zero_s[0] = 0
    g_v[...] = jnp.zeros(g_v.shape, U32)
    x1_v[...] = jnp.zeros(x1_v.shape, F32)

    ri = jax.lax.broadcasted_iota(jnp.int32, (80, 128), 0)
    ci = jax.lax.broadcasted_iota(jnp.int32, (80, 128), 1)

    def head_of(i):
        return jnp.where(i < 64, i // 32, (i - 64) // 8)

    def pos_of(i):
        return jnp.where(i < 64, i % 32, 32 + (i - 64) % 8)

    same = head_of(ri) == head_of(ci)
    pr, pc = pos_of(ri), pos_of(ci)
    keep = jnp.logical_or(pr < M, pr >= pc)
    code_v[...] = jnp.where(same, jnp.where(keep, 0.0, -1e9), -jnp.inf).astype(F32)

    for cp in small_copies():
        cp.wait()
    cf = c_v[...].astype(F32)
    sc_v[...] = _pack(jnp.broadcast_to(cf * jax.nn.sigmoid(cf), (16, D)))
    bias_v[:, 0:FF] = jnp.broadcast_to(b1_v[...].astype(F32).reshape(1, FF), (8, FF))
    bias_v[:, FF:] = jnp.broadcast_to(b2_v[...].astype(F32).reshape(1, D), (8, D))

    x_copy(0).wait()

    def xh_body(i, carry):
        for h in range(2):
            s0 = pl.multiple_of((i * 2 + h) * 8, 8)
            xh = _ln(x_v[pl.ds(s0, 8), 24:32, :].astype(F32).reshape(64, D))
            r0 = pl.multiple_of((i * 2 + h) * 64, 64)
            for kt in range(8):
                xh_v[kt, pl.ds(r0, 64), :] = xh[:, kt * 128:(kt + 1) * 128]
        return carry

    jax.lax.fori_loop(0, 4, xh_body, 0)

    def mod_slab(i):
        modq_v[i] = _dot(_unpack(sc_v[...]), wcol(wm0_v, i))[0:8]

    def h3_store(dst, kt, mc):
        sa = modq_v[2 * kt, 0:1, :]
        ca = modq_v[2 * kt + 1, 0:1, :]
        dst[:, mc * 128:(mc + 1) * 128] = _pack(
            xh_v[kt, mc * 128:(mc + 1) * 128, :] * (1.0 + ca) + sa)

    for cp in first_copies():
        cp.wait()
    modq_v[2:16] = jnp.zeros((14, 8, 128), F32)
    for i in range(2):
        mod_slab(i)
    for mc in range(4):
        h3_store(h3_v.at[0], 0, mc)
    relayout(stage.at[0, pl.ds(0, 128)], wqkv, 0, 64)

    def q_body(j, carry):
        q_copies(j, lambda cp: cp.wait())
        kt, hf = j >> 1, j & 1
        ktn = jnp.minimum(j + 1, 15) >> 1
        hfn = jnp.where(j < 15, (j + 1) & 1, 2)
        hview = h3_v.at[pl.ds(kt, 2)]
        wview = wqkv.at[pl.ds(pl.multiple_of(hf * (16 * PITCH) + kt * 64, 8), 16 * PITCH - 448), :]
        aview = acc_v.at[pl.ds(pl.multiple_of(hf * 8, 8), 8)]
        qsrc = stage.at[hfn, pl.ds(pl.multiple_of(ktn * 128, 128), 128)]
        qdst = wqkv.at[pl.ds(pl.multiple_of(hfn * (16 * PITCH) + ktn * 64, 8), 16 * PITCH + 64), :]
        jk = jnp.maximum(j - 1, 0)
        ksrc = stage.at[jnp.where(j > 0, 2, 0), pl.ds(pl.multiple_of(jk * 64, 64), 64)]
        kdst = wqkv.at[pl.ds(pl.multiple_of(32 * PITCH + jk * 32, 8), 16 * PITCH + 32), :]
        for p in range(8):
            lhs = jnp.concatenate([hview[0, :, mc * 128:(mc + 1) * 128] for mc in range(4)], axis=0)
            y = _dot(_unpack(lhs), wpair(wview, 2 * p, 64))
            aview[p] = jnp.where(kt > 0, aview[p], 0.0) + y
            if p == 1:
                mod_slab(jnp.minimum(j + 2, 15))
            if p >= 4:
                h3_store(hview.at[1], jnp.minimum(kt + 1, 7), p - 4)
            if p % 2 == 1:
                relayout(qsrc, qdst, 8 * p - 8, 8 * p + 8)
                relayout(ksrc, kdst, 4 * p - 4, 4 * p + 4)
        return carry

    jax.lax.fori_loop(0, 16, q_body, 0)
    for kt in range(8):
        mod_v[:, kt * 128:(kt + 1) * 128] = modq_v[2 * kt]
        mod_v[:, D + kt * 128:D + (kt + 1) * 128] = modq_v[2 * kt + 1]
    for cp in unit_copies(6):
        cp.start()
    x_copy(1).wait()

    def ln1(xb):
        return _ln(xb.astype(F32)) * (1.0 + modrow(1)) + modrow(0)

    def store_x3(dst, half, mc, y):
        y = y.reshape(16, 8, 256)
        y = jnp.concatenate([y[:, :, :128], y[:, :, 128:]], axis=1).reshape(256, DH)
        dst[mc * 128:(mc + 1) * 128, half * DH:(half + 1) * DH] = _pack(y)

    def unit_body(u, carry):
        gn = jnp.minimum((u >> 1) + 1, 5)
        src = stage.at[gn & (NSTAGE - 1), pl.ds(pl.multiple_of((u & 1) * 512, 512), 512)]
        wm = wm1_v.at[pl.ds(4 * (u - 4), 4)]
        pltpu.make_async_copy(wm, wm, sem_u.at[u - 4]).wait()

        @pl.when(u < 10)
        def _():
            pltpu.make_async_copy(src, src, sem_u.at[u - 4]).wait()

        for k, cps in [(7, w1_copies), (4, lambda: unit_copies(7) + unit_copies(8)),
                       (5, lambda: unit_copies(9) + unit_copies(10) + unit_copies(11)),
                       (6, wo_copies), (8, w2_copies), (9, lambda: [x_copy(2)])]:
            @pl.when(u == k)
            def _(cps=cps):
                for cp in cps():
                    cp.start()

        lhs_v[...] = _pack(jnp.concatenate([mem0_v[...].astype(F32), ln1(x_v[0, 0:24, :])], axis=0))
        dst = wqkv.at[pl.ds(pl.multiple_of(gn * (16 * PITCH) + (u & 1) * 256, 8), 16 * PITCH + 256), :]
        view = wqkv.at[pl.ds(pl.multiple_of(u * (8 * PITCH), 8), 8 * PITCH), :]
        for p in range(4):
            for mc in range(4):
                lhs = _unpack(jnp.concatenate(
                    [h3_v[kt, :, mc * 128:(mc + 1) * 128] for kt in range(8)], axis=1))
                store_x3(qkv3.at[2 * u + p // 2], p % 2, mc, _dot(lhs, wpair(view, 2 * p)))
                relayout(src, dst, 16 * (4 * p + mc), 16 * (4 * p + mc + 1))
                if mc == 1:
                    modr_v[4 * (u - 4) + p] = _dot(_unpack(sc_v[...]), wcol(wm, p))[0:8]
                if p % 2 == 0:
                    store_x3(qkv3.at[u - 4], p // 2, mc,
                             acc_v[2 * (u - 4) + p // 2, mc * 128:(mc + 1) * 128, :])
        return carry

    jax.lax.fori_loop(4, 12, unit_body, 0)

    for cp in wo_copies():
        cp.wait()
    for j in range(32):
        mod_v[:, 2 * D + j * 128:2 * D + (j + 1) * 128] = modr_v[j]

    zpad = jnp.zeros((24, DH), U32)

    def proj(gg, mat):
        y = None
        for kt in range(0, 8, 2):
            w = jnp.concatenate(
                [_unpack(wqkv[pl.ds((mat * H + 4 * gg + i) * PITCH + 64 * kt, 128), :])
                 for i in range(4)], axis=1)
            d = _dot(_unpack(lhs_v[:, kt * 128:(kt + 2) * 128]), w)
            y = d if y is None else y + d
        for i in range(4):
            cs = pl.ds(((2 * gg + i // 2) * 3 + mat) * DH, DH)
            qkv_s[16 * (i % 2):16 * (i % 2 + 1), cs] = _pack(y[:, i * DH:(i + 1) * DH])

    def get(g, mat, seg):
        u3, p3 = divmod(mat * NPAIR + g, 2)
        parts = [qkv_s[:, pl.ds((g * 3 + mat) * DH, DH)],
                 qkv3[u3, pl.ds(mo(seg * 8, 8), 8), p3 * DH:(p3 + 1) * DH]]
        if mat > 0:
            parts.append(zpad)
        return _unpack(jnp.concatenate(parts, axis=0))

    def scores(g, seg):
        s = _dot_nt(get(g, 0, seg), get(g, 1, seg)) * SCALE
        code = code_v[...]
        s = jnp.where(code == 0.0, s, code)
        e = jnp.exp(s - jnp.max(s, axis=-1, keepdims=True))
        l = jnp.sum(e, axis=-1, keepdims=True)
        p_s[:, pl.ds(g * DH, DH)] = _pack(e * (1.0 / l))

    def pv(g, seg, second):
        o = _dot(_unpack(p_s[:, pl.ds(g * DH, DH)]), get(g, 2, seg))
        c0, c1 = (h * DH for h in _pair_heads(g))
        obuf[0:16, c0:c0 + DH] = _pack(o[0:32])
        obuf[0:16, c1:c1 + DH] = _pack(o[32:64])
        if not second:
            o3a[:, c0:c0 + DH] = o[64:72]
            o3a[:, c1:c1 + DH] = o[72:80]
        else:
            obuf[16:24, c0:c0 + DH] = _pack(jnp.concatenate([o3a[:, c0:c0 + DH], o[64:72]], axis=0))
            obuf[16:24, c1:c1 + DH] = _pack(jnp.concatenate([o3a[:, c1:c1 + DH], o[72:80]], axis=0))

    def wo_cols(pairs):
        return sorted(h for g in pairs for h in _pair_heads(g))

    def wo_dot(j, heads, nrow):
        lhs = jnp.concatenate([obuf[0:nrow, h * DH:(h + 1) * DH] for h in heads], axis=1)
        wu = wo_v.at[j].bitcast(U32)
        w = jnp.concatenate([wu[h * 64:(h + 1) * 64, :] for h in heads], axis=0)
        return _dot(_unpack(lhs), _unpack(w))

    def next_rows(seg):
        z = pl.multiple_of(zero_s[0], 8)
        obuf[pl.ds(24 + z, 24), 0:D] = pltpu.bitcast(ln1(x_v[seg, 0:24, :]), U32)

    def step(seg, second, fillers):
        part = functools.partial
        nrow = 24 if second else 16
        wsplit = 0 if fillers else WSPLIT0
        early, late = wo_cols(range(NPAIR - wsplit)), wo_cols(range(NPAIR - wsplit, NPAIR))

        def wo_early(j):
            wacc[0:2 * nrow, j * 128:(j + 1) * 128] = wo_dot(j, early, nrow)

        def wo_final(j):
            cs = slice(j * 128, (j + 1) * 128)
            if wsplit:
                y = wacc[0:2 * nrow, cs] + wo_dot(j, late, nrow)
            else:
                y = wo_dot(j, early, nrow)
            hn = pltpu.bitcast(obuf[24:48, cs], F32)
            lhs_v[:, cs] = _pack(jnp.concatenate([y[0:8], hn], axis=0))
            ga = mod_v[0:1, 2 * D + j * 128:2 * D + (j + 1) * 128]
            res = lambda sg, r0, n, yy: x_v[sg, r0:r0 + n, cs].astype(F32) + ga * yy
            if not second:
                x1n_v[0:24, cs] = res(seg, 0, 24, y[8:32])
            else:
                x1n_v[32:56, cs] = res(seg, 0, 24, y[8:32])
                x1n_v[24:32, cs] = res(seg - 1, 24, 8, y[32:40])
                x1n_v[56:64, cs] = res(seg, 24, 8, y[40:48])

        ev = list(fillers)
        for gg in range(NPAIR // 2):
            ev += [(2 * gg + 0.66 * mat, part(proj, gg, mat)) for mat in range(3)]
        for g in range(NPAIR):
            ev.append((SCORE_KEYS[second][g] if fillers else g + SOFF0, part(scores, g, seg)))
            ev.append((PV_KEYS[second][g] if fillers else g + POFF0, part(pv, g, seg, second)))
        ev.append((NEXT_KEYS[second] if fillers else NEXT0,
                   part(next_rows, jnp.minimum(seg + 1, NSEG - 1))))
        if wsplit:
            ev += [(WEARLY0[j], part(wo_early, j)) for j in range(8)]
        ev += [(100 + j, part(wo_final, j)) for j in range(8)]
        ev.sort(key=lambda e: e[0])
        for _, f in ev:
            f()

    def ffn_pre():
        x1 = x1n_v[...]
        x1_v[...] = x1
        h2_v[...] = _pack(_ln(x1) * (1.0 + modrow(4)) + modrow(3))

    def ffn1(j):
        cs = slice(j * 128, (j + 1) * 128)
        y = _dot(_unpack(h2_v[...]), wcol(w1_v, j)) + bias_v[0:1, cs]
        g_v[:, cs] = _pack(jax.nn.gelu(y, approximate=True))

    def ffn2(tp, j):
        cs = slice(j * 128, (j + 1) * 128)
        y = _dot(_unpack(g_v[...]), wcol(w2_v, j)) + bias_v[0:1, FF + j * 128:FF + (j + 1) * 128]
        o = x1_v[:, cs] + mod_v[0:1, 5 * D + j * 128:5 * D + (j + 1) * 128] * y
        out_v[tp, :, cs] = o.astype(BF16)

    step(0, False, [])
    step(1, True, [])
    for cp in w1_copies() + w2_copies():
        cp.wait()

    def body(t, carry):
        @pl.when(t == 2)
        def _():
            x_copy(2).wait()

        part = functools.partial
        held = [(HELD_KEY, part(ffn2, jnp.maximum(t - 2, 0), 7)), (HELD_KEY + 0.01, ffn_pre)]
        step(2 * t, False, held + [(k, part(ffn1, j)) for j, k in enumerate(FFN1_KEYS)])
        step(2 * t + 1, True, [(k, part(ffn2, t - 1, j)) for j, k in enumerate(FFN2_KEYS)])

        @pl.when(t >= 2)
        def _():
            pltpu.make_async_copy(out_v.at[t - 2], out_hbm.at[t - 2], sem_out.at[0]).start()
        return carry

    jax.lax.fori_loop(1, NDS, body, 0)

    ffn2(NDS - 2, 7)
    pltpu.make_async_copy(out_v.at[NDS - 2], out_hbm.at[NDS - 2], sem_out.at[0]).start()
    ffn_pre()
    for j in range(FF // 128):
        ffn1(j)
    for lo, hi in [(0, 7), (7, 8)]:
        for j in range(lo, hi):
            ffn2(NDS - 1, j)
        cols = pl.ds(lo * 128, (hi - lo) * 128)
        pltpu.make_async_copy(out_v.at[NDS - 1, :, cols], out_hbm.at[NDS - 1, :, cols],
                              sem_out.at[0]).start()
    pltpu.make_async_copy(out_v, out_hbm, sem_out.at[0]).wait()


@jax.jit
def pallas_adaLN_cond__memory_aug_recurrent_mem_tr__dense_activation_gelu__prompt_kernel(
    A_x, A_mem0, A_Wq, A_Wk, A_Wv, A_Wo, A_seg_len, B_x, B_w1, B_b1, B_w2, B_b2, c, w_mod,
):
    del A_seg_len, B_x
    assert A_x.shape == (1, S, D) and A_mem0.shape == (1, M, D)
    assert A_Wq.shape == (D, H, DH) and B_w1.shape == (D, FF)
    any_spec = pl.BlockSpec(memory_space=pl.ANY)
    scratch = [
        pltpu.VMEM((NSEG, SEG, D), BF16),
        pltpu.VMEM((NSEG // 2, 2 * SEG, D), BF16),
        pltpu.VMEM((NSTAGE, D, 16, DH), BF16),
        pltpu.VMEM(((3 * H + 1) * PITCH, DH), U32),
        pltpu.VMEM((8, H * DH, 128), BF16),
        pltpu.VMEM((FF // 128, D, 128), BF16),
        pltpu.VMEM((8, FF, 128), BF16),
        pltpu.VMEM((16, D, 128), BF16),
        pltpu.VMEM((32, D, 128), BF16),
        pltpu.VMEM((M, D), BF16),
        pltpu.VMEM((FF,), BF16),
        pltpu.VMEM((D,), BF16),
        pltpu.VMEM((1, D), BF16),
        pltpu.VMEM((8, 6 * D), F32),
        pltpu.VMEM((16, 8, 128), F32),
        pltpu.VMEM((32, 8, 128), F32),
        pltpu.VMEM((8, D), U32),
        pltpu.VMEM((8, FF + D), F32),
        pltpu.VMEM((8, NSEG * 8, 128), F32),
        pltpu.VMEM((9, 64, 512), U32),
        pltpu.VMEM((NPAIR, NSEG * 8, 2 * DH), F32),
        pltpu.VMEM((24, NSEG * 8, 2 * DH), U32),
        pltpu.VMEM((80, 128), F32),
        pltpu.VMEM((16, D), U32),
        pltpu.VMEM((32, NPAIR * 3 * DH), U32),
        pltpu.VMEM((40, NPAIR * DH), U32),
        pltpu.VMEM((48, D), F32),
        pltpu.VMEM((48, H * DH), U32),
        pltpu.VMEM((8, H * DH), F32),
        pltpu.VMEM((64, D), F32),
        pltpu.VMEM((64, D), F32),
        pltpu.VMEM((32, D), U32),
        pltpu.VMEM((32, FF), U32),
        pltpu.SMEM((1,), jnp.int32),
        pltpu.SemaphoreType.DMA((4,)),
        pltpu.SemaphoreType.DMA((3,)),
        pltpu.SemaphoreType.DMA((17,)),
        pltpu.SemaphoreType.DMA((8,)),
        pltpu.SemaphoreType.DMA((3,)),
        pltpu.SemaphoreType.DMA((1,)),
    ]
    out = pl.pallas_call(
        _kernel,
        out_shape=jax.ShapeDtypeStruct((NSEG // 2, 2 * SEG, D), BF16),
        in_specs=[any_spec] * 12,
        out_specs=any_spec,
        scratch_shapes=scratch,
        compiler_params=pltpu.CompilerParams(vmem_limit_bytes=120 * 1024 * 1024,
                                             disable_bounds_checks=not CHECKS,
                                             disable_semaphore_checks=not CHECKS),
    )(
        A_x.reshape(NSEG, SEG, D), A_mem0.reshape(M, D), A_Wq, A_Wk, A_Wv,
        A_Wo.reshape(H * DH, D), B_w1, B_b1, B_w2, B_b2,
        c, w_mod,
    )
    return out.reshape(1, S, D)
```

```python
import functools

import jax
import jax.numpy as jnp
import jax.experimental.pallas as pl
import jax.experimental.pallas.tpu as pltpu

F32 = jnp.float32
BF16 = jnp.bfloat16
U32 = jnp.uint32

S = 2048
D = 1024
H = 32
DH = 128
M = 8
SEG = 32
NSEG = S // SEG
FF = 3584
NPAIR = H // 2
PITCH = 516
XA = 8
NSTAGE = 4
NDS = NSEG // 2
FFN1_KEYS = [20 + j for j in range(FF // 128)]
FFN2_KEYS = [20 + 4 * j for j in range(D // 128 - 1)]
HELD_KEY = 19.0
SCORE_KEYS = [[20.5 + 1.3 * g for g in range(NPAIR)],
              [20.5 + 4 * (g * 5 // 16) + 0.1 * g for g in range(NPAIR)]]
PV_KEYS = [[25.6 + 1.3 * g for g in range(NPAIR)],
           [27.0 + 4 * (g * 5 // 16) + 0.01 * g for g in range(NPAIR)]]
NEXT_KEYS = [47.5, 43.9]
SOFF0, POFF0, NEXT0, WSPLIT0 = 2.1, 4.2, 10, 5
WEARLY0 = [16.0 + 0.5 * j for j in range(8)]
QREL = {3: ((0, 24), (0, 8)), 5: ((24, 44), (8, 20)), 7: ((44, 64), (20, 32))}
UREL = [0, 16, 16, 40, 64]
CHECKS = False
EPS = 1e-5
SCALE = DH ** (-0.5)


def _pair_heads(gp):
    half, r = divmod(gp, 8)
    par, i = divmod(r, 4)
    h0 = 16 * half + 4 * i + par
    return h0, h0 + 2


def _ln(xf):
    m = jnp.mean(xf, axis=-1, keepdims=True)
    xc = xf - m
    v = jnp.mean(xc * xc, axis=-1, keepdims=True)
    return xc * jax.lax.rsqrt(v + EPS)


def _dot(a, b):
    return jnp.dot(a, b, preferred_element_type=F32)


def _dot_nt(a, b):
    return jax.lax.dot_general(a, b, (((1,), (1,)), ((), ())), preferred_element_type=F32)


def _pack(xf):
    return pltpu.bitcast(xf.astype(BF16), U32)


def _unpack(u):
    return pltpu.bitcast(u, BF16)


def _kernel(x_hbm, mem0_hbm, wq_hbm, wk_hbm, wv_hbm, wo_hbm, w1_hbm, b1_hbm, w2_hbm, b2_hbm,
            c_hbm, wmod_hbm,
            out_hbm,
            x_v, out_v, stage, wqkv, wo_v, w1_v, w2_v, wm0_v, wm1_v,
            mem0_v, b1_v, b2_v, c_v,
            mod_v, modq_v, modr_v, sc_v, bias_v, xh_v, h3_v, acc_v, qkv3, code_v,
            lhs_v, qkv_s, p_s, wacc, obuf, o3a, x1n_v, x1_v, h2_v, g_v, zero_s,
            sem_small, sem_x, sem_q, sem_u, sem_w, sem_out):
    w_hbms = (wq_hbm, wk_hbm, wv_hbm)

    def mo(i, n):
        return i if isinstance(i, int) else pl.multiple_of(i, n)

    def small_copies():
        return [pltpu.make_async_copy(c_hbm, c_v, sem_small.at[0]),
                pltpu.make_async_copy(mem0_hbm, mem0_v, sem_small.at[1]),
                pltpu.make_async_copy(b1_hbm, b1_v, sem_small.at[2]),
                pltpu.make_async_copy(b2_hbm, b2_v, sem_small.at[3])]

    def x_copy(part):
        s0, ns, lo, n = [(0, NSEG, 24, 8), (0, XA, 0, 24), (XA, NSEG - XA, 0, 24)][part]
        return pltpu.make_async_copy(x_hbm.at[pl.ds(s0, ns), pl.ds(lo, n), :],
                                     x_v.at[pl.ds(s0, ns), pl.ds(lo, n), :], sem_x.at[part])

    def wq_chunk_copy(j, sem):
        d0 = mo((j >> 1) * 128, 128)
        hf = j & 1
        return pltpu.make_async_copy(wq_hbm.at[pl.ds(d0, 128), pl.ds(mo(16 * hf, 16), 16), :],
                                     stage.at[hf, pl.ds(d0, 128)], sem)

    def wm0_copy(i, sem):
        c0 = mo((i & 1) * D + (i >> 1) * 128, 128)
        return pltpu.make_async_copy(wmod_hbm.at[:, pl.ds(c0, 128)], wm0_v.at[i], sem)

    def g2_piece_copy(j, sem):
        d0 = mo(j * 64, 64)
        return pltpu.make_async_copy(wk_hbm.at[pl.ds(d0, 64), pl.ds(0, 16), :],
                                     stage.at[2, pl.ds(d0, 64)], sem)

    def unit_copies(u):
        cps = [pltpu.make_async_copy(wmod_hbm.at[:, pl.ds(2 * D + j * 128, 128)], wm1_v.at[j],
                                     sem_u.at[u - 4]) for j in range(4 * (u - 4), 4 * (u - 3))]
        if u < 10:
            grp = u // 2 + 1
            mat, half = divmod(grp, 2)
            rows = pl.ds((u % 2) * 512, 512)
            cps.append(pltpu.make_async_copy(w_hbms[mat].at[rows, pl.ds(16 * half, 16), :],
                                             stage.at[grp % NSTAGE, rows], sem_u.at[u + 4]))
        return cps

    def slab_copies(src, dst, sem):
        return [pltpu.make_async_copy(src.at[:, pl.ds(j * 128, 128)], dst.at[j], sem)
                for j in range(dst.shape[0])]

    wo_copies = lambda: slab_copies(wo_hbm, wo_v, sem_w.at[0])
    w1_copies = lambda: slab_copies(w1_hbm, w1_v, sem_w.at[1])
    w2_copies = lambda: slab_copies(w2_hbm, w2_v, sem_w.at[2])

    def wcol(ref, j):
        return _unpack(ref.at[j].bitcast(U32)[...])

    def relayout(src, dst, j0, j1):
        srcu = src.bitcast(U32)
        for j in range(j0, j1):
            a = srcu[2 * j]
            b = srcu[2 * j + 1]
            dst[pl.ds(j, 8, stride=PITCH), :] = (a & jnp.uint32(0xFFFF)) | (b << 16)
            dst[pl.ds(8 * PITCH + j, 8, stride=PITCH), :] = (a >> 16) | (b & jnp.uint32(0xFFFF0000))

    def wpair(ref, slab0, n=D // 2):
        return jnp.concatenate([_unpack(ref[pl.ds(slab0 * PITCH, n), :]),
                                _unpack(ref[pl.ds((slab0 + 1) * PITCH, n), :])], axis=1)

    def modrow(i):
        return mod_v[0:1, i * D:(i + 1) * D]

    def first_copies():
        return [wm0_copy(i, sem_q.at[16]) for i in range(2)] + [wq_chunk_copy(0, sem_q.at[16])]

    def q_copies(j, do):
        @pl.when(j > 0)
        def _():
            do(g2_piece_copy(j - 1, sem_q.at[j]))

        @pl.when(j == 15)
        def _():
            do(g2_piece_copy(15, sem_q.at[j]))

        @pl.when(j < 15)
        def _():
            do(wq_chunk_copy(j + 1, sem_q.at[j]))

        @pl.when(j < 14)
        def _():
            do(wm0_copy(j + 2, sem_q.at[j]))

    def issue(i, carry):
        @pl.when(i == 0)
        def _():
            for cp in small_copies():
                cp.start()
            x_copy(0).start()

        @pl.when(i == 1)
        def _():
            for cp in first_copies():
                cp.start()

        @pl.when(jnp.logical_and(i >= 2, i < 18))
        def _():
            q_copies(i - 2, lambda cp: cp.start())

        @pl.when(i == 18)
        def _():
            for cp in unit_copies(4) + [x_copy(1)]:
                cp.start()

        @pl.when(i == 19)
        def _():
            for cp in unit_copies(5):
                cp.start()
        return carry

    jax.lax.fori_loop(0, 20, issue, 0)
    zero_s[0] = 0
    g_v[...] = jnp.zeros(g_v.shape, U32)
    x1_v[...] = jnp.zeros(x1_v.shape, F32)

    ri = jax.lax.broadcasted_iota(jnp.int32, (80, 128), 0)
    ci = jax.lax.broadcasted_iota(jnp.int32, (80, 128), 1)

    def head_of(i):
        return jnp.where(i < 64, i // 32, (i - 64) // 8)

    def pos_of(i):
        return jnp.where(i < 64, i % 32, 32 + (i - 64) % 8)

    same = head_of(ri) == head_of(ci)
    pr, pc = pos_of(ri), pos_of(ci)
    keep = jnp.logical_or(pr < M, pr >= pc)
    code_v[...] = jnp.where(same, jnp.where(keep, 0.0, -1e9), -jnp.inf).astype(F32)

    for cp in small_copies():
        cp.wait()
    cf = c_v[...].astype(F32)
    sc_v[...] = _pack(jnp.broadcast_to(cf * jax.nn.sigmoid(cf), (16, D)))
    bias_v[:, 0:FF] = jnp.broadcast_to(b1_v[...].astype(F32).reshape(1, FF), (8, FF))
    bias_v[:, FF:] = jnp.broadcast_to(b2_v[...].astype(F32).reshape(1, D), (8, D))

    x_copy(0).wait()

    def xh_body(i, carry):
        for h in range(2):
            s0 = pl.multiple_of((i * 2 + h) * 8, 8)
            xh = _ln(x_v[pl.ds(s0, 8), 24:32, :].astype(F32).reshape(64, D))
            r0 = pl.multiple_of((i * 2 + h) * 64, 64)
            for kt in range(8):
                xh_v[kt, pl.ds(r0, 64), :] = xh[:, kt * 128:(kt + 1) * 128]
        return carry

    jax.lax.fori_loop(0, 4, xh_body, 0)

    def mod_slab(i):
        modq_v[i] = _dot(_unpack(sc_v[...]), wcol(wm0_v, i))[0:8]

    def h3_store(dst, kt, mc):
        sa = modq_v[2 * kt, 0:1, :]
        ca = modq_v[2 * kt + 1, 0:1, :]
        dst[:, mc * 128:(mc + 1) * 128] = _pack(
            xh_v[kt, mc * 128:(mc + 1) * 128, :] * (1.0 + ca) + sa)

    for cp in first_copies():
        cp.wait()
    modq_v[2:16] = jnp.zeros((14, 8, 128), F32)
    for i in range(2):
        mod_slab(i)
    for mc in range(4):
        h3_store(h3_v.at[0], 0, mc)
    relayout(stage.at[0, pl.ds(0, 128)], wqkv, 0, 64)

    def q_body(j, carry):
        q_copies(j, lambda cp: cp.wait())
        kt, hf = j >> 1, j & 1
        ktn = jnp.minimum(j + 1, 15) >> 1
        hfn = jnp.where(j < 15, (j + 1) & 1, 2)
        hview = h3_v.at[pl.ds(kt, 2)]
        wview = wqkv.at[pl.ds(pl.multiple_of(hf * (16 * PITCH) + kt * 64, 8), 16 * PITCH - 448), :]
        aview = acc_v.at[pl.ds(pl.multiple_of(hf * 8, 8), 8)]
        qsrc = stage.at[hfn, pl.ds(pl.multiple_of(ktn * 128, 128), 128)]
        qdst = wqkv.at[pl.ds(pl.multiple_of(hfn * (16 * PITCH) + ktn * 64, 8), 16 * PITCH + 64), :]
        jk = jnp.maximum(j - 1, 0)
        ksrc = stage.at[jnp.where(j > 0, 2, 0), pl.ds(pl.multiple_of(jk * 64, 64), 64)]
        kdst = wqkv.at[pl.ds(pl.multiple_of(32 * PITCH + jk * 32, 8), 16 * PITCH + 32), :]
        for p in range(8):
            lhs = jnp.concatenate([hview[0, :, mc * 128:(mc + 1) * 128] for mc in range(4)], axis=0)
            y = _dot(_unpack(lhs), wpair(wview, 2 * p, 64))
            aview[p] = jnp.where(kt > 0, aview[p], 0.0) + y
            if p == 1:
                mod_slab(jnp.minimum(j + 2, 15))
            if p >= 4:
                h3_store(hview.at[1], jnp.minimum(kt + 1, 7), p - 4)
            if p in QREL:
                relayout(qsrc, qdst, *QREL[p][0])
                relayout(ksrc, kdst, *QREL[p][1])
        return carry

    jax.lax.fori_loop(0, 16, q_body, 0)
    for kt in range(8):
        mod_v[:, kt * 128:(kt + 1) * 128] = modq_v[2 * kt]
        mod_v[:, D + kt * 128:D + (kt + 1) * 128] = modq_v[2 * kt + 1]
    for cp in unit_copies(6):
        cp.start()
    x_copy(1).wait()

    def ln1(xb):
        return _ln(xb.astype(F32)) * (1.0 + modrow(1)) + modrow(0)

    def store_x3(dst, half, mc, y):
        y = y.reshape(16, 8, 256)
        y = jnp.concatenate([y[:, :, :128], y[:, :, 128:]], axis=1).reshape(256, DH)
        dst[mc * 128:(mc + 1) * 128, half * DH:(half + 1) * DH] = _pack(y)

    def unit_body(u, carry):
        gn = jnp.minimum((u >> 1) + 1, 5)
        src = stage.at[gn & (NSTAGE - 1), pl.ds(pl.multiple_of((u & 1) * 512, 512), 512)]
        wm = wm1_v.at[pl.ds(4 * (u - 4), 4)]
        pltpu.make_async_copy(wm, wm, sem_u.at[u - 4]).wait()

        @pl.when(u < 10)
        def _():
            pltpu.make_async_copy(src, src, sem_u.at[u + 4]).wait()

        for k, cps in [(7, w1_copies), (4, lambda: unit_copies(7) + unit_copies(8)),
                       (5, lambda: unit_copies(9) + unit_copies(10) + unit_copies(11)),
                       (6, wo_copies), (8, w2_copies), (9, lambda: [x_copy(2)])]:
            @pl.when(u == k)
            def _(cps=cps):
                for cp in cps():
                    cp.start()

        lhs_v[...] = _pack(jnp.concatenate([mem0_v[...].astype(F32), ln1(x_v[0, 0:24, :])], axis=0))
        dst = wqkv.at[pl.ds(pl.multiple_of(gn * (16 * PITCH) + (u & 1) * 256, 8), 16 * PITCH + 256), :]
        view = wqkv.at[pl.ds(pl.multiple_of(u * (8 * PITCH), 8), 8 * PITCH), :]
        for p in range(4):
            for mc in range(4):
                lhs = _unpack(jnp.concatenate(
                    [h3_v[kt, :, mc * 128:(mc + 1) * 128] for kt in range(8)], axis=1))
                store_x3(qkv3.at[2 * u + p // 2], p % 2, mc, _dot(lhs, wpair(view, 2 * p)))
                relayout(src, dst, 64 * p + UREL[mc], 64 * p + UREL[mc + 1])
                if mc == 1:
                    modr_v[4 * (u - 4) + p] = _dot(_unpack(sc_v[...]), wcol(wm, p))[0:8]
                if p % 2 == 0:
                    store_x3(qkv3.at[u - 4], p // 2, mc,
                             acc_v[2 * (u - 4) + p // 2, mc * 128:(mc + 1) * 128, :])
        return carry

    jax.lax.fori_loop(4, 12, unit_body, 0)

    for cp in wo_copies():
        cp.wait()
    for j in range(32):
        mod_v[:, 2 * D + j * 128:2 * D + (j + 1) * 128] = modr_v[j]

    zpad = jnp.zeros((24, DH), U32)

    def proj(gg, mat):
        y = None
        for kt in range(0, 8, 2):
            w = jnp.concatenate(
                [_unpack(wqkv[pl.ds((mat * H + 4 * gg + i) * PITCH + 64 * kt, 128), :])
                 for i in range(4)], axis=1)
            d = _dot(_unpack(lhs_v[:, kt * 128:(kt + 2) * 128]), w)
            y = d if y is None else y + d
        for i in range(4):
            cs = pl.ds(((2 * gg + i // 2) * 3 + mat) * DH, DH)
            qkv_s[16 * (i % 2):16 * (i % 2 + 1), cs] = _pack(y[:, i * DH:(i + 1) * DH])

    def get(g, mat, seg):
        u3, p3 = divmod(mat * NPAIR + g, 2)
        parts = [qkv_s[:, pl.ds((g * 3 + mat) * DH, DH)],
                 qkv3[u3, pl.ds(mo(seg * 8, 8), 8), p3 * DH:(p3 + 1) * DH]]
        if mat > 0:
            parts.append(zpad)
        return _unpack(jnp.concatenate(parts, axis=0))

    def scores(g, seg):
        s = _dot_nt(get(g, 0, seg), get(g, 1, seg)) * SCALE
        code = code_v[...]
        s = jnp.where(code == 0.0, s, code)
        e = jnp.exp(s - jnp.max(s, axis=-1, keepdims=True))
        l = jnp.sum(e, axis=-1, keepdims=True)
        p_s[:, pl.ds(g * DH, DH)] = _pack(e * (1.0 / l))

    def pv(g, seg, second):
        o = _dot(_unpack(p_s[:, pl.ds(g * DH, DH)]), get(g, 2, seg))
        c0, c1 = (h * DH for h in _pair_heads(g))
        obuf[0:16, c0:c0 + DH] = _pack(o[0:32])
        obuf[0:16, c1:c1 + DH] = _pack(o[32:64])
        if not second:
            o3a[:, c0:c0 + DH] = o[64:72]
            o3a[:, c1:c1 + DH] = o[72:80]
        else:
            obuf[16:24, c0:c0 + DH] = _pack(jnp.concatenate([o3a[:, c0:c0 + DH], o[64:72]], axis=0))
            obuf[16:24, c1:c1 + DH] = _pack(jnp.concatenate([o3a[:, c1:c1 + DH], o[72:80]], axis=0))

    def wo_cols(pairs):
        return sorted(h for g in pairs for h in _pair_heads(g))

    def wo_dot(j, heads, nrow):
        lhs = jnp.concatenate([obuf[0:nrow, h * DH:(h + 1) * DH] for h in heads], axis=1)
        wu = wo_v.at[j].bitcast(U32)
        w = jnp.concatenate([wu[h * 64:(h + 1) * 64, :] for h in heads], axis=0)
        return _dot(_unpack(lhs), _unpack(w))

    def next_rows(seg):
        z = pl.multiple_of(zero_s[0], 8)
        obuf[pl.ds(24 + z, 24), 0:D] = pltpu.bitcast(ln1(x_v[seg, 0:24, :]), U32)

    def step(seg, second, fillers):
        part = functools.partial
        nrow = 24 if second else 16
        wsplit = 0 if fillers else WSPLIT0
        early, late = wo_cols(range(NPAIR - wsplit)), wo_cols(range(NPAIR - wsplit, NPAIR))

        def wo_early(j):
            wacc[0:2 * nrow, j * 128:(j + 1) * 128] = wo_dot(j, early, nrow)

        def wo_final(j):
            cs = slice(j * 128, (j + 1) * 128)
            if wsplit:
                y = wacc[0:2 * nrow, cs] + wo_dot(j, late, nrow)
            else:
                y = wo_dot(j, early, nrow)
            hn = pltpu.bitcast(obuf[24:48, cs], F32)
            lhs_v[:, cs] = _pack(jnp.concatenate([y[0:8], hn], axis=0))
            ga = mod_v[0:1, 2 * D + j * 128:2 * D + (j + 1) * 128]
            res = lambda sg, r0, n, yy: x_v[sg, r0:r0 + n, cs].astype(F32) + ga * yy
            if not second:
                x1n_v[0:24, cs] = res(seg, 0, 24, y[8:32])
            else:
                x1n_v[32:56, cs] = res(seg, 0, 24, y[8:32])
                x1n_v[24:32, cs] = res(seg - 1, 24, 8, y[32:40])
                x1n_v[56:64, cs] = res(seg, 24, 8, y[40:48])

        ev = list(fillers)
        for gg in range(NPAIR // 2):
            ev += [(2 * gg + 0.66 * mat, part(proj, gg, mat)) for mat in range(3)]
        for g in range(NPAIR):
            ev.append((SCORE_KEYS[second][g] if fillers else g + SOFF0, part(scores, g, seg)))
            ev.append((PV_KEYS[second][g] if fillers else g + POFF0, part(pv, g, seg, second)))
        ev.append((NEXT_KEYS[second] if fillers else NEXT0,
                   part(next_rows, jnp.minimum(seg + 1, NSEG - 1))))
        if wsplit:
            ev += [(WEARLY0[j], part(wo_early, j)) for j in range(8)]
        ev += [(100 + j, part(wo_final, j)) for j in range(8)]
        ev.sort(key=lambda e: e[0])
        for _, f in ev:
            f()

    def ffn_pre():
        x1 = x1n_v[...]
        x1_v[...] = x1
        h2_v[...] = _pack(_ln(x1) * (1.0 + modrow(4)) + modrow(3))

    def ffn1(j):
        cs = slice(j * 128, (j + 1) * 128)
        y = _dot(_unpack(h2_v[...]), wcol(w1_v, j)) + bias_v[0:1, cs]
        g_v[:, cs] = _pack(jax.nn.gelu(y, approximate=True))

    def ffn2(tp, j):
        cs = slice(j * 128, (j + 1) * 128)
        y = _dot(_unpack(g_v[...]), wcol(w2_v, j)) + bias_v[0:1, FF + j * 128:FF + (j + 1) * 128]
        o = x1_v[:, cs] + mod_v[0:1, 5 * D + j * 128:5 * D + (j + 1) * 128] * y
        out_v[tp, :, cs] = o.astype(BF16)

    step(0, False, [])
    step(1, True, [])
    for cp in w1_copies() + w2_copies():
        cp.wait()

    def body(t, carry):
        @pl.when(t == 2)
        def _():
            x_copy(2).wait()

        part = functools.partial
        held = [(HELD_KEY, part(ffn2, jnp.maximum(t - 2, 0), 7)), (HELD_KEY + 0.01, ffn_pre)]
        step(2 * t, False, held + [(k, part(ffn1, j)) for j, k in enumerate(FFN1_KEYS)])
        step(2 * t + 1, True, [(k, part(ffn2, t - 1, j)) for j, k in enumerate(FFN2_KEYS)])

        @pl.when(t >= 2)
        def _():
            pltpu.make_async_copy(out_v.at[t - 2], out_hbm.at[t - 2], sem_out.at[0]).start()
        return carry

    jax.lax.fori_loop(1, NDS, body, 0)

    ffn2(NDS - 2, 7)
    pltpu.make_async_copy(out_v.at[NDS - 2], out_hbm.at[NDS - 2], sem_out.at[0]).start()
    ffn_pre()
    for j in range(FF // 128):
        ffn1(j)
    for lo, hi in [(0, 5), (5, 7), (7, 8)]:
        for j in range(lo, hi):
            ffn2(NDS - 1, j)
        cols = pl.ds(lo * 128, (hi - lo) * 128)
        pltpu.make_async_copy(out_v.at[NDS - 1, :, cols], out_hbm.at[NDS - 1, :, cols],
                              sem_out.at[0]).start()
    pltpu.make_async_copy(out_v, out_hbm, sem_out.at[0]).wait()


@jax.jit
def pallas_adaLN_cond__memory_aug_recurrent_mem_tr__dense_activation_gelu__prompt_kernel(
    A_x, A_mem0, A_Wq, A_Wk, A_Wv, A_Wo, A_seg_len, B_x, B_w1, B_b1, B_w2, B_b2, c, w_mod,
):
    del A_seg_len, B_x
    assert A_x.shape == (1, S, D) and A_mem0.shape == (1, M, D)
    assert A_Wq.shape == (D, H, DH) and B_w1.shape == (D, FF)
    any_spec = pl.BlockSpec(memory_space=pl.ANY)
    scratch = [
        pltpu.VMEM((NSEG, SEG, D), BF16),
        pltpu.VMEM((NSEG // 2, 2 * SEG, D), BF16),
        pltpu.VMEM((NSTAGE, D, 16, DH), BF16),
        pltpu.VMEM(((3 * H + 1) * PITCH, DH), U32),
        pltpu.VMEM((8, H * DH, 128), BF16),
        pltpu.VMEM((FF // 128, D, 128), BF16),
        pltpu.VMEM((8, FF, 128), BF16),
        pltpu.VMEM((16, D, 128), BF16),
        pltpu.VMEM((32, D, 128), BF16),
        pltpu.VMEM((M, D), BF16),
        pltpu.VMEM((FF,), BF16),
        pltpu.VMEM((D,), BF16),
        pltpu.VMEM((1, D), BF16),
        pltpu.VMEM((8, 6 * D), F32),
        pltpu.VMEM((16, 8, 128), F32),
        pltpu.VMEM((32, 8, 128), F32),
        pltpu.VMEM((8, D), U32),
        pltpu.VMEM((8, FF + D), F32),
        pltpu.VMEM((8, NSEG * 8, 128), F32),
        pltpu.VMEM((9, 64, 512), U32),
        pltpu.VMEM((NPAIR, NSEG * 8, 2 * DH), F32),
        pltpu.VMEM((24, NSEG * 8, 2 * DH), U32),
        pltpu.VMEM((80, 128), F32),
        pltpu.VMEM((16, D), U32),
        pltpu.VMEM((32, NPAIR * 3 * DH), U32),
        pltpu.VMEM((40, NPAIR * DH), U32),
        pltpu.VMEM((48, D), F32),
        pltpu.VMEM((48, H * DH), U32),
        pltpu.VMEM((8, H * DH), F32),
        pltpu.VMEM((64, D), F32),
        pltpu.VMEM((64, D), F32),
        pltpu.VMEM((32, D), U32),
        pltpu.VMEM((32, FF), U32),
        pltpu.SMEM((1,), jnp.int32),
        pltpu.SemaphoreType.DMA((4,)),
        pltpu.SemaphoreType.DMA((3,)),
        pltpu.SemaphoreType.DMA((17,)),
        pltpu.SemaphoreType.DMA((14,)),
        pltpu.SemaphoreType.DMA((3,)),
        pltpu.SemaphoreType.DMA((1,)),
    ]
    out = pl.pallas_call(
        _kernel,
        out_shape=jax.ShapeDtypeStruct((NSEG // 2, 2 * SEG, D), BF16),
        in_specs=[any_spec] * 12,
        out_specs=any_spec,
        scratch_shapes=scratch,
        compiler_params=pltpu.CompilerParams(vmem_limit_bytes=120 * 1024 * 1024,
                                             disable_bounds_checks=not CHECKS,
                                             disable_semaphore_checks=not CHECKS),
    )(
        A_x.reshape(NSEG, SEG, D), A_mem0.reshape(M, D), A_Wq, A_Wk, A_Wv,
        A_Wo.reshape(H * DH, D), B_w1, B_b1, B_w2, B_b2,
        c, w_mod,
    )
    return out.reshape(1, S, D)
```
